```python
import jax
import jax.numpy as jnp

def _softmax(x, axis=-1):
    return jax.nn.softmax(x, axis=axis)
def _gelu(x):
    return jax.nn.gelu(x, approximate=True)
def _silu(x):
    return jax.nn.silu(x)
def _sigmoid(x):
    return jax.nn.sigmoid(x)
def _layernorm(x, axis=-1, eps=1e-5):
    m = jnp.mean(x, axis=axis, keepdims=True)
    v = jnp.var(x, axis=axis, keepdims=True)
    return (x - m) / jnp.sqrt(v + eps)
def _scatter_add(tgt, idx, src, axis=0):
    return tgt.at[idx].add(src)
def _segment_sum(src, seg, n):
    return jax.ops.segment_sum(src, seg, n)
class _Rng:
    def __init__(self, key):
        self._k = key
    def _next(self):
        self._k, sub = jax.random.split(self._k)
        return sub
    def normal(self, shape):
        return jax.random.normal(self._next(), shape, dtype=jnp.bfloat16)
    def randint(self, lo, hi, shape):
        return jax.random.randint(self._next(), shape, lo, hi, dtype=jnp.int32)
    def uniform(self, shape, lo=0.0, hi=1.0):
        return jax.random.uniform(self._next(), shape, jnp.bfloat16, lo, hi)
    def permutation(self, n):
        return jax.random.permutation(self._next(), n)


kernel_name = 'gated_mix__compressed_kv_cla__sliding_block_cached__decode'

def setup_inputs():
    _rng = _Rng(jax.random.key(int.from_bytes(__import__("os").urandom(4), "little")))
    _w = (lambda a: (lambda t: t.astype(jnp.bfloat16) if jnp.issubdtype(t.dtype, jnp.floating) else t)(jnp.asarray(a)))
    def _A_setup():
        B, H, Sq, Sk, D, M = 8, 32, 1, 4096, 128, 512
        Dc = 4 * D
        return {
            "x": _w((lambda *s: _rng.normal(s) * 0.05)(B, Sq, M)),
            "c_kv": _w((lambda *s: _rng.normal(s) * 0.05)(B, Sk, Dc)),
            "w_q": _w((lambda *s: _rng.normal(s) * 0.05)(M, H, D) * (M ** -0.5)),
            "w_uk": _w((lambda *s: _rng.normal(s) * 0.05)(Dc, H, D) * (Dc ** -0.5)),
            "w_uv": _w((lambda *s: _rng.normal(s) * 0.05)(Dc, H, D) * (Dc ** -0.5)),
            "w_o": _w((lambda *s: _rng.normal(s) * 0.05)(H, D, M) * ((H * D) ** -0.5)),
        }
    _A_in = _A_setup()

    def _B_setup():
        B, Sq, D = 8, 1, 512
        Hq, Hkv, Sk, Dh = 32, 8, 4096, 128
        assert Hq % Hkv == 0, (Hq, Hkv)
        return {
            "x": _w((lambda *s: _rng.normal(s) * 0.05)(B, Sq, D)),
            "k_cache": _w((lambda *s: _rng.normal(s) * 0.05)(B, Hkv, Sk, Dh)),
            "v_cache": _w((lambda *s: _rng.normal(s) * 0.05)(B, Hkv, Sk, Dh)),
            "wq": _w((lambda *s: _rng.normal(s) * 0.05)(D, Hq * Dh) * (D ** -0.5)),
            "wo": _w((lambda *s: _rng.normal(s) * 0.05)(Hq * Dh, D) * ((Hq * Dh) ** -0.5)),
        }
    _B_in = _B_setup()

    return {
        "A_x": _A_in["x"],
        "A_c_kv": _A_in["c_kv"],
        "A_w_q": _A_in["w_q"],
        "A_w_uk": _A_in["w_uk"],
        "A_w_uv": _A_in["w_uv"],
        "A_w_o": _A_in["w_o"],
        "B_x": _B_in["x"],
        "B_k_cache": _B_in["k_cache"],
        "B_v_cache": _B_in["v_cache"],
        "B_wq": _B_in["wq"],
        "B_wo": _B_in["wo"],
        "gate_w": _w((lambda *s: _rng.normal(s) * 0.05)(512)),
    }

def reference(A_x, A_c_kv, A_w_q, A_w_uk, A_w_uv, A_w_o, B_x, B_k_cache, B_v_cache, B_wq, B_wo, gate_w):
    def _A_ref(x, c_kv, w_q, w_uk, w_uv, w_o):
        B, Sq, M = x.shape[0], x.shape[1], x.shape[2]
        Sk = c_kv.shape[1]
        H, D = w_q.shape[1], w_q.shape[2]
        q = jnp.einsum("bqm,mhd->bhqd", x, w_q)
        k = jnp.einsum("bkc,chd->bhkd", c_kv, w_uk)
        v = jnp.einsum("bkc,chd->bhkd", c_kv, w_uv)
        scores = jnp.einsum("bhqd,bhkd->bhqk", q, k) * (D ** -0.5)
        off = Sk - Sq
        qi = jnp.arange(Sq)[:, None]
        kj = jnp.arange(Sk)[None, :]
        cmask = kj <= (qi + off)
        scores = jnp.where(cmask[None, None], scores, -1e9)
        p = _softmax(scores, axis=-1)
        ctx = jnp.einsum("bhqk,bhkd->bhqd", p, v)
        return jnp.einsum("bhqd,hdm->bqm", ctx, w_o)

    def _B_ref(x, k_cache, v_cache, wq, wo):
        B, Sq, D = x.shape
        Hq, Dh = 32, 128
        Hkv, Sk = k_cache.shape[1], k_cache.shape[2]
        W = min(4096, max(256, Sk // 4))
        rep = Hq // Hkv
        q = (lambda x, *d: x.transpose(*d))((x @ wq).reshape(B, Sq, Hq, Dh), 0, 2, 1, 3)
        k = jnp.repeat(k_cache[:, :, Sk - W:, :], rep, axis=1)
        v = jnp.repeat(v_cache[:, :, Sk - W:, :], rep, axis=1)
        scores = jnp.einsum("bhqd,bhkd->bhqk", q, k) * (Dh ** -0.5)
        p = _softmax(scores, axis=-1)
        o = jnp.einsum("bhqk,bhkd->bhqd", p, v)
        return (lambda x, *d: x.transpose(*d))(o, 0, 2, 1, 3).reshape(B, Sq, Hq * Dh) @ wo

    x = A_x
    g = _sigmoid((x * gate_w).sum(-1, keepdims=True))
    a = _A_ref(x, A_c_kv, A_w_q, A_w_uk, A_w_uv, A_w_o)
    b = _B_ref(x, B_k_cache, B_v_cache, B_wq, B_wo)
    return g * a + (1 - g) * b
```

```python
import jax
import jax.numpy as jnp
import jax.experimental.pallas as pl
import jax.experimental.pallas.tpu as pltpu

F32 = jnp.float32
BF16 = jnp.bfloat16
U32 = jnp.uint32

_NT = (((1,), (1,)), ((), ()))


def _head_pair(w_u32, j, rows, heads):
    half = heads // 2
    ev = w_u32[pl.ds(j, rows // 2, stride=heads), :]
    od = w_u32[pl.ds(j + half, rows // 2, stride=heads), :]
    lo = (ev & jnp.uint32(0xFFFF)) | (od << 16)
    hi = (ev >> 16) | (od & jnp.uint32(0xFFFF0000))
    return pltpu.bitcast(lo, BF16), pltpu.bitcast(hi, BF16)


def _make_kernel(B, M, H, D, Dc, Sk, Hkv, SkB, W, ckv_splits, k_splits, v_splits, wo_splits):
    rep = H // Hkv
    scale = float(D) ** -0.5

    def kernel(x_h, gw_h, ckv_h, wq_h, wuk_h, wuv_h, wo_h, kc_h, vc_h, bwq_h, bwo_h,
               o_ref,
               x_v, gw_v, ckv_v, wq_v, wuk_v, wuv_v, wo_v, kc_v, vc_v, bwq_v, bwo_v,
               qabs_s, lat_s, ctx_s, qb_s, p_s, ob_s, sems):
        copies = []

        def add(src, dst):
            c = pltpu.make_async_copy(src, dst, sems.at[len(copies)])
            copies.append(c)
            c.start()
            return c

        c_x = add(x_h, x_v)
        c_wq = add(wq_h, wq_v.bitcast(BF16))
        c_wuk = add(wuk_h, wuk_v.bitcast(BF16))
        c_gw = add(gw_h, gw_v)
        c_ckv = []
        b0 = 0
        for n in ckv_splits:
            c_ckv.append((b0, n, add(ckv_h.at[pl.ds(b0, n)], ckv_v.at[pl.ds(b0, n)])))
            b0 += n
        c_bwq = add(bwq_h, bwq_v)
        c_wuv = add(wuv_h, wuv_v.bitcast(BF16))
        c_k = []
        b0 = 0
        for n in k_splits:
            c_k.append((b0, n, add(kc_h.at[pl.ds(b0, n), :, pl.ds(SkB - W, W)], kc_v.at[pl.ds(b0, n)])))
            b0 += n
        c_v = []
        b0 = 0
        for n in v_splits:
            c_v.append((b0, n, add(vc_h.at[pl.ds(b0, n), :, pl.ds(SkB - W, W)], vc_v.at[pl.ds(b0, n)])))
            b0 += n
        c_wo = add(wo_h, wo_v)
        c_bwo = []
        r0 = 0
        for n in wo_splits:
            c_bwo.append((r0, n, add(bwo_h.at[pl.ds(r0, n)], bwo_v.at[pl.ds(r0, n)])))
            r0 += n

        c_x.wait()
        c_wq.wait()
        c_wuk.wait()
        x = x_v[...]
        wq_u = wq_v
        wuk_u = wuk_v

        def qabs_body(j, carry):
            wq0, wq1 = _head_pair(wq_u, j, M, H)
            wk0, wk1 = _head_pair(wuk_u, j, Dc, H)
            for p, (wq_, wk_) in enumerate(((wq0, wk0), (wq1, wk1))):
                q = jnp.dot(x, wq_, preferred_element_type=F32).astype(BF16)
                qa = jax.lax.dot_general(q, wk_, _NT, preferred_element_type=F32)
                row = pl.multiple_of((2 * j + p) * B, B)
                qa = qa * scale
                for t in range(Dc // 128):
                    qabs_s[t, pl.ds(row, B), :] = qa[:, t * 128:(t + 1) * 128]
            return carry

        jax.lax.fori_loop(0, H // 2, qabs_body, 0)

        def attn_a(b, carry):
            qa = jnp.concatenate(
                [qabs_s[t, pl.ds(b, H, stride=B), :] for t in range(Dc // 128)],
                axis=1).astype(BF16)
            c = ckv_v[b]
            s = jax.lax.dot_general(qa, c, _NT, preferred_element_type=F32)
            m = jnp.max(s, axis=-1, keepdims=True)
            p = jnp.exp(s - m)
            l = jnp.sum(p, axis=-1, keepdims=True)
            lat = jnp.dot(p.astype(BF16), c, preferred_element_type=F32)
            lat = lat / l
            row = pl.multiple_of(b * H, H)
            for t in range(Dc // 128):
                lat_s[t, pl.ds(row, H), :] = lat[:, t * 128:(t + 1) * 128]
            return carry

        for b0, n, c in c_ckv:
            c.wait()
            jax.lax.fori_loop(b0, b0 + n, attn_a, 0)

        c_bwq.wait()
        qb = jnp.dot(x, bwq_v[...], preferred_element_type=F32)
        qb = qb.astype(BF16).astype(F32)
        for h in range(H):
            qb_s[h * B:(h + 1) * B, :] = qb[:, h * D:(h + 1) * D]

        c_wuv.wait()
        wuv_u = wuv_v

        def ctx_body(j, carry):
            wv = _head_pair(wuv_u, j, Dc, H)
            for p in range(2):
                lat = jnp.concatenate(
                    [lat_s[t, pl.ds(2 * j + p, B, stride=H), :] for t in range(Dc // 128)],
                    axis=1).astype(BF16)
                ctx_s[2 * j + p] = jnp.dot(lat, wv[p], preferred_element_type=F32)
            return carry

        jax.lax.fori_loop(0, H // 2, ctx_body, 0)

        npair = Hkv // 2
        first = jax.lax.broadcasted_iota(jnp.int32, (2 * rep, 1), 0) < rep

        def qk_b(i, carry):
            b = i // npair
            g = (i % npair) * 2
            q = qb_s[pl.ds(g * rep * B + b, 2 * rep, stride=B), :].astype(BF16)
            s0 = jax.lax.dot_general(q, kc_v[b, g], _NT, preferred_element_type=F32)
            s1 = jax.lax.dot_general(q, kc_v[b, g + 1], _NT, preferred_element_type=F32)
            s = jnp.where(first, s0, s1) * scale
            m = jnp.max(s, axis=-1, keepdims=True)
            p = jnp.exp(s - m)
            l = jnp.sum(p, axis=-1, keepdims=True)
            p_s[i] = p / l
            return carry

        for b0, n, c in c_k:
            c.wait()
            jax.lax.fori_loop(b0 * npair, (b0 + n) * npair, qk_b, 0)

        def pv_b(i, carry):
            b = i // npair
            g = (i % npair) * 2
            p = p_s[i].astype(BF16)
            o0 = jnp.dot(p, vc_v[b, g], preferred_element_type=F32)
            o1 = jnp.dot(p, vc_v[b, g + 1], preferred_element_type=F32)
            row = pl.multiple_of(i * 2 * rep, 2 * rep)
            ob_s[pl.ds(row, 2 * rep), :] = jnp.where(first, o0, o1)
            return carry

        for b0, n, c in c_v:
            c.wait()
            jax.lax.fori_loop(b0 * npair, (b0 + n) * npair, pv_b, 0)

        c_gw.wait()
        xf = x.astype(F32)
        gw = gw_v[...].astype(F32)
        t = xf[:, 0:128] * gw[0:1, :]
        for i in range(1, M // 128):
            t = t + xf[:, i * 128:(i + 1) * 128] * gw[i:i + 1, :]
        gate = jax.nn.sigmoid(jnp.sum(t, axis=-1, keepdims=True))

        ob = jnp.concatenate(
            [ob_s[pl.ds(h, B, stride=H), :] for h in range(H)], axis=1).astype(BF16)
        ctx = jnp.concatenate([ctx_s[h] for h in range(H)], axis=1).astype(BF16)
        c_wo.wait()
        a = jnp.dot(ctx, wo_v[...], preferred_element_type=F32)
        acc = jnp.zeros((B, M), F32)
        for r0, n, c in c_bwo:
            c.wait()
            acc = acc + jnp.dot(ob[:, r0:r0 + n], bwo_v[r0:r0 + n, :], preferred_element_type=F32)
        o_ref[...] = (gate * a + (1.0 - gate) * acc).astype(o_ref.dtype)

    return kernel


@jax.jit
def pallas_gated_mix__compressed_kv_cla__sliding_block_cached__decode_kernel(
    A_x: jax.Array,
    A_c_kv: jax.Array,
    A_w_q: jax.Array,
    A_w_uk: jax.Array,
    A_w_uv: jax.Array,
    A_w_o: jax.Array,
    B_x: jax.Array,
    B_k_cache: jax.Array,
    B_v_cache: jax.Array,
    B_wq: jax.Array,
    B_wo: jax.Array,
    gate_w: jax.Array,
):
    B, Sq, M = A_x.shape
    assert Sq == 1
    _, Sk, Dc = A_c_kv.shape
    _, H, D = A_w_q.shape
    _, Hkv, SkB, _ = B_k_cache.shape
    W = min(4096, max(256, SkB // 4))
    rep = H // Hkv

    ckv_splits = (2, 2, 2, 2)
    k_splits = (4, 4)
    v_splits = (4, 4)
    wo_splits = (2048, 1024, 512, 256, 128, 128)
    n_dma = 7 + len(ckv_splits) + len(k_splits) + len(v_splits) + len(wo_splits)

    kernel = _make_kernel(B, M, H, D, Dc, Sk, Hkv, SkB, W,
                          ckv_splits, k_splits, v_splits, wo_splits)
    any_spec = pl.BlockSpec(memory_space=pl.ANY)
    out = pl.pallas_call(
        kernel,
        out_shape=jax.ShapeDtypeStruct((B, M), A_x.dtype),
        in_specs=[any_spec] * 11,
        out_specs=pl.BlockSpec(memory_space=pltpu.VMEM),
        scratch_shapes=[
            pltpu.VMEM((B, M), BF16),
            pltpu.VMEM((M // 128, 128), BF16),
            pltpu.VMEM((B, Sk, Dc), BF16),
            pltpu.VMEM((M * H // 2, D), U32),
            pltpu.VMEM((Dc * H // 2, D), U32),
            pltpu.VMEM((Dc * H // 2, D), U32),
            pltpu.VMEM((H * D, M), BF16),
            pltpu.VMEM((B, Hkv, W, D), BF16),
            pltpu.VMEM((B, Hkv, W, D), BF16),
            pltpu.VMEM((M, H * D), BF16),
            pltpu.VMEM((H * D, M), BF16),
            pltpu.VMEM((Dc // 128, H * B, 128), F32),
            pltpu.VMEM((Dc // 128, B * H, 128), F32),
            pltpu.VMEM((H, B, D), F32),
            pltpu.VMEM((H * B, D), F32),
            pltpu.VMEM((B * Hkv // 2, 2 * rep, W), F32),
            pltpu.VMEM((B * H, D), F32),
            pltpu.SemaphoreType.DMA((n_dma,)),
        ],
        compiler_params=pltpu.CompilerParams(vmem_limit_bytes=112 * 1024 * 1024),
        name="gated_mix_decode",
    )(
        A_x.reshape(B, M),
        gate_w.reshape(M // 128, 128),
        A_c_kv,
        A_w_q.reshape(M * H, D),
        A_w_uk.reshape(Dc * H, D),
        A_w_uv.reshape(Dc * H, D),
        A_w_o.reshape(H * D, M),
        B_k_cache,
        B_v_cache,
        B_wq,
        B_wo,
    )
    return out.reshape(B, 1, M)
```

```python
import jax
import jax.numpy as jnp
import jax.experimental.pallas as pl
import jax.experimental.pallas.tpu as pltpu

F32 = jnp.float32
BF16 = jnp.bfloat16
U32 = jnp.uint32

_NT = (((1,), (1,)), ((), ()))

NSTR = 8
BURST = 8


def _head_pair(w_u32, j, heads):
    ns, rr, d = w_u32.shape
    n = rr // heads
    ev = w_u32[:, pl.ds(j, n, stride=heads), :].reshape(ns * n, d)
    od = w_u32[:, pl.ds(j + heads // 2, n, stride=heads), :].reshape(ns * n, d)
    lo = (ev & jnp.uint32(0xFFFF)) | (od << 16)
    hi = (ev >> 16) | (od & jnp.uint32(0xFFFF0000))
    return pltpu.bitcast(lo, BF16), pltpu.bitcast(hi, BF16)


def _make_kernel(B, M, H, D, Dc, Sk, Hkv, SkB, W, cfg):
    rep = H // Hkv
    scale = float(D) ** -0.5
    HD = H * D
    CS = 4
    CR = Sk // CS
    OR = HD // NSTR
    tail_blocks = cfg["tail_blocks"]

    def kernel(x_h, gw_h, ckv_h, wq_h, wuk_h, wuv_h, wo_h, kc_h, vc_h, bwq_h, bwo_h,
               o_ref,
               x_v, gw_v, ckv_v, wq_v, wuk_v, wuv_v, wo_v, kc_v, vc_v, bwq_v, bwo_v,
               qabs_s, lat_s, ctx_s, qb_s, ob_s, sems):
        S_X, S_GW, S_WQ, S_WUK, S_BWQ, S_WUV, S_CKV, S_KV, S_W3 = 0, 1, 2, 3, 4, 5, 6, 8, 24

        def start(src, dst, sem, prio):
            pltpu.make_async_copy(src, dst, sems.at[sem]).start(priority=prio)

        def wait(buf, sem):
            pltpu.make_async_copy(buf, buf, sems.at[sem]).wait()

        wq_b, wuk_b, wuv_b = wq_v.bitcast(BF16), wuk_v.bitcast(BF16), wuv_v.bitcast(BF16)

        def rows16(src, dst, j, sem, prio):
            sl = (slice(None), pl.ds(pl.multiple_of(j * 16, 16), 16), slice(None))
            start(src.at[sl], dst.at[sl], sem, prio)

        def tiles2(src, dst, lead, j, ncb, sem, prio):
            r = pl.multiple_of((j // ncb) * 8, 8)
            c = pl.multiple_of((j % ncb) * 256, 256)
            sl = (lead, pl.ds(r, 8), pl.ds(c, 256))
            start(src.at[sl], dst.at[sl], sem, prio)

        def pair_w1(j):
            rows16(wq_h, wq_b, j, S_WQ, 0)
            rows16(wuk_h, wuk_b, j, S_WUK, 1)

        def pair_w2(j):
            tiles2(bwq_h, bwq_v, slice(None), j, HD // 256, S_BWQ, 0)
            rows16(wuv_h, wuv_b, j, S_WUV, 1)

        ckv_pairs = (CR // 8) * (Dc // 256)

        def pair_ckv(j):
            half = j // ckv_pairs
            jj = j % ckv_pairs
            for t in range(2):
                lead = pl.ds((2 * half + t) * NSTR, NSTR)
                tiles2(ckv_h, ckv_v, lead, jj, Dc // 256, S_CKV + half, t)

        kv_pairs = W // 16

        def pair_kv(j):
            b = j // kv_pairs
            r = pl.multiple_of((j % kv_pairs) * 16, 16)
            for t, (src, dst) in enumerate(((kc_h, kc_v), (vc_h, vc_v))):
                start(src.at[b, :, pl.ds(SkB - W + r, 16)], dst.at[b, :, pl.ds(r, 16)],
                      S_KV + 2 * b + t, t)

        w3_bands = OR // 128 - 1
        band_pairs = (128 // 8) * (M // 256)

        def pair_w3(j):
            band = j // band_pairs
            tiles2(wo_h, wo_v, slice(None), j, M // 256, S_W3 + 2 * band, 0)
            tiles2(bwo_h, bwo_v, slice(None), j, M // 256, S_W3 + 2 * band + 1, 1)

        plan = []
        u0 = 0
        for name, fn, npairs in (("w1", pair_w1, wq_b.shape[1] // 16),
                                 ("w2", pair_w2, wuv_b.shape[1] // 16),
                                 ("ckv", pair_ckv, 2 * ckv_pairs),
                                 ("kv", pair_kv, B * kv_pairs),
                                 ("w3", pair_w3, w3_bands * band_pairs)):
            assert npairs % BURST == 0
            plan.append((u0, npairs // BURST, fn))
            u0 += npairs // BURST
        n_bursts = u0

        def run_pairs(fn, j0, n):
            def body(i, c):
                fn(j0 + i)
                return c
            jax.lax.fori_loop(0, n, body, 0)

        def issue_static(lo, hi):
            for u0, n, fn in plan:
                a, b = max(lo, u0), min(hi, u0 + n)
                if a < b:
                    run_pairs(fn, (a - u0) * BURST, (b - a) * BURST)

        def issue_dyn(u, lo, hi):
            hits = [(u0, n, fn) for u0, n, fn in plan if u0 < hi and lo < u0 + n]
            for u0, n, fn in hits:
                if len(hits) == 1:
                    run_pairs(fn, (u - u0) * BURST, BURST)
                else:
                    @pl.when(jnp.logical_and(u >= u0, u < u0 + n))
                    def _(u0=u0, fn=fn):
                        run_pairs(fn, (u - u0) * BURST, BURST)

        class Cursor:
            pos = 0

            def to(self, hi):
                assert self.pos <= hi <= n_bursts, (self.pos, hi)
                issue_static(self.pos, hi)
                self.pos = hi

            def loop(self, iters, per_iter):
                lo, hi = self.pos, self.pos + iters * per_iter
                assert hi <= n_bursts
                self.pos = hi
                return lambda i, k: issue_dyn(lo + i * per_iter + k, lo, hi)

        cur = Cursor()

        start(x_h, x_v, S_X, 0)
        start(gw_h, gw_v, S_GW, 1)
        cur.to(cfg["u_qabs"])

        wait(x_v, S_X)
        wait(gw_v, S_GW)
        wait(wq_b, S_WQ)
        wait(wuk_b, S_WUK)
        nb = cfg["n_qabs"]
        iss = cur.loop(H // 2, nb)

        def qabs_body(j, carry):
            x = x_v[...]
            wq0, wq1 = _head_pair(wq_v, j, H)
            wk0, wk1 = _head_pair(wuk_v, j, H)
            for p, (wq_, wk_) in enumerate(((wq0, wk0), (wq1, wk1))):
                q = jnp.dot(x, wq_, preferred_element_type=F32).astype(BF16)
                qa = jax.lax.dot_general(q, wk_, _NT, preferred_element_type=F32)
                row = pl.multiple_of((2 * j + p) * B, B)
                qa = qa * scale
                for t in range(Dc // 128):
                    qabs_s[t, pl.ds(row, B), :] = qa[:, t * 128:(t + 1) * 128]
            for k in range(nb):
                iss(j, k)
            return carry

        jax.lax.fori_loop(0, H // 2, qabs_body, 0)

        wait(bwq_v, S_BWQ)
        wait(wuv_b, S_WUV)
        qb = jnp.dot(x_v[...], bwq_v[...].reshape(M, HD), preferred_element_type=F32)
        qb = qb.astype(BF16).astype(F32)
        for h in range(H):
            qb_s[h * B:(h + 1) * B, :] = qb[:, h * D:(h + 1) * D]

        cur.to(cfg["u_attn_a"])
        na1, na2 = cfg["n_attn_a"]
        iss_a = cur.loop(B, na1 + na2)
        half_b = B // 2

        def attn_a(b, carry):
            for half in range(2):
                @pl.when(b == half * half_b)
                def _(half=half):
                    wait(ckv_v.at[pl.ds(half * 2 * NSTR, 2 * NSTR)], S_CKV + half)

            qa = jnp.concatenate(
                [qabs_s[t, pl.ds(b, H, stride=B), :] for t in range(Dc // 128)],
                axis=1).astype(BF16)
            c = ckv_v[pl.ds(b * CS, CS)].reshape(Sk, Dc)
            s = jax.lax.dot_general(qa, c, _NT, preferred_element_type=F32)
            for k in range(na1):
                iss_a(b, k)
            m = jnp.max(s, axis=-1, keepdims=True)
            p = jnp.exp(s - m)
            l = jnp.sum(p, axis=-1, keepdims=True)
            c = ckv_v[pl.ds(b * CS, CS)].reshape(Sk, Dc)
            lat = jnp.dot(p.astype(BF16), c, preferred_element_type=F32)
            lat = lat / l
            row = pl.multiple_of(b * H, H)
            for t in range(Dc // 128):
                lat_s[t, pl.ds(row, H), :] = lat[:, t * 128:(t + 1) * 128]
            for k in range(na2):
                iss_a(b, na1 + k)
            return carry

        jax.lax.fori_loop(0, B, attn_a, 0)

        nc = cfg["n_ctx"]
        iss_c = cur.loop(H // 2, nc)

        def ctx_body(j, carry):
            wv = _head_pair(wuv_v, j, H)
            for p in range(2):
                lat = jnp.concatenate(
                    [lat_s[t, pl.ds(2 * j + p, B, stride=H), :] for t in range(Dc // 128)],
                    axis=1).astype(BF16)
                ctx_s[2 * j + p] = jnp.dot(lat, wv[p], preferred_element_type=F32)
            for k in range(nc):
                iss_c(j, k)
            return carry

        jax.lax.fori_loop(0, H // 2, ctx_body, 0)

        cur.to(cfg["u_attn_b"])
        nbb = cfg["n_attn_b"]
        iss_b = cur.loop(B, nbb)
        first = jax.lax.broadcasted_iota(jnp.int32, (2 * rep, 1), 0) < rep

        def attn_b(b, carry):
            for k in range(nbb):
                iss_b(b, k)
            wait(kc_v.at[b], S_KV + 2 * b)
            wait(vc_v.at[b], S_KV + 2 * b + 1)
            for g in range(0, Hkv, 2):
                q = qb_s[pl.ds(g * rep * B + b, 2 * rep, stride=B), :].astype(BF16)
                s0 = jax.lax.dot_general(q, kc_v[b, g], _NT, preferred_element_type=F32)
                s1 = jax.lax.dot_general(q, kc_v[b, g + 1], _NT, preferred_element_type=F32)
                s = jnp.where(first, s0, s1) * scale
                m = jnp.max(s, axis=-1, keepdims=True)
                p = jnp.exp(s - m)
                l = jnp.sum(p, axis=-1, keepdims=True)
                p = p.astype(BF16)
                o0 = jnp.dot(p, vc_v[b, g], preferred_element_type=F32)
                o1 = jnp.dot(p, vc_v[b, g + 1], preferred_element_type=F32)
                row = pl.multiple_of(b * H + g * rep, 2 * rep)
                ob_s[pl.ds(row, 2 * rep), :] = jnp.where(first, o0, o1) / l
            return carry

        jax.lax.fori_loop(0, B, attn_b, 0)
        cur.to(n_bursts)

        r_last = w3_bands * 128
        tail = []
        s0 = 0
        sem = S_W3 + 2 * w3_bands
        for ns in tail_blocks:
            rows = 32 // ns
            for r in range(r_last, r_last + 128, rows):
                sl = (pl.ds(s0, ns), pl.ds(r, rows), slice(None))
                start(wo_h.at[sl], wo_v.at[sl], sem, 0)
                start(bwo_h.at[sl], bwo_v.at[sl], sem + 1, 1)
            tail.append((s0, ns, sem))
            s0 += ns
            sem += 2

        xf = x_v[...].astype(F32)
        gw = gw_v[...].astype(F32)
        t = xf[:, 0:128] * gw[0:1, :]
        for i in range(1, M // 128):
            t = t + xf[:, i * 128:(i + 1) * 128] * gw[i:i + 1, :]
        gate = jax.nn.sigmoid(jnp.sum(t, axis=-1, keepdims=True))

        hs = OR // D
        ctx = [ctx_s[h].astype(BF16) for h in range(H)]
        ob = [ob_s[pl.ds(h, B, stride=H), :].astype(BF16) for h in range(H)]

        def proj(acc_a, acc_b, s0, ns, band):
            rs = pl.ds(band * 128, 128)
            la = jnp.concatenate([ctx[s * hs + band] for s in range(s0, s0 + ns)], axis=1)
            lb = jnp.concatenate([ob[s * hs + band] for s in range(s0, s0 + ns)], axis=1)
            wa = wo_v[pl.ds(s0, ns), rs, :].reshape(ns * 128, M)
            wb = bwo_v[pl.ds(s0, ns), rs, :].reshape(ns * 128, M)
            return (acc_a + jnp.dot(la, wa, preferred_element_type=F32),
                    acc_b + jnp.dot(lb, wb, preferred_element_type=F32))

        acc_a = jnp.zeros((B, M), F32)
        acc_b = jnp.zeros((B, M), F32)
        for band in range(w3_bands):
            rs = pl.ds(band * 128, 128)
            wait(wo_v.at[:, rs], S_W3 + 2 * band)
            wait(bwo_v.at[:, rs], S_W3 + 2 * band + 1)
            acc_a, acc_b = proj(acc_a, acc_b, 0, NSTR, band)
        for s0, ns, sem in tail:
            sl = (pl.ds(s0, ns), pl.ds(r_last, 128))
            wait(wo_v.at[sl], sem)
            wait(bwo_v.at[sl], sem + 1)
            acc_a, acc_b = proj(acc_a, acc_b, s0, ns, w3_bands)
        o_ref[...] = (gate * acc_a + (1.0 - gate) * acc_b).astype(o_ref.dtype)

    n_sems = 24 + 2 * (OR // 128 - 1) + 2 * len(tail_blocks)
    return kernel, n_sems


DEFAULT_CFG = dict(
    u_qabs=22, n_qabs=2,
    u_attn_a=78, n_attn_a=(3, 3),
    n_ctx=1,
    u_attn_b=142, n_attn_b=3,
    tail_blocks=(4, 2, 1, 1),
)


def _forward(A_x, A_c_kv, A_w_q, A_w_uk, A_w_uv, A_w_o, B_k_cache, B_v_cache, B_wq, B_wo,
             gate_w, cfg, params):
    B, Sq, M = A_x.shape
    assert Sq == 1
    _, Sk, Dc = A_c_kv.shape
    _, H, D = A_w_q.shape
    _, Hkv, SkB, _ = B_k_cache.shape
    W = min(4096, max(256, SkB // 4))
    HD = H * D

    kernel, n_sems = _make_kernel(B, M, H, D, Dc, Sk, Hkv, SkB, W, cfg)
    any_spec = pl.BlockSpec(memory_space=pl.ANY)
    out = pl.pallas_call(
        kernel,
        out_shape=jax.ShapeDtypeStruct((B, M), A_x.dtype),
        in_specs=[any_spec] * 11,
        out_specs=pl.BlockSpec(memory_space=pltpu.VMEM),
        scratch_shapes=[
            pltpu.VMEM((B, M), BF16),
            pltpu.VMEM((M // 128, 128), BF16),
            pltpu.VMEM((B * 4, Sk // 4, Dc), BF16),
            pltpu.VMEM((NSTR, M * H // NSTR // 2, D), U32),
            pltpu.VMEM((NSTR, Dc * H // NSTR // 2, D), U32),
            pltpu.VMEM((NSTR, Dc * H // NSTR // 2, D), U32),
            pltpu.VMEM((NSTR, HD // NSTR, M), BF16),
            pltpu.VMEM((B, Hkv, W, D), BF16),
            pltpu.VMEM((B, Hkv, W, D), BF16),
            pltpu.VMEM((NSTR, M // NSTR, HD), BF16),
            pltpu.VMEM((NSTR, HD // NSTR, M), BF16),
            pltpu.VMEM((Dc // 128, H * B, 128), F32),
            pltpu.VMEM((Dc // 128, B * H, 128), F32),
            pltpu.VMEM((H, B, D), F32),
            pltpu.VMEM((H * B, D), F32),
            pltpu.VMEM((B * H, D), F32),
            pltpu.SemaphoreType.DMA((n_sems,)),
        ],
        compiler_params=pltpu.CompilerParams(vmem_limit_bytes=112 * 1024 * 1024, **params),
        name="gated_mix_decode",
    )(
        A_x.reshape(B, M),
        gate_w.reshape(M // 128, 128),
        A_c_kv.reshape(B * 4, Sk // 4, Dc),
        A_w_q.reshape(NSTR, M * H // NSTR, D),
        A_w_uk.reshape(NSTR, Dc * H // NSTR, D),
        A_w_uv.reshape(NSTR, Dc * H // NSTR, D),
        A_w_o.reshape(NSTR, HD // NSTR, M),
        B_k_cache,
        B_v_cache,
        B_wq.reshape(NSTR, M // NSTR, HD),
        B_wo.reshape(NSTR, HD // NSTR, M),
    )
    return out.reshape(B, 1, M)


@jax.jit
def pallas_gated_mix__compressed_kv_cla__sliding_block_cached__decode_kernel(
    A_x: jax.Array,
    A_c_kv: jax.Array,
    A_w_q: jax.Array,
    A_w_uk: jax.Array,
    A_w_uv: jax.Array,
    A_w_o: jax.Array,
    B_x: jax.Array,
    B_k_cache: jax.Array,
    B_v_cache: jax.Array,
    B_wq: jax.Array,
    B_wo: jax.Array,
    gate_w: jax.Array,
):
    return _forward(A_x, A_c_kv, A_w_q, A_w_uk, A_w_uv, A_w_o, B_k_cache, B_v_cache,
                    B_wq, B_wo, gate_w, DEFAULT_CFG,
                    dict(disable_bounds_checks=True, disable_semaphore_checks=True))
```

```python
import jax
import jax.numpy as jnp
import jax.experimental.pallas as pl
import jax.experimental.pallas.tpu as pltpu

F32 = jnp.float32
BF16 = jnp.bfloat16
U32 = jnp.uint32

_NT = (((1,), (1,)), ((), ()))

NSTR = 8
BURST = 8


def _head_pair(w_u32, j, heads):
    ns, rr, d = w_u32.shape
    n = rr // heads
    ev = w_u32[:, pl.ds(j, n, stride=heads), :].reshape(ns * n, d)
    od = w_u32[:, pl.ds(j + heads // 2, n, stride=heads), :].reshape(ns * n, d)
    lo = (ev & jnp.uint32(0xFFFF)) | (od << 16)
    hi = (ev >> 16) | (od & jnp.uint32(0xFFFF0000))
    return pltpu.bitcast(lo, BF16), pltpu.bitcast(hi, BF16)


def _divmod_pow2(u, n):
    assert n & (n - 1) == 0
    return u >> (n.bit_length() - 1), u & (n - 1)


def _mult(v, n):
    return v if isinstance(v, int) else pl.multiple_of(v, n)


def _make_kernel(B, M, H, D, Dc, Sk, Hkv, SkB, W, cfg):
    rep = H // Hkv
    scale = float(D) ** -0.5
    HD = H * D
    CS = 4
    CR = Sk // CS
    OR = HD // NSTR
    NBAND = OR // D
    tail_blocks = cfg["tail_blocks"]

    S_X, S_GW, S_WQ, S_WUK, S_BWQ, S_WUV, S_CKV = 0, 1, 2, 3, 4, 5, 6
    S_KV = S_CKV + 2
    S_W3 = S_KV + 2 * B
    S_TAIL = S_W3 + 2 * NBAND - 1
    n_sems = S_TAIL + len(tail_blocks)

    def kernel(x_h, gw_h, ckv_h, wq_h, wuk_h, wuv_h, wo_h, kc_h, vc_h, bwq_h, bwo_h,
               o_ref,
               x_v, gw_v, ckv_v, wq_v, wuk_v, wuv_v, wo_v, kc_v, vc_v, bwq_v, bwo_v,
               qabs_s, lat_s, ctx_s, qb_s, ob_s, acc_s, sems):
        def start(src, dst, sem, prio):
            pltpu.make_async_copy(src, dst, sems.at[sem]).start(priority=prio)

        def wait(buf, sem):
            pltpu.make_async_copy(buf, buf, sems.at[sem]).wait()

        wq_b, wuk_b, wuv_b = wq_v.bitcast(BF16), wuk_v.bitcast(BF16), wuv_v.bitcast(BF16)
        every = slice(None)

        def rows16(src, dst, r, sem, prio):
            sl = (every, pl.ds(_mult(r, 16), 16), every)
            start(src.at[sl], dst.at[sl], sem, prio)

        def tiles2(src, dst, lead, r, c, sem, prio):
            sl = (lead, pl.ds(_mult(r, 8), 8), pl.ds(_mult(c, 256), 256))
            start(src.at[sl], dst.at[sl], sem, prio)

        def burst_w1(u):
            for i in range(BURST):
                r = u * (16 * BURST) + 16 * i
                rows16(wq_h, wq_b, r, S_WQ, 0)
                rows16(wuk_h, wuk_b, r, S_WUK, 1)

        def burst_w2(u):
            rb, ch = _divmod_pow2(u, HD // 256 // BURST)
            for i in range(BURST):
                tiles2(bwq_h, bwq_v, every, rb * 8, ch * (256 * BURST) + 256 * i, S_BWQ, 0)
                rows16(wuv_h, wuv_b, u * (16 * BURST) + 16 * i, S_WUV, 1)

        ncc = Dc // 256
        ckv_bursts = (CR // 8) * ncc // BURST

        def burst_ckv(u):
            half, uu = _divmod_pow2(u, ckv_bursts)
            for i in range(BURST):
                r = uu * (8 * BURST // ncc) + 8 * (i // ncc)
                for t in range(2):
                    lead = pl.ds(half * (2 * NSTR) + t * NSTR, NSTR)
                    tiles2(ckv_h, ckv_v, lead, r, 256 * (i % ncc), S_CKV + half, t)

        kv_bursts = W // 16 // BURST

        def burst_kv(u):
            b, uu = _divmod_pow2(u, kv_bursts)
            for i in range(BURST):
                r = uu * (16 * BURST) + 16 * i
                for t, (src, dst) in enumerate(((kc_h, kc_v), (vc_h, vc_v))):
                    start(src.at[b, :, pl.ds(_mult(SkB - W + r, 16), 16)],
                          dst.at[b, :, pl.ds(_mult(r, 16), 16)], S_KV + 2 * b + t, t)

        nmc = M // 256
        band_bursts = (D // 8) * nmc // BURST

        def burst_w3(u):
            band, _ = _divmod_pow2(u, band_bursts)
            for i in range(BURST):
                r = u * (8 * BURST // nmc) + 8 * (i // nmc)
                c = 256 * (i % nmc)
                tiles2(wo_h, wo_v, every, r, c, S_W3 + 2 * band, 0)
                tiles2(bwo_h, bwo_v, every, r, c, S_W3 + 2 * band + 1, 1)

        plan = []
        u0 = 0
        for fn, n in ((burst_w1, wq_b.shape[1] // 16 // BURST),
                      (burst_w2, wuv_b.shape[1] // 16 // BURST),
                      (burst_ckv, 2 * ckv_bursts),
                      (burst_kv, B * kv_bursts),
                      (burst_w3, (NBAND - 1) * band_bursts)):
            plan.append((u0, n, fn))
            u0 += n
        n_bursts = u0

        def issue(first, count, lo, hi):
            hits = [(u0, n, fn) for u0, n, fn in plan if u0 < hi and lo < u0 + n]

            def one(u):
                for u0, n, fn in hits:
                    if len(hits) == 1:
                        fn(u - u0)
                    else:
                        pl.when(jnp.logical_and(u >= u0, u < u0 + n))(lambda: fn(u - u0))

            if count == 1:
                one(first)
            else:
                def body(i, c):
                    one(first + i)
                    return c
                jax.lax.fori_loop(0, count, body, 0)

        class Cursor:
            pos = 0

            def to(self, hi):
                assert self.pos <= hi <= n_bursts, (self.pos, hi)
                for u0, n, _ in plan:
                    a, b = max(self.pos, u0), min(hi, u0 + n)
                    if a < b:
                        issue(a, b - a, a, b)
                self.pos = hi

            def loop(self, iters, counts):
                per = sum(counts)
                lo, hi = self.pos, self.pos + iters * per
                assert hi <= n_bursts
                self.pos = hi

                def f(i, k):
                    if counts[k]:
                        issue(lo + i * per + sum(counts[:k]), counts[k], lo, hi)
                return f

        cur = Cursor()

        start(x_h, x_v, S_X, 0)
        start(gw_h, gw_v, S_GW, 1)
        cur.to(cfg["u_qabs"])

        wait(x_v, S_X)
        wait(gw_v, S_GW)
        wait(wq_b, S_WQ)
        wait(wuk_b, S_WUK)
        iss_q = cur.loop(H // 2, cfg["n_qabs"])

        def qabs_body(j, carry):
            x = x_v[...]
            wq0, wq1 = _head_pair(wq_v, j, H)
            wk0, wk1 = _head_pair(wuk_v, j, H)
            for p, (wq_, wk_) in enumerate(((wq0, wk0), (wq1, wk1))):
                q = jnp.dot(x, wq_, preferred_element_type=F32).astype(BF16)
                qa = jax.lax.dot_general(q, wk_, _NT, preferred_element_type=F32)
                row = pl.multiple_of((2 * j + p) * B, B)
                qa = qa * scale
                for t in range(Dc // 128):
                    qabs_s[t, pl.ds(row, B), :] = qa[:, t * 128:(t + 1) * 128]
            iss_q(j, 0)
            return carry

        jax.lax.fori_loop(0, H // 2, qabs_body, 0)

        wait(bwq_v, S_BWQ)
        wait(wuv_b, S_WUV)
        qb = jnp.dot(x_v[...], bwq_v[...].reshape(M, HD), preferred_element_type=F32)
        qb = qb.astype(BF16).astype(F32)
        for h in range(H):
            qb_s[h * B:(h + 1) * B, :] = qb[:, h * D:(h + 1) * D]

        cur.to(cfg["u_attn_a"])
        iss_a = cur.loop(B, cfg["n_attn_a"])

        def attn_a(b, carry):
            for half in range(2):
                pl.when(b == half * (B // 2))(
                    lambda: wait(ckv_v.at[pl.ds(half * 2 * NSTR, 2 * NSTR)], S_CKV + half))

            qa = jnp.concatenate(
                [qabs_s[t, pl.ds(b, H, stride=B), :] for t in range(Dc // 128)],
                axis=1).astype(BF16)
            c = ckv_v[pl.ds(b * CS, CS)].reshape(Sk, Dc)
            s = jax.lax.dot_general(qa, c, _NT, preferred_element_type=F32)
            iss_a(b, 0)
            m = jnp.max(s, axis=-1, keepdims=True)
            p = jnp.exp(s - m)
            l = jnp.sum(p, axis=-1, keepdims=True)
            c = ckv_v[pl.ds(b * CS, CS)].reshape(Sk, Dc)
            lat = jnp.dot(p.astype(BF16), c, preferred_element_type=F32)
            lat = lat / l
            row = pl.multiple_of(b * H, H)
            for t in range(Dc // 128):
                lat_s[t, pl.ds(row, H), :] = lat[:, t * 128:(t + 1) * 128]
            iss_a(b, 1)
            return carry

        jax.lax.fori_loop(0, B, attn_a, 0)

        iss_c = cur.loop(H // 2, cfg["n_ctx"])

        def ctx_body(j, carry):
            wv = _head_pair(wuv_v, j, H)
            for p in range(2):
                lat = jnp.concatenate(
                    [lat_s[t, pl.ds(2 * j + p, B, stride=H), :] for t in range(Dc // 128)],
                    axis=1).astype(BF16)
                ctx_s[2 * j + p] = jnp.dot(lat, wv[p], preferred_element_type=F32)
            iss_c(j, 0)
            return carry

        jax.lax.fori_loop(0, H // 2, ctx_body, 0)

        cur.to(cfg["u_attn_b"])
        iss_b = cur.loop(B, cfg["n_attn_b"])
        first = jax.lax.broadcasted_iota(jnp.int32, (2 * rep, 1), 0) < rep

        def attn_b(b, carry):
            iss_b(b, 0)
            wait(kc_v.at[b], S_KV + 2 * b)
            wait(vc_v.at[b], S_KV + 2 * b + 1)
            for g in range(0, Hkv, 2):
                if g == Hkv // 2:
                    iss_b(b, 1)
                q = qb_s[pl.ds(g * rep * B + b, 2 * rep, stride=B), :].astype(BF16)
                s0 = jax.lax.dot_general(q, kc_v[b, g], _NT, preferred_element_type=F32)
                s1 = jax.lax.dot_general(q, kc_v[b, g + 1], _NT, preferred_element_type=F32)
                s = jnp.where(first, s0, s1) * scale
                m = jnp.max(s, axis=-1, keepdims=True)
                p = jnp.exp(s - m)
                l = jnp.sum(p, axis=-1, keepdims=True)
                p = p.astype(BF16)
                o0 = jnp.dot(p, vc_v[b, g], preferred_element_type=F32)
                o1 = jnp.dot(p, vc_v[b, g + 1], preferred_element_type=F32)
                row = pl.multiple_of(b * H + g * rep, 2 * rep)
                ob_s[pl.ds(row, 2 * rep), :] = jnp.where(first, o0, o1) / l
            return carry

        jax.lax.fori_loop(0, B, attn_b, 0)

        def lhs(which, s0, ns, band):
            hs = [s * NBAND + band for s in range(s0, s0 + ns)]
            if which == 0:
                parts = [ctx_s[h] for h in hs]
            else:
                parts = [ob_s[pl.ds(h, B, stride=H), :] for h in hs]
            return jnp.concatenate(parts, axis=1).astype(BF16)

        def proj(l, which, s0, ns, band):
            w = (wo_v, bwo_v)[which][pl.ds(s0, ns), pl.ds(band * D, D), :].reshape(ns * D, M)
            return jnp.dot(l, w, preferred_element_type=F32)

        def do_band(which, band):
            wait((wo_v, bwo_v)[which].at[:, pl.ds(band * D, D)], S_W3 + 2 * band + which)
            r = proj(lhs(which, 0, NSTR, band), which, 0, NSTR, band)
            acc_s[which] = r if band == 0 else acc_s[which] + r

        last = NBAND - 1
        todo = [(which, band) for band in range(NBAND) for which in range(2)][:-1]
        for u, n in cfg["u_band"]:
            cur.to(u)
            for _ in range(n):
                do_band(*todo.pop(0))
        cur.to(n_bursts)

        narrow = []
        s0 = 0
        for k, ns in enumerate(tail_blocks):
            rows = 32 // ns
            narrow += [((pl.ds(s0, ns), pl.ds(r, rows), every), S_TAIL + k)
                       for r in range(last * D, (last + 1) * D, rows)]
            s0 += ns
        for i, (sl, sem) in enumerate(narrow):
            tiles2(wo_h, wo_v, every, last * D + 8 * (i // nmc), 256 * (i % nmc), S_W3 + 2 * last, 0)
            start(bwo_h.at[sl], bwo_v.at[sl], sem, 1)

        xf = x_v[...].astype(F32)
        gw = gw_v[...].astype(F32)
        t = xf[:, 0:128] * gw[0:1, :]
        for i in range(1, M // 128):
            t = t + xf[:, i * 128:(i + 1) * 128] * gw[i:i + 1, :]
        gate = jax.nn.sigmoid(jnp.sum(t, axis=-1, keepdims=True))

        for which, band in todo:
            do_band(which, band)
        starts = [sum(tail_blocks[:k]) for k in range(len(tail_blocks))]
        tail_lhs = [lhs(1, s0, ns, last) for s0, ns in zip(starts, tail_blocks)]
        out = gate * acc_s[0]
        acc = acc_s[1]
        for k, (s0, ns) in enumerate(zip(starts, tail_blocks)):
            wait(bwo_v.at[pl.ds(s0, ns), pl.ds(last * D, D)], S_TAIL + k)
            acc = acc + proj(tail_lhs[k], 1, s0, ns, last)
        o_ref[...] = (out + (1.0 - gate) * acc).astype(o_ref.dtype)

    return kernel, n_sems


DEFAULT_CFG = dict(
    u_qabs=22, n_qabs=(2,),
    u_attn_a=78, n_attn_a=(3, 3),
    n_ctx=(1,),
    u_attn_b=144, n_attn_b=(2, 1),
    u_band=((169, 2), (172, 1)),
    tail_blocks=(4, 2, 1, 1),
)
DEFAULT_PARAMS = dict(disable_bounds_checks=True, disable_semaphore_checks=True)


def _forward(A_x, A_c_kv, A_w_q, A_w_uk, A_w_uv, A_w_o, B_k_cache, B_v_cache, B_wq, B_wo,
             gate_w, cfg, params):
    B, Sq, M = A_x.shape
    assert Sq == 1
    _, Sk, Dc = A_c_kv.shape
    _, H, D = A_w_q.shape
    _, Hkv, SkB, _ = B_k_cache.shape
    W = min(4096, max(256, SkB // 4))
    HD = H * D

    kernel, n_sems = _make_kernel(B, M, H, D, Dc, Sk, Hkv, SkB, W, cfg)
    any_spec = pl.BlockSpec(memory_space=pl.ANY)
    out = pl.pallas_call(
        kernel,
        out_shape=jax.ShapeDtypeStruct((B, M), A_x.dtype),
        in_specs=[any_spec] * 11,
        out_specs=pl.BlockSpec(memory_space=pltpu.VMEM),
        scratch_shapes=[
            pltpu.VMEM((B, M), BF16),
            pltpu.VMEM((M // 128, 128), BF16),
            pltpu.VMEM((B * 4, Sk // 4, Dc), BF16),
            pltpu.VMEM((NSTR, M * H // NSTR // 2, D), U32),
            pltpu.VMEM((NSTR, Dc * H // NSTR // 2, D), U32),
            pltpu.VMEM((NSTR, Dc * H // NSTR // 2, D), U32),
            pltpu.VMEM((NSTR, HD // NSTR, M), BF16),
            pltpu.VMEM((B, Hkv, W, D), BF16),
            pltpu.VMEM((B, Hkv, W, D), BF16),
            pltpu.VMEM((NSTR, M // NSTR, HD), BF16),
            pltpu.VMEM((NSTR, HD // NSTR, M), BF16),
            pltpu.VMEM((Dc // 128, H * B, 128), F32),
            pltpu.VMEM((Dc // 128, B * H, 128), F32),
            pltpu.VMEM((H, B, D), F32),
            pltpu.VMEM((H * B, D), F32),
            pltpu.VMEM((B * H, D), F32),
            pltpu.VMEM((2, B, M), F32),
            pltpu.SemaphoreType.DMA((n_sems,)),
        ],
        compiler_params=pltpu.CompilerParams(vmem_limit_bytes=112 * 1024 * 1024, **params),
        name="gated_mix_decode",
    )(
        A_x.reshape(B, M),
        gate_w.reshape(M // 128, 128),
        A_c_kv.reshape(B * 4, Sk // 4, Dc),
        A_w_q.reshape(NSTR, M * H // NSTR, D),
        A_w_uk.reshape(NSTR, Dc * H // NSTR, D),
        A_w_uv.reshape(NSTR, Dc * H // NSTR, D),
        A_w_o.reshape(NSTR, HD // NSTR, M),
        B_k_cache,
        B_v_cache,
        B_wq.reshape(NSTR, M // NSTR, HD),
        B_wo.reshape(NSTR, HD // NSTR, M),
    )
    return out.reshape(B, 1, M)


@jax.jit
def pallas_gated_mix__compressed_kv_cla__sliding_block_cached__decode_kernel(
    A_x: jax.Array,
    A_c_kv: jax.Array,
    A_w_q: jax.Array,
    A_w_uk: jax.Array,
    A_w_uv: jax.Array,
    A_w_o: jax.Array,
    B_x: jax.Array,
    B_k_cache: jax.Array,
    B_v_cache: jax.Array,
    B_wq: jax.Array,
    B_wo: jax.Array,
    gate_w: jax.Array,
):
    return _forward(A_x, A_c_kv, A_w_q, A_w_uk, A_w_uv, A_w_o, B_k_cache, B_v_cache,
                    B_wq, B_wo, gate_w, DEFAULT_CFG, DEFAULT_PARAMS)
```

```python
import jax
import jax.numpy as jnp
import jax.experimental.pallas as pl
import jax.experimental.pallas.tpu as pltpu

F32 = jnp.float32
BF16 = jnp.bfloat16
U32 = jnp.uint32

_NT = (((1,), (1,)), ((), ()))

NSTR = 8
BURST = 8


def _head_pair(w_u32, j, heads):
    ns, rr, d = w_u32.shape
    n = rr // heads
    ev = w_u32[:, pl.ds(j, n, stride=heads), :].reshape(ns * n, d)
    od = w_u32[:, pl.ds(j + heads // 2, n, stride=heads), :].reshape(ns * n, d)
    lo = (ev & jnp.uint32(0xFFFF)) | (od << 16)
    hi = (ev >> 16) | (od & jnp.uint32(0xFFFF0000))
    return pltpu.bitcast(lo, BF16), pltpu.bitcast(hi, BF16)


def _divmod_pow2(u, n):
    assert n & (n - 1) == 0
    return u >> (n.bit_length() - 1), u & (n - 1)


def _mult(v, n):
    return v if isinstance(v, int) else pl.multiple_of(v, n)


def _make_kernel(B, M, H, D, Dc, Sk, Hkv, SkB, W, cfg):
    rep = H // Hkv
    scale = float(D) ** -0.5
    HD = H * D
    CS = 4
    CR = Sk // CS
    OR = HD // NSTR
    NBAND = OR // D
    tail_blocks = cfg["tail_blocks"]

    S_X, S_GW, S_WQ, S_WUK, S_BWQ, S_WUV, S_CKV = 0, 1, 2, 3, 4, 5, 6
    S_KV = S_CKV + 2
    HP = Hkv // 2
    UB = NSTR // HP
    S_W3 = S_KV + 2 * (B // UB)
    S_TAIL = S_W3 + 2 * NBAND - 1
    n_sems = S_TAIL + len(tail_blocks)

    def kernel(x_h, gw_h, ckv_h, wq_h, wuk_h, wuv_h, wo_h, kc_h, vc_h, bwq_h, bwo_h,
               o_ref,
               x_v, gw_v, ckv_v, wq_v, wuk_v, wuv_v, wo_v, kc_v, vc_v, bwq_v, bwo_v,
               qabs_s, lat_s, ctx_s, qb_s, ob_s, acc_s, sems):
        def start(src, dst, sem, prio):
            pltpu.make_async_copy(src, dst, sems.at[sem]).start(priority=prio)

        def wait(buf, sem):
            pltpu.make_async_copy(buf, buf, sems.at[sem]).wait()

        wq_b, wuk_b, wuv_b = wq_v.bitcast(BF16), wuk_v.bitcast(BF16), wuv_v.bitcast(BF16)
        every = slice(None)

        def rows16(src, dst, r, sem, prio):
            sl = (every, pl.ds(_mult(r, 16), 16), every)
            start(src.at[sl], dst.at[sl], sem, prio)

        def tiles2(src, dst, lead, r, c, sem, prio):
            sl = (lead, pl.ds(_mult(r, 8), 8), pl.ds(_mult(c, 256), 256))
            start(src.at[sl], dst.at[sl], sem, prio)

        def burst_w1(u):
            for i in range(BURST):
                r = u * (16 * BURST) + 16 * i
                rows16(wq_h, wq_b, r, S_WQ, 0)
                rows16(wuk_h, wuk_b, r, S_WUK, 1)

        def burst_w2(u):
            rb, ch = _divmod_pow2(u, HD // 256 // BURST)
            for i in range(BURST):
                tiles2(bwq_h, bwq_v, every, rb * 8, ch * (256 * BURST) + 256 * i, S_BWQ, 0)
                rows16(wuv_h, wuv_b, u * (16 * BURST) + 16 * i, S_WUV, 1)

        ncc = Dc // 256
        ckv_bursts = (CR // 8) * ncc // BURST

        def burst_ckv(u):
            half, uu = _divmod_pow2(u, ckv_bursts)
            for i in range(BURST):
                r = uu * (8 * BURST // ncc) + 8 * (i // ncc)
                for t in range(2):
                    lead = pl.ds(half * (2 * NSTR) + t * NSTR, NSTR)
                    tiles2(ckv_h, ckv_v, lead, r, 256 * (i % ncc), S_CKV + half, t)

        kv_bursts = W // 16 // BURST

        def burst_kv(u):
            q, uu = _divmod_pow2(u, kv_bursts)
            unit, par = _divmod_pow2(q, 2)
            lead = pl.ds(unit * NSTR, NSTR)
            for i in range(BURST):
                r = uu * (16 * BURST) + 16 * i
                for t, (src, dst) in enumerate(((kc_h, kc_v), (vc_h, vc_v))):
                    start(src.at[lead, par, pl.ds(_mult(SkB - W + r, 16), 16)],
                          dst.at[lead, par, pl.ds(_mult(r, 16), 16)], S_KV + 2 * unit + t, t)

        nmc = M // 256
        band_bursts = (D // 8) * nmc // BURST

        def burst_w3(u):
            band, _ = _divmod_pow2(u, band_bursts)
            for i in range(BURST):
                r = u * (8 * BURST // nmc) + 8 * (i // nmc)
                c = 256 * (i % nmc)
                tiles2(wo_h, wo_v, every, r, c, S_W3 + 2 * band, 0)
                tiles2(bwo_h, bwo_v, every, r, c, S_W3 + 2 * band + 1, 1)

        plan = []
        u0 = 0
        for fn, n in ((burst_w1, wq_b.shape[1] // 16 // BURST),
                      (burst_w2, wuv_b.shape[1] // 16 // BURST),
                      (burst_ckv, 2 * ckv_bursts),
                      (burst_kv, B * kv_bursts),
                      (burst_w3, (NBAND - 1) * band_bursts)):
            plan.append((u0, n, fn))
            u0 += n
        n_bursts = u0

        def issue(first, count, lo, hi):
            hits = [(u0, n, fn) for u0, n, fn in plan if u0 < hi and lo < u0 + n]

            def one(u):
                for u0, n, fn in hits:
                    if len(hits) == 1:
                        fn(u - u0)
                    else:
                        pl.when(jnp.logical_and(u >= u0, u < u0 + n))(lambda: fn(u - u0))

            if count == 1:
                one(first)
            else:
                def body(i, c):
                    one(first + i)
                    return c
                jax.lax.fori_loop(0, count, body, 0)

        class Cursor:
            pos = 0

            def to(self, hi):
                assert self.pos <= hi <= n_bursts, (self.pos, hi)
                for u0, n, _ in plan:
                    a, b = max(self.pos, u0), min(hi, u0 + n)
                    if a < b:
                        issue(a, b - a, a, b)
                self.pos = hi

            def loop(self, iters, counts):
                per = sum(counts)
                lo, hi = self.pos, self.pos + iters * per
                assert hi <= n_bursts
                self.pos = hi

                def f(i, k):
                    if counts[k]:
                        issue(lo + i * per + sum(counts[:k]), counts[k], lo, hi)
                return f

        cur = Cursor()

        start(x_h, x_v, S_X, 0)
        start(gw_h, gw_v, S_GW, 1)
        cur.to(cfg["u_qabs"])

        wait(x_v, S_X)
        wait(gw_v, S_GW)
        wait(wq_b, S_WQ)
        wait(wuk_b, S_WUK)
        iss_q = cur.loop(H // 2, cfg["n_qabs"])

        def qabs_body(j, carry):
            x = x_v[...]
            wq0, wq1 = _head_pair(wq_v, j, H)
            wk0, wk1 = _head_pair(wuk_v, j, H)
            for p, (wq_, wk_) in enumerate(((wq0, wk0), (wq1, wk1))):
                q = jnp.dot(x, wq_, preferred_element_type=F32).astype(BF16)
                qa = jax.lax.dot_general(q, wk_, _NT, preferred_element_type=F32)
                row = pl.multiple_of((2 * j + p) * B, B)
                qa = qa * scale
                for t in range(Dc // 128):
                    qabs_s[t, pl.ds(row, B), :] = qa[:, t * 128:(t + 1) * 128]
            iss_q(j, 0)
            return carry

        jax.lax.fori_loop(0, H // 2, qabs_body, 0)

        wait(bwq_v, S_BWQ)
        wait(wuv_b, S_WUV)
        qb = jnp.dot(x_v[...], bwq_v[...].reshape(M, HD), preferred_element_type=F32)
        qb = qb.astype(BF16).astype(F32)
        for h in range(H):
            qb_s[h * B:(h + 1) * B, :] = qb[:, h * D:(h + 1) * D]

        cur.to(cfg["u_attn_a"])
        iss_a = cur.loop(B, cfg["n_attn_a"])

        def attn_a(b, carry):
            for half in range(2):
                pl.when(b == half * (B // 2))(
                    lambda: wait(ckv_v.at[pl.ds(half * 2 * NSTR, 2 * NSTR)], S_CKV + half))

            qa = jnp.concatenate(
                [qabs_s[t, pl.ds(b, H, stride=B), :] for t in range(Dc // 128)],
                axis=1).astype(BF16)
            c = ckv_v[pl.ds(b * CS, CS)].reshape(Sk, Dc)
            s = jax.lax.dot_general(qa, c, _NT, preferred_element_type=F32)
            iss_a(b, 0)
            m = jnp.max(s, axis=-1, keepdims=True)
            p = jnp.exp(s - m)
            l = jnp.sum(p, axis=-1, keepdims=True)
            c = ckv_v[pl.ds(b * CS, CS)].reshape(Sk, Dc)
            lat = jnp.dot(p.astype(BF16), c, preferred_element_type=F32)
            lat = lat / l
            row = pl.multiple_of(b * H, H)
            for t in range(Dc // 128):
                lat_s[t, pl.ds(row, H), :] = lat[:, t * 128:(t + 1) * 128]
            iss_a(b, 1)
            return carry

        jax.lax.fori_loop(0, B, attn_a, 0)

        iss_c = cur.loop(H // 2, cfg["n_ctx"])

        def ctx_body(j, carry):
            wv = _head_pair(wuv_v, j, H)
            for p in range(2):
                lat = jnp.concatenate(
                    [lat_s[t, pl.ds(2 * j + p, B, stride=H), :] for t in range(Dc // 128)],
                    axis=1).astype(BF16)
                ctx_s[2 * j + p] = jnp.dot(lat, wv[p], preferred_element_type=F32)
            iss_c(j, 0)
            return carry

        jax.lax.fori_loop(0, H // 2, ctx_body, 0)

        cur.to(cfg["u_attn_b"])
        iss_b = cur.loop(B, cfg["n_attn_b"])
        first = jax.lax.broadcasted_iota(jnp.int32, (2 * rep, 1), 0) < rep

        def attn_b(b, carry):
            iss_b(b, 0)
            unit, sub = _divmod_pow2(b, UB)

            @pl.when(sub == 0)
            def _():
                wait(kc_v.at[pl.ds(unit * NSTR, NSTR)], S_KV + 2 * unit)
                wait(vc_v.at[pl.ds(unit * NSTR, NSTR)], S_KV + 2 * unit + 1)

            for gp in range(HP):
                if gp == HP // 2:
                    iss_b(b, 1)
                a = b * HP + gp
                q = qb_s[pl.ds(gp * 2 * rep * B + b, 2 * rep, stride=B), :].astype(BF16)
                s0 = jax.lax.dot_general(q, kc_v[a, 0], _NT, preferred_element_type=F32)
                s1 = jax.lax.dot_general(q, kc_v[a, 1], _NT, preferred_element_type=F32)
                s = jnp.where(first, s0, s1) * scale
                m = jnp.max(s, axis=-1, keepdims=True)
                p = jnp.exp(s - m)
                l = jnp.sum(p, axis=-1, keepdims=True)
                p = p.astype(BF16)
                o0 = jnp.dot(p, vc_v[a, 0], preferred_element_type=F32)
                o1 = jnp.dot(p, vc_v[a, 1], preferred_element_type=F32)
                row = pl.multiple_of(a * 2 * rep, 2 * rep)
                ob_s[pl.ds(row, 2 * rep), :] = jnp.where(first, o0, o1) / l
            return carry

        jax.lax.fori_loop(0, B, attn_b, 0)

        def lhs(which, s0, ns, band):
            hs = [s * NBAND + band for s in range(s0, s0 + ns)]
            if which == 0:
                parts = [ctx_s[h] for h in hs]
            else:
                parts = [ob_s[pl.ds(h, B, stride=H), :] for h in hs]
            return jnp.concatenate(parts, axis=1).astype(BF16)

        def proj(l, which, s0, ns, band):
            w = (wo_v, bwo_v)[which][pl.ds(s0, ns), pl.ds(band * D, D), :].reshape(ns * D, M)
            return jnp.dot(l, w, preferred_element_type=F32)

        def do_band(which, band):
            wait((wo_v, bwo_v)[which].at[:, pl.ds(band * D, D)], S_W3 + 2 * band + which)
            r = proj(lhs(which, 0, NSTR, band), which, 0, NSTR, band)
            acc_s[which] = r if band == 0 else acc_s[which] + r

        last = NBAND - 1
        todo = [(which, band) for band in range(NBAND) for which in range(2)][:-1]
        for u, n in cfg["u_band"]:
            cur.to(u)
            for _ in range(n):
                do_band(*todo.pop(0))
        cur.to(n_bursts)

        narrow = []
        s0 = 0
        for k, ns in enumerate(tail_blocks):
            rows = 32 // ns
            narrow += [((pl.ds(s0, ns), pl.ds(r, rows), every), S_TAIL + k)
                       for r in range(last * D, (last + 1) * D, rows)]
            s0 += ns
        for i, (sl, sem) in enumerate(narrow):
            tiles2(wo_h, wo_v, every, last * D + 8 * (i // nmc), 256 * (i % nmc), S_W3 + 2 * last, 0)
            start(bwo_h.at[sl], bwo_v.at[sl], sem, 1)

        xf = x_v[...].astype(F32)
        gw = gw_v[...].astype(F32)
        t = xf[:, 0:128] * gw[0:1, :]
        for i in range(1, M // 128):
            t = t + xf[:, i * 128:(i + 1) * 128] * gw[i:i + 1, :]
        gate = jax.nn.sigmoid(jnp.sum(t, axis=-1, keepdims=True))

        for which, band in todo:
            do_band(which, band)
        starts = [sum(tail_blocks[:k]) for k in range(len(tail_blocks))]
        tail_lhs = [lhs(1, s0, ns, last) for s0, ns in zip(starts, tail_blocks)]
        out = gate * acc_s[0]
        acc = acc_s[1]
        for k, (s0, ns) in enumerate(zip(starts, tail_blocks)):
            wait(bwo_v.at[pl.ds(s0, ns), pl.ds(last * D, D)], S_TAIL + k)
            acc = acc + proj(tail_lhs[k], 1, s0, ns, last)
        o_ref[...] = (out + (1.0 - gate) * acc).astype(o_ref.dtype)

    return kernel, n_sems


DEFAULT_CFG = dict(
    u_qabs=22, n_qabs=(2,),
    u_attn_a=78, n_attn_a=(3, 3),
    n_ctx=(1,),
    u_attn_b=148, n_attn_b=(2, 1),
    u_band=((172, 3),),
    tail_blocks=(4, 2, 1, 1),
)
DEFAULT_PARAMS = dict(disable_bounds_checks=True, disable_semaphore_checks=True)


def _forward(A_x, A_c_kv, A_w_q, A_w_uk, A_w_uv, A_w_o, B_k_cache, B_v_cache, B_wq, B_wo,
             gate_w, cfg, params):
    B, Sq, M = A_x.shape
    assert Sq == 1
    _, Sk, Dc = A_c_kv.shape
    _, H, D = A_w_q.shape
    _, Hkv, SkB, _ = B_k_cache.shape
    W = min(4096, max(256, SkB // 4))
    HD = H * D

    kernel, n_sems = _make_kernel(B, M, H, D, Dc, Sk, Hkv, SkB, W, cfg)
    any_spec = pl.BlockSpec(memory_space=pl.ANY)
    out = pl.pallas_call(
        kernel,
        out_shape=jax.ShapeDtypeStruct((B, M), A_x.dtype),
        in_specs=[any_spec] * 11,
        out_specs=pl.BlockSpec(memory_space=pltpu.VMEM),
        scratch_shapes=[
            pltpu.VMEM((B, M), BF16),
            pltpu.VMEM((M // 128, 128), BF16),
            pltpu.VMEM((B * 4, Sk // 4, Dc), BF16),
            pltpu.VMEM((NSTR, M * H // NSTR // 2, D), U32),
            pltpu.VMEM((NSTR, Dc * H // NSTR // 2, D), U32),
            pltpu.VMEM((NSTR, Dc * H // NSTR // 2, D), U32),
            pltpu.VMEM((NSTR, HD // NSTR, M), BF16),
            pltpu.VMEM((B * Hkv // 2, 2, W, D), BF16),
            pltpu.VMEM((B * Hkv // 2, 2, W, D), BF16),
            pltpu.VMEM((NSTR, M // NSTR, HD), BF16),
            pltpu.VMEM((NSTR, HD // NSTR, M), BF16),
            pltpu.VMEM((Dc // 128, H * B, 128), F32),
            pltpu.VMEM((Dc // 128, B * H, 128), F32),
            pltpu.VMEM((H, B, D), F32),
            pltpu.VMEM((H * B, D), F32),
            pltpu.VMEM((B * H, D), F32),
            pltpu.VMEM((2, B, M), F32),
            pltpu.SemaphoreType.DMA((n_sems,)),
        ],
        compiler_params=pltpu.CompilerParams(vmem_limit_bytes=112 * 1024 * 1024, **params),
        name="gated_mix_decode",
    )(
        A_x.reshape(B, M),
        gate_w.reshape(M // 128, 128),
        A_c_kv.reshape(B * 4, Sk // 4, Dc),
        A_w_q.reshape(NSTR, M * H // NSTR, D),
        A_w_uk.reshape(NSTR, Dc * H // NSTR, D),
        A_w_uv.reshape(NSTR, Dc * H // NSTR, D),
        A_w_o.reshape(NSTR, HD // NSTR, M),
        B_k_cache.reshape(B * Hkv // 2, 2, SkB, D),
        B_v_cache.reshape(B * Hkv // 2, 2, SkB, D),
        B_wq.reshape(NSTR, M // NSTR, HD),
        B_wo.reshape(NSTR, HD // NSTR, M),
    )
    return out.reshape(B, 1, M)


@jax.jit
def pallas_gated_mix__compressed_kv_cla__sliding_block_cached__decode_kernel(
    A_x: jax.Array,
    A_c_kv: jax.Array,
    A_w_q: jax.Array,
    A_w_uk: jax.Array,
    A_w_uv: jax.Array,
    A_w_o: jax.Array,
    B_x: jax.Array,
    B_k_cache: jax.Array,
    B_v_cache: jax.Array,
    B_wq: jax.Array,
    B_wo: jax.Array,
    gate_w: jax.Array,
):
    return _forward(A_x, A_c_kv, A_w_q, A_w_uk, A_w_uv, A_w_o, B_k_cache, B_v_cache,
                    B_wq, B_wo, gate_w, DEFAULT_CFG, DEFAULT_PARAMS)
```

```python
import jax
import jax.numpy as jnp
import jax.experimental.pallas as pl
import jax.experimental.pallas.tpu as pltpu

F32 = jnp.float32
BF16 = jnp.bfloat16
U32 = jnp.uint32

_NT = (((1,), (1,)), ((), ()))

NSTR = 8
BURST = 8
PLANE = 264


def _split_heads(w_v, t_s, step, nsteps, heads):
    ns, rr, _ = w_v.shape
    per_stream = nsteps // ns
    stream, part = _divmod_pow2(step, per_stream)
    rows = rr // per_stream
    half = heads // 2
    for k in range(rows // (2 * heads)):
        r0 = pl.multiple_of(part * rows + k * 2 * heads, 2 * heads)
        w = pltpu.bitcast(w_v[stream, pl.ds(r0, 2 * heads), :], U32)
        ev, od = w[:half], w[half:]
        lo = (ev & jnp.uint32(0xFFFF)) | (od << 16)
        hi = (ev >> 16) | (od & jnp.uint32(0xFFFF0000))
        i = step * (rows // (2 * heads)) + k
        t_s[pl.ds(i, half, stride=PLANE), :] = lo
        t_s[pl.ds(half * PLANE + i, half, stride=PLANE), :] = hi


def _head(t_s, j, p, heads, rows):
    r0 = pl.multiple_of((p * (heads // 2) + j) * PLANE, 8)
    return pltpu.bitcast(t_s[pl.ds(r0, rows // 2), :], BF16)


def _divmod_pow2(u, n):
    assert n & (n - 1) == 0
    return u >> (n.bit_length() - 1), u & (n - 1)


def _mult(v, n):
    return v if isinstance(v, int) else pl.multiple_of(v, n)


def _make_kernel(B, M, H, D, Dc, Sk, Hkv, SkB, W, cfg):
    rep = H // Hkv
    scale = float(D) ** -0.5
    HD = H * D
    CS = 4
    CR = Sk // CS
    OR = HD // NSTR
    NBAND = OR // D
    tail_blocks = cfg["tail_blocks"]

    S_X, S_GW, S_WQ, S_WUK, S_BWQ, S_WUV, S_CKV = 0, 1, 2, 3, 4, 5, 6
    S_KV = S_CKV + 2
    HP = Hkv // 2
    UB = NSTR // HP
    S_W3 = S_KV + 2 * (B // UB)
    S_TAIL = S_W3 + 2 * NBAND - 1
    n_sems = S_TAIL + len(tail_blocks)

    def kernel(x_h, gw_h, ckv_h, wq_h, wuk_h, wuv_h, wo_h, kc_h, vc_h, bwq_h, bwo_h,
               o_ref,
               x_v, gw_v, ckv_v, wq_v, wuk_v, wuv_v, wo_v, kc_v, vc_v, bwq_v, bwo_v,
               t0_s, t1_s, qabs_s, lat_s, ctx_s, qb_s, ob_s, acc_s, sems):
        def start(src, dst, sem, prio):
            pltpu.make_async_copy(src, dst, sems.at[sem]).start(priority=prio)

        def wait(buf, sem):
            pltpu.make_async_copy(buf, buf, sems.at[sem]).wait()

        every = slice(None)

        def rows16(src, dst, r, sem, prio):
            sl = (every, pl.ds(_mult(r, 16), 16), every)
            start(src.at[sl], dst.at[sl], sem, prio)

        def tiles2(src, dst, lead, r, c, sem, prio):
            sl = (lead, pl.ds(_mult(r, 8), 8), pl.ds(_mult(c, 256), 256))
            start(src.at[sl], dst.at[sl], sem, prio)

        def burst_w1(u):
            for i in range(BURST):
                r = u * (16 * BURST) + 16 * i
                rows16(wq_h, wq_v, r, S_WQ, 0)
                rows16(wuk_h, wuk_v, r, S_WUK, 1)

        def burst_w2(u):
            rb, ch = _divmod_pow2(u, HD // 256 // BURST)
            for i in range(BURST):
                tiles2(bwq_h, bwq_v, every, rb * 8, ch * (256 * BURST) + 256 * i, S_BWQ, 0)
                rows16(wuv_h, wuv_v, u * (16 * BURST) + 16 * i, S_WUV, 1)

        ncc = Dc // 256
        ckv_bursts = (CR // 8) * ncc // BURST

        def burst_ckv(u):
            half, uu = _divmod_pow2(u, ckv_bursts)
            for i in range(BURST):
                r = uu * (8 * BURST // ncc) + 8 * (i // ncc)
                for t in range(2):
                    lead = pl.ds(half * (2 * NSTR) + t * NSTR, NSTR)
                    tiles2(ckv_h, ckv_v, lead, r, 256 * (i % ncc), S_CKV + half, t)

        kv_bursts = W // 16 // BURST

        def burst_kv(u):
            q, uu = _divmod_pow2(u, kv_bursts)
            unit, par = _divmod_pow2(q, 2)
            lead = pl.ds(unit * NSTR, NSTR)
            for i in range(BURST):
                r = uu * (16 * BURST) + 16 * i
                for t, (src, dst) in enumerate(((kc_h, kc_v), (vc_h, vc_v))):
                    start(src.at[lead, par, pl.ds(_mult(SkB - W + r, 16), 16)],
                          dst.at[lead, par, pl.ds(_mult(r, 16), 16)], S_KV + 2 * unit + t, t)

        nmc = M // 256
        band_bursts = (D // 8) * nmc // BURST

        def burst_w3(u):
            band, _ = _divmod_pow2(u, band_bursts)
            for i in range(BURST):
                r = u * (8 * BURST // nmc) + 8 * (i // nmc)
                c = 256 * (i % nmc)
                tiles2(wo_h, wo_v, every, r, c, S_W3 + 2 * band, 0)
                tiles2(bwo_h, bwo_v, every, r, c, S_W3 + 2 * band + 1, 1)

        plan = []
        u0 = 0
        for fn, n in ((burst_w1, wq_v.shape[1] // 16 // BURST),
                      (burst_w2, wuv_v.shape[1] // 16 // BURST),
                      (burst_ckv, 2 * ckv_bursts),
                      (burst_kv, B * kv_bursts),
                      (burst_w3, (NBAND - 1) * band_bursts)):
            plan.append((u0, n, fn))
            u0 += n
        n_bursts = u0

        def issue(first, count, lo, hi):
            hits = [(u0, n, fn) for u0, n, fn in plan if u0 < hi and lo < u0 + n]

            def one(u):
                for u0, n, fn in hits:
                    if len(hits) == 1:
                        fn(u - u0)
                    else:
                        pl.when(jnp.logical_and(u >= u0, u < u0 + n))(lambda: fn(u - u0))

            if count == 1:
                one(first)
            else:
                def body(i, c):
                    one(first + i)
                    return c
                jax.lax.fori_loop(0, count, body, 0)

        class Cursor:
            pos = 0

            def to(self, hi):
                assert self.pos <= hi <= n_bursts, (self.pos, hi)
                for u0, n, _ in plan:
                    a, b = max(self.pos, u0), min(hi, u0 + n)
                    if a < b:
                        issue(a, b - a, a, b)
                self.pos = hi

            def loop(self, iters, counts):
                per = sum(counts)
                lo, hi = self.pos, self.pos + iters * per
                assert hi <= n_bursts
                self.pos = hi

                def f(i, k):
                    if counts[k]:
                        issue(lo + i * per + sum(counts[:k]), counts[k], lo, hi)
                return f

        cur = Cursor()

        start(x_h, x_v, S_X, 0)
        start(gw_h, gw_v, S_GW, 1)
        cur.to(cfg["u_qabs"])

        wait(x_v, S_X)
        wait(gw_v, S_GW)
        wait(wq_v, S_WQ)
        wait(wuk_v, S_WUK)
        nsp = cfg["split_steps"]
        iss_s = cur.loop(nsp, cfg["n_split"])

        def split_qk(i, carry):
            _split_heads(wq_v, t0_s, i, nsp, H)
            _split_heads(wuk_v, t1_s, i, nsp, H)
            iss_s(i, 0)
            return carry

        jax.lax.fori_loop(0, nsp, split_qk, 0)
        iss_q = cur.loop(H // 2, cfg["n_qabs"])

        def qabs_body(j, carry):
            x = x_v[...]
            for p in range(2):
                wq_ = _head(t0_s, j, p, H, M)
                wk_ = _head(t1_s, j, p, H, Dc)
                q = jnp.dot(x, wq_, preferred_element_type=F32).astype(BF16)
                qa = jax.lax.dot_general(q, wk_, _NT, preferred_element_type=F32)
                row = pl.multiple_of((2 * j + p) * B, B)
                qa = qa * scale
                for t in range(Dc // 128):
                    qabs_s[t, pl.ds(row, B), :] = qa[:, t * 128:(t + 1) * 128]
            iss_q(j, 0)
            return carry

        jax.lax.fori_loop(0, H // 2, qabs_body, 0)

        wait(bwq_v, S_BWQ)
        wait(wuv_v, S_WUV)
        qb = jnp.dot(x_v[...], bwq_v[...].reshape(M, HD), preferred_element_type=F32)
        qb = qb.astype(BF16).astype(F32)
        for h in range(H):
            qb_s[h * B:(h + 1) * B, :] = qb[:, h * D:(h + 1) * D]

        iss_v = cur.loop(nsp // 2, cfg["n_split"])

        def split_v(i, carry):
            iss_v(i, 0)
            _split_heads(wuv_v, t0_s, i, nsp // 2, H)
            return carry

        jax.lax.fori_loop(0, nsp // 2, split_v, 0)

        cur.to(cfg["u_attn_a"])
        iss_a = cur.loop(B, cfg["n_attn_a"])

        def attn_a(b, carry):
            for half in range(2):
                pl.when(b == half * (B // 2))(
                    lambda: wait(ckv_v.at[pl.ds(half * 2 * NSTR, 2 * NSTR)], S_CKV + half))

            qa = jnp.concatenate(
                [qabs_s[t, pl.ds(b, H, stride=B), :] for t in range(Dc // 128)],
                axis=1).astype(BF16)
            c = ckv_v[pl.ds(b * CS, CS)].reshape(Sk, Dc)
            s = jax.lax.dot_general(qa, c, _NT, preferred_element_type=F32)
            iss_a(b, 0)
            m = jnp.max(s, axis=-1, keepdims=True)
            p = jnp.exp(s - m)
            l = jnp.sum(p, axis=-1, keepdims=True)
            c = ckv_v[pl.ds(b * CS, CS)].reshape(Sk, Dc)
            lat = jnp.dot(p.astype(BF16), c, preferred_element_type=F32)
            lat = lat / l
            row = pl.multiple_of(b * H, H)
            for t in range(Dc // 128):
                lat_s[t, pl.ds(row, H), :] = lat[:, t * 128:(t + 1) * 128]
            iss_a(b, 1)
            return carry

        jax.lax.fori_loop(0, B, attn_a, 0)

        iss_c = cur.loop(H // 2, cfg["n_ctx"])

        def ctx_body(j, carry):
            for p in range(2):
                lat = jnp.concatenate(
                    [lat_s[t, pl.ds(2 * j + p, B, stride=H), :] for t in range(Dc // 128)],
                    axis=1).astype(BF16)
                ctx_s[2 * j + p] = jnp.dot(lat, _head(t0_s, j, p, H, Dc),
                                           preferred_element_type=F32)
            iss_c(j, 0)
            return carry

        jax.lax.fori_loop(0, H // 2, ctx_body, 0)

        cur.to(cfg["u_attn_b"])
        iss_b = cur.loop(B, cfg["n_attn_b"])
        first = jax.lax.broadcasted_iota(jnp.int32, (2 * rep, 1), 0) < rep

        def attn_b(b, carry):
            iss_b(b, 0)
            unit, sub = _divmod_pow2(b, UB)

            @pl.when(sub == 0)
            def _():
                wait(kc_v.at[pl.ds(unit * NSTR, NSTR)], S_KV + 2 * unit)
                wait(vc_v.at[pl.ds(unit * NSTR, NSTR)], S_KV + 2 * unit + 1)

            for gp in range(HP):
                if gp == HP // 2:
                    iss_b(b, 1)
                a = b * HP + gp
                q = qb_s[pl.ds(gp * 2 * rep * B + b, 2 * rep, stride=B), :].astype(BF16)
                s0 = jax.lax.dot_general(q, kc_v[a, 0], _NT, preferred_element_type=F32)
                s1 = jax.lax.dot_general(q, kc_v[a, 1], _NT, preferred_element_type=F32)
                s = jnp.where(first, s0, s1) * scale
                m = jnp.max(s, axis=-1, keepdims=True)
                p = jnp.exp(s - m)
                l = jnp.sum(p, axis=-1, keepdims=True)
                p = p.astype(BF16)
                o0 = jnp.dot(p, vc_v[a, 0], preferred_element_type=F32)
                o1 = jnp.dot(p, vc_v[a, 1], preferred_element_type=F32)
                row = pl.multiple_of(a * 2 * rep, 2 * rep)
                ob_s[pl.ds(row, 2 * rep), :] = jnp.where(first, o0, o1) / l
            return carry

        jax.lax.fori_loop(0, B, attn_b, 0)

        def lhs(which, s0, ns, band):
            hs = [s * NBAND + band for s in range(s0, s0 + ns)]
            if which == 0:
                parts = [ctx_s[h] for h in hs]
            else:
                parts = [ob_s[pl.ds(h, B, stride=H), :] for h in hs]
            return jnp.concatenate(parts, axis=1).astype(BF16)

        def proj(l, which, s0, ns, band):
            w = (wo_v, bwo_v)[which][pl.ds(s0, ns), pl.ds(band * D, D), :].reshape(ns * D, M)
            return jnp.dot(l, w, preferred_element_type=F32)

        def do_band(which, band):
            wait((wo_v, bwo_v)[which].at[:, pl.ds(band * D, D)], S_W3 + 2 * band + which)
            r = proj(lhs(which, 0, NSTR, band), which, 0, NSTR, band)
            acc_s[which] = r if band == 0 else acc_s[which] + r

        last = NBAND - 1
        todo = [(which, band) for band in range(NBAND) for which in range(2)][:-1]
        for u, n in cfg["u_band"]:
            cur.to(u)
            for _ in range(n):
                do_band(*todo.pop(0))
        cur.to(n_bursts)

        narrow = []
        s0 = 0
        for k, ns in enumerate(tail_blocks):
            rows = 32 // ns
            narrow += [((pl.ds(s0, ns), pl.ds(r, rows), every), S_TAIL + k)
                       for r in range(last * D, (last + 1) * D, rows)]
            s0 += ns
        for i, (sl, sem) in enumerate(narrow):
            tiles2(wo_h, wo_v, every, last * D + 8 * (i // nmc), 256 * (i % nmc), S_W3 + 2 * last, 0)
            start(bwo_h.at[sl], bwo_v.at[sl], sem, 1)

        xf = x_v[...].astype(F32)
        gw = gw_v[...].astype(F32)
        t = xf[:, 0:128] * gw[0:1, :]
        for i in range(1, M // 128):
            t = t + xf[:, i * 128:(i + 1) * 128] * gw[i:i + 1, :]
        gate = jax.nn.sigmoid(jnp.sum(t, axis=-1, keepdims=True))

        for which, band in todo:
            do_band(which, band)
        starts = [sum(tail_blocks[:k]) for k in range(len(tail_blocks))]
        tail_lhs = [lhs(1, s0, ns, last) for s0, ns in zip(starts, tail_blocks)]
        out = gate * acc_s[0]
        acc = acc_s[1]
        for k, (s0, ns) in enumerate(zip(starts, tail_blocks)):
            wait(bwo_v.at[pl.ds(s0, ns), pl.ds(last * D, D)], S_TAIL + k)
            acc = acc + proj(tail_lhs[k], 1, s0, ns, last)
        o_ref[...] = (out + (1.0 - gate) * acc).astype(o_ref.dtype)

    return kernel, n_sems


DEFAULT_CFG = dict(
    u_qabs=22, split_steps=16, n_split=(1,), n_qabs=(1,),
    u_attn_a=78, n_attn_a=(3, 3),
    n_ctx=(1,),
    u_attn_b=148, n_attn_b=(2, 1),
    u_band=((172, 3),),
    tail_blocks=(4, 2, 1, 1),
)
DEFAULT_PARAMS = dict(disable_bounds_checks=True, disable_semaphore_checks=True)


def _forward(A_x, A_c_kv, A_w_q, A_w_uk, A_w_uv, A_w_o, B_k_cache, B_v_cache, B_wq, B_wo,
             gate_w, cfg, params):
    B, Sq, M = A_x.shape
    assert Sq == 1
    _, Sk, Dc = A_c_kv.shape
    _, H, D = A_w_q.shape
    _, Hkv, SkB, _ = B_k_cache.shape
    W = min(4096, max(256, SkB // 4))
    HD = H * D

    kernel, n_sems = _make_kernel(B, M, H, D, Dc, Sk, Hkv, SkB, W, cfg)
    any_spec = pl.BlockSpec(memory_space=pl.ANY)
    out = pl.pallas_call(
        kernel,
        out_shape=jax.ShapeDtypeStruct((B, M), A_x.dtype),
        in_specs=[any_spec] * 11,
        out_specs=pl.BlockSpec(memory_space=pltpu.VMEM),
        scratch_shapes=[
            pltpu.VMEM((B, M), BF16),
            pltpu.VMEM((M // 128, 128), BF16),
            pltpu.VMEM((B * 4, Sk // 4, Dc), BF16),
            pltpu.VMEM((NSTR, M * H // NSTR, D), BF16),
            pltpu.VMEM((NSTR, Dc * H // NSTR, D), BF16),
            pltpu.VMEM((NSTR, Dc * H // NSTR, D), BF16),
            pltpu.VMEM((NSTR, HD // NSTR, M), BF16),
            pltpu.VMEM((B * Hkv // 2, 2, W, D), BF16),
            pltpu.VMEM((B * Hkv // 2, 2, W, D), BF16),
            pltpu.VMEM((NSTR, M // NSTR, HD), BF16),
            pltpu.VMEM((NSTR, HD // NSTR, M), BF16),
            pltpu.VMEM((H * PLANE, D), U32),
            pltpu.VMEM((H * PLANE, D), U32),
            pltpu.VMEM((Dc // 128, H * B, 128), F32),
            pltpu.VMEM((Dc // 128, B * H, 128), F32),
            pltpu.VMEM((H, B, D), F32),
            pltpu.VMEM((H * B, D), F32),
            pltpu.VMEM((B * H, D), F32),
            pltpu.VMEM((2, B, M), F32),
            pltpu.SemaphoreType.DMA((n_sems,)),
        ],
        compiler_params=pltpu.CompilerParams(vmem_limit_bytes=112 * 1024 * 1024, **params),
        name="gated_mix_decode",
    )(
        A_x.reshape(B, M),
        gate_w.reshape(M // 128, 128),
        A_c_kv.reshape(B * 4, Sk // 4, Dc),
        A_w_q.reshape(NSTR, M * H // NSTR, D),
        A_w_uk.reshape(NSTR, Dc * H // NSTR, D),
        A_w_uv.reshape(NSTR, Dc * H // NSTR, D),
        A_w_o.reshape(NSTR, HD // NSTR, M),
        B_k_cache.reshape(B * Hkv // 2, 2, SkB, D),
        B_v_cache.reshape(B * Hkv // 2, 2, SkB, D),
        B_wq.reshape(NSTR, M // NSTR, HD),
        B_wo.reshape(NSTR, HD // NSTR, M),
    )
    return out.reshape(B, 1, M)


@jax.jit
def pallas_gated_mix__compressed_kv_cla__sliding_block_cached__decode_kernel(
    A_x: jax.Array,
    A_c_kv: jax.Array,
    A_w_q: jax.Array,
    A_w_uk: jax.Array,
    A_w_uv: jax.Array,
    A_w_o: jax.Array,
    B_x: jax.Array,
    B_k_cache: jax.Array,
    B_v_cache: jax.Array,
    B_wq: jax.Array,
    B_wo: jax.Array,
    gate_w: jax.Array,
):
    return _forward(A_x, A_c_kv, A_w_q, A_w_uk, A_w_uv, A_w_o, B_k_cache, B_v_cache,
                    B_wq, B_wo, gate_w, DEFAULT_CFG, DEFAULT_PARAMS)
```

```python
import jax
import jax.numpy as jnp
import jax.experimental.pallas as pl
import jax.experimental.pallas.tpu as pltpu

F32 = jnp.float32
BF16 = jnp.bfloat16
U32 = jnp.uint32

_NT = (((1,), (1,)), ((), ()))

NSTR = 8
BURST = 8
PLANE = 264


def _divmod_pow2(u, n):
    assert n & (n - 1) == 0
    return u >> (n.bit_length() - 1), u & (n - 1)


def _mult(v, n):
    return v if isinstance(v, int) else pl.multiple_of(v, n)


def _split_heads(w_v, t_s, step, nsteps, heads):
    ns, rr, _ = w_v.shape
    per_stream = nsteps // ns
    stream, part = _divmod_pow2(step, per_stream)
    rows = rr // per_stream
    half = heads // 2
    for k in range(rows // (2 * heads)):
        r0 = pl.multiple_of(part * rows + k * 2 * heads, 2 * heads)
        w = pltpu.bitcast(w_v[stream, pl.ds(r0, 2 * heads), :], U32)
        ev, od = w[:half], w[half:]
        lo = (ev & jnp.uint32(0xFFFF)) | (od << 16)
        hi = (ev >> 16) | (od & jnp.uint32(0xFFFF0000))
        i = step * (rows // (2 * heads)) + k
        t_s[pl.ds(i, half, stride=PLANE), :] = lo
        t_s[pl.ds(half * PLANE + i, half, stride=PLANE), :] = hi


def _head(t_s, j, p, heads, rows):
    r0 = pl.multiple_of((p * (heads // 2) + j) * PLANE, 8)
    return pltpu.bitcast(t_s[pl.ds(r0, rows // 2), :], BF16)


def _make_kernel(B, M, H, D, Dc, Sk, Hkv, SkB, W, cfg):
    rep = H // Hkv
    scale = float(D) ** -0.5
    HD = H * D
    CS = 4
    CR = Sk // CS
    OR = HD // NSTR
    NBAND = OR // D
    HP = Hkv // 2
    UB = NSTR // HP
    tail_blocks = cfg["tail_blocks"]
    assert sum(tail_blocks) == NSTR and max(M, Dc) // 2 <= PLANE

    S_X, S_GW, S_WQ, S_WUK, S_BWQ, S_WUV, S_CKV = 0, 1, 2, 3, 4, 5, 6
    S_KV = S_CKV + 2
    S_W3 = S_KV + 2 * (B // UB)
    S_TAIL = S_W3 + 2 * NBAND - 1
    n_sems = S_TAIL + len(tail_blocks)

    def kernel(x_h, gw_h, ckv_h, wq_h, wuk_h, wuv_h, wo_h, kc_h, vc_h, bwq_h, bwo_h,
               o_ref,
               x_v, gw_v, ckv_v, wq_v, wuk_v, wuv_v, wo_v, kc_v, vc_v, bwq_v, bwo_v,
               t0_s, t1_s, qabs_s, lat_s, ctx_s, qb_s, ob_s, acc_s, sems):
        def start(src, dst, sem, prio):
            pltpu.make_async_copy(src, dst, sems.at[sem]).start(priority=prio)

        def wait(buf, sem):
            pltpu.make_async_copy(buf, buf, sems.at[sem]).wait()

        every = slice(None)

        def rows16(src, dst, r, sem, prio):
            sl = (every, pl.ds(_mult(r, 16), 16), every)
            start(src.at[sl], dst.at[sl], sem, prio)

        def tiles2(src, dst, lead, r, c, sem, prio):
            sl = (lead, pl.ds(_mult(r, 8), 8), pl.ds(_mult(c, 256), 256))
            start(src.at[sl], dst.at[sl], sem, prio)

        def burst_w1(u):
            rb, ch = _divmod_pow2(u, HD // 256 // BURST)
            for i in range(BURST):
                rows16(wq_h, wq_v, u * (16 * BURST) + 16 * i, S_WQ, 0)
                tiles2(bwq_h, bwq_v, every, rb * 8, ch * (256 * BURST) + 256 * i, S_BWQ, 1)

        def burst_w2(u):
            for i in range(BURST):
                r = u * (16 * BURST) + 16 * i
                rows16(wuk_h, wuk_v, r, S_WUK, 0)
                rows16(wuv_h, wuv_v, r, S_WUV, 1)

        ncc = Dc // 256
        ckv_bursts = (CR // 8) * ncc // BURST

        def burst_ckv(u):
            half, uu = _divmod_pow2(u, ckv_bursts)
            for i in range(BURST):
                r = uu * (8 * BURST // ncc) + 8 * (i // ncc)
                for t in range(2):
                    lead = pl.ds(half * (2 * NSTR) + t * NSTR, NSTR)
                    tiles2(ckv_h, ckv_v, lead, r, 256 * (i % ncc), S_CKV + half, t)

        kv_bursts = W // 16 // BURST

        def burst_kv(u):
            q, uu = _divmod_pow2(u, kv_bursts)
            unit, par = _divmod_pow2(q, 2)
            lead = pl.ds(unit * NSTR, NSTR)
            for i in range(BURST):
                r = uu * (16 * BURST) + 16 * i
                for t, (src, dst) in enumerate(((kc_h, kc_v), (vc_h, vc_v))):
                    start(src.at[lead, par, pl.ds(_mult(SkB - W + r, 16), 16)],
                          dst.at[lead, par, pl.ds(_mult(r, 16), 16)], S_KV + 2 * unit + t, t)

        nmc = M // 256
        band_bursts = (D // 8) * nmc // BURST

        def burst_w3(u):
            band, _ = _divmod_pow2(u, band_bursts)
            for i in range(BURST):
                r = u * (8 * BURST // nmc) + 8 * (i // nmc)
                c = 256 * (i % nmc)
                tiles2(wo_h, wo_v, every, r, c, S_W3 + 2 * band, 0)
                tiles2(bwo_h, bwo_v, every, r, c, S_W3 + 2 * band + 1, 1)

        plan = []
        u0 = 0
        for fn, n in ((burst_w1, wq_v.shape[1] // 16 // BURST),
                      (burst_w2, wuv_v.shape[1] // 16 // BURST),
                      (burst_ckv, 2 * ckv_bursts),
                      (burst_kv, B * kv_bursts),
                      (burst_w3, (NBAND - 1) * band_bursts)):
            plan.append((u0, n, fn))
            u0 += n
        n_bursts = u0
        u_w2, u_ckv, u_kv, u_w3 = (p[0] for p in plan[1:])

        def issue(first, count, lo, hi):
            hits = [(u0, n, fn) for u0, n, fn in plan if u0 < hi and lo < u0 + n]

            def one(u):
                for u0, n, fn in hits:
                    if len(hits) == 1:
                        fn(u - u0)
                    else:
                        pl.when(jnp.logical_and(u >= u0, u < u0 + n))(lambda: fn(u - u0))

            if count == 1:
                one(first)
            else:
                def body(i, c):
                    one(first + i)
                    return c
                jax.lax.fori_loop(0, count, body, 0)

        class Cursor:
            pos = 0

            def to(self, hi):
                assert self.pos <= hi <= n_bursts, (self.pos, hi)
                for u0, n, _ in plan:
                    a, b = max(self.pos, u0), min(hi, u0 + n)
                    if a < b:
                        issue(a, b - a, a, b)
                self.pos = hi

            def loop(self, iters, counts):
                per = sum(counts)
                lo, hi = self.pos, self.pos + iters * per
                assert hi <= n_bursts
                self.pos = hi

                def f(i, k):
                    if counts[k]:
                        issue(lo + i * per + sum(counts[:k]), counts[k], lo, hi)
                return f

        cur = Cursor()

        def split_loop(w_v, t_s):
            n = cfg["split_steps"]
            iss = cur.loop(n, cfg["n_split"])

            def body(i, carry):
                iss(i, 0)
                _split_heads(w_v, t_s, i, n, H)
                return carry

            jax.lax.fori_loop(0, n, body, 0)

        cur.to(1)
        start(x_h, x_v, S_X, 0)
        start(gw_h, gw_v, S_GW, 1)
        cur.to(cfg["u_q"])

        assert cur.pos >= u_w2
        wait(x_v, S_X)
        wait(gw_v, S_GW)
        wait(wq_v, S_WQ)
        wait(bwq_v, S_BWQ)
        qb = jnp.dot(x_v[...], bwq_v[...].reshape(M, HD), preferred_element_type=F32)
        qb = qb.astype(BF16).astype(F32)
        for h in range(H):
            qb_s[h * B:(h + 1) * B, :] = qb[:, h * D:(h + 1) * D]

        split_loop(wq_v, t0_s)
        cur.to(cfg["u_uk"])
        assert cur.pos >= u_ckv
        wait(wuk_v, S_WUK)
        wait(wuv_v, S_WUV)
        split_loop(wuk_v, t1_s)
        iss_q = cur.loop(H // 2, cfg["n_qabs"])

        def qabs_body(j, carry):
            x = x_v[...]
            for p in range(2):
                q = jnp.dot(x, _head(t0_s, j, p, H, M),
                            preferred_element_type=F32).astype(BF16)
                qa = jax.lax.dot_general(q, _head(t1_s, j, p, H, Dc), _NT,
                                         preferred_element_type=F32) * scale
                row = pl.multiple_of((2 * j + p) * B, B)
                for t in range(Dc // 128):
                    qabs_s[t, pl.ds(row, B), :] = qa[:, t * 128:(t + 1) * 128]
            iss_q(j, 0)
            return carry

        jax.lax.fori_loop(0, H // 2, qabs_body, 0)
        split_loop(wuv_v, t0_s)

        cur.to(cfg["u_attn_a"])
        for half in range(2):
            assert cur.pos + half * (B // 2) * sum(cfg["n_attn_a"]) >= u_ckv + (half + 1) * ckv_bursts
        iss_a = cur.loop(B, cfg["n_attn_a"])

        def attn_a(b, carry):
            for half in range(2):
                pl.when(b == half * (B // 2))(
                    lambda: wait(ckv_v.at[pl.ds(half * 2 * NSTR, 2 * NSTR)], S_CKV + half))

            qa = jnp.concatenate(
                [qabs_s[t, pl.ds(b, H, stride=B), :] for t in range(Dc // 128)],
                axis=1).astype(BF16)
            c = ckv_v[pl.ds(b * CS, CS)].reshape(Sk, Dc)
            s = jax.lax.dot_general(qa, c, _NT, preferred_element_type=F32)
            iss_a(b, 0)
            m = jnp.max(s, axis=-1, keepdims=True)
            p = jnp.exp(s - m)
            l = jnp.sum(p, axis=-1, keepdims=True)
            c = ckv_v[pl.ds(b * CS, CS)].reshape(Sk, Dc)
            lat = jnp.dot(p.astype(BF16), c, preferred_element_type=F32)
            lat = lat / l
            row = pl.multiple_of(b * H, H)
            for t in range(Dc // 128):
                lat_s[t, pl.ds(row, H), :] = lat[:, t * 128:(t + 1) * 128]
            iss_a(b, 1)
            return carry

        jax.lax.fori_loop(0, B, attn_a, 0)

        iss_c = cur.loop(H // 2, cfg["n_ctx"])

        def ctx_body(j, carry):
            for p in range(2):
                lat = jnp.concatenate(
                    [lat_s[t, pl.ds(2 * j + p, B, stride=H), :] for t in range(Dc // 128)],
                    axis=1).astype(BF16)
                ctx_s[2 * j + p] = jnp.dot(lat, _head(t0_s, j, p, H, Dc),
                                           preferred_element_type=F32)
            iss_c(j, 0)
            return carry

        jax.lax.fori_loop(0, H // 2, ctx_body, 0)

        cur.to(cfg["u_attn_b"])
        for unit in range(B // UB):
            assert (cur.pos + unit * UB * sum(cfg["n_attn_b"]) + cfg["n_attn_b"][0]
                    >= u_kv + (unit + 1) * 2 * kv_bursts)
        iss_b = cur.loop(B, cfg["n_attn_b"])
        first = jax.lax.broadcasted_iota(jnp.int32, (2 * rep, 1), 0) < rep

        def attn_b(b, carry):
            iss_b(b, 0)
            unit, sub = _divmod_pow2(b, UB)

            @pl.when(sub == 0)
            def _():
                wait(kc_v.at[pl.ds(unit * NSTR, NSTR)], S_KV + 2 * unit)
                wait(vc_v.at[pl.ds(unit * NSTR, NSTR)], S_KV + 2 * unit + 1)

            for gp in range(HP):
                if gp == HP // 2:
                    iss_b(b, 1)
                a = b * HP + gp
                q = qb_s[pl.ds(gp * 2 * rep * B + b, 2 * rep, stride=B), :].astype(BF16)
                s0 = jax.lax.dot_general(q, kc_v[a, 0], _NT, preferred_element_type=F32)
                s1 = jax.lax.dot_general(q, kc_v[a, 1], _NT, preferred_element_type=F32)
                s = jnp.where(first, s0, s1) * scale
                m = jnp.max(s, axis=-1, keepdims=True)
                p = jnp.exp(s - m)
                l = jnp.sum(p, axis=-1, keepdims=True)
                p = p.astype(BF16)
                o0 = jnp.dot(p, vc_v[a, 0], preferred_element_type=F32)
                o1 = jnp.dot(p, vc_v[a, 1], preferred_element_type=F32)
                row = pl.multiple_of(a * 2 * rep, 2 * rep)
                ob_s[pl.ds(row, 2 * rep), :] = jnp.where(first, o0, o1) / l
            return carry

        jax.lax.fori_loop(0, B, attn_b, 0)

        def lhs(which, s0, ns, band):
            hs = [s * NBAND + band for s in range(s0, s0 + ns)]
            if which == 0:
                parts = [ctx_s[h] for h in hs]
            else:
                parts = [ob_s[pl.ds(h, B, stride=H), :] for h in hs]
            return jnp.concatenate(parts, axis=1).astype(BF16)

        def proj(l, which, s0, ns, band):
            w = (wo_v, bwo_v)[which][pl.ds(s0, ns), pl.ds(band * D, D), :].reshape(ns * D, M)
            return jnp.dot(l, w, preferred_element_type=F32)

        def do_band(which, band):
            wait((wo_v, bwo_v)[which].at[:, pl.ds(band * D, D)], S_W3 + 2 * band + which)
            r = proj(lhs(which, 0, NSTR, band), which, 0, NSTR, band)
            acc_s[which] = r if band == 0 else acc_s[which] + r

        last = NBAND - 1
        todo = [(which, band) for band in range(NBAND) for which in range(2)][:-1]
        for u, n in cfg["u_band"]:
            cur.to(u)
            for _ in range(n):
                which, band = todo.pop(0)
                assert band < last and cur.pos >= u_w3 + (band + 1) * band_bursts
                do_band(which, band)
        cur.to(n_bursts)

        starts = [sum(tail_blocks[:k]) for k in range(len(tail_blocks))]
        narrow = []
        for k, (s0, ns) in enumerate(zip(starts, tail_blocks)):
            rows = 32 // ns
            narrow += [((pl.ds(s0, ns), pl.ds(r, rows), every), S_TAIL + k)
                       for r in range(last * D, (last + 1) * D, rows)]
        assert len(narrow) == (D // 8) * nmc
        for i, (sl, sem) in enumerate(narrow):
            tiles2(wo_h, wo_v, every, last * D + 8 * (i // nmc), 256 * (i % nmc), S_W3 + 2 * last, 0)
            start(bwo_h.at[sl], bwo_v.at[sl], sem, 1)

        xf = x_v[...].astype(F32)
        gw = gw_v[...].astype(F32)
        t = xf[:, 0:128] * gw[0:1, :]
        for i in range(1, M // 128):
            t = t + xf[:, i * 128:(i + 1) * 128] * gw[i:i + 1, :]
        gate = jax.nn.sigmoid(jnp.sum(t, axis=-1, keepdims=True))

        for which, band in todo:
            do_band(which, band)
        tail_lhs = [lhs(1, s0, ns, last) for s0, ns in zip(starts, tail_blocks)]
        out = gate * acc_s[0]
        acc = acc_s[1]
        for k, (s0, ns) in enumerate(zip(starts, tail_blocks)):
            wait(bwo_v.at[pl.ds(s0, ns), pl.ds(last * D, D)], S_TAIL + k)
            acc = acc + proj(tail_lhs[k], 1, s0, ns, last)
        o_ref[...] = (out + (1.0 - gate) * acc).astype(o_ref.dtype)

    return kernel, n_sems


DEFAULT_CFG = dict(
    u_q=22, split_steps=8, n_split=(1,), u_uk=38, n_qabs=(1,),
    u_attn_a=78, n_attn_a=(3, 3),
    n_ctx=(1,),
    u_attn_b=148, n_attn_b=(2, 1),
    u_band=((172, 3),),
    tail_blocks=(4, 2, 1, 1),
)
DEFAULT_PARAMS = dict(disable_bounds_checks=True, disable_semaphore_checks=True)


def _forward(A_x, A_c_kv, A_w_q, A_w_uk, A_w_uv, A_w_o, B_k_cache, B_v_cache, B_wq, B_wo,
             gate_w, cfg, params):
    B, Sq, M = A_x.shape
    assert Sq == 1
    _, Sk, Dc = A_c_kv.shape
    _, H, D = A_w_q.shape
    _, Hkv, SkB, _ = B_k_cache.shape
    W = min(4096, max(256, SkB // 4))
    HD = H * D

    kernel, n_sems = _make_kernel(B, M, H, D, Dc, Sk, Hkv, SkB, W, cfg)
    any_spec = pl.BlockSpec(memory_space=pl.ANY)
    out = pl.pallas_call(
        kernel,
        out_shape=jax.ShapeDtypeStruct((B, M), A_x.dtype),
        in_specs=[any_spec] * 11,
        out_specs=pl.BlockSpec(memory_space=pltpu.VMEM),
        scratch_shapes=[
            pltpu.VMEM((B, M), BF16),
            pltpu.VMEM((M // 128, 128), BF16),
            pltpu.VMEM((B * 4, Sk // 4, Dc), BF16),
            pltpu.VMEM((NSTR, M * H // NSTR, D), BF16),
            pltpu.VMEM((NSTR, Dc * H // NSTR, D), BF16),
            pltpu.VMEM((NSTR, Dc * H // NSTR, D), BF16),
            pltpu.VMEM((NSTR, HD // NSTR, M), BF16),
            pltpu.VMEM((B * Hkv // 2, 2, W, D), BF16),
            pltpu.VMEM((B * Hkv // 2, 2, W, D), BF16),
            pltpu.VMEM((NSTR, M // NSTR, HD), BF16),
            pltpu.VMEM((NSTR, HD // NSTR, M), BF16),
            pltpu.VMEM((H * PLANE, D), U32),
            pltpu.VMEM((H * PLANE, D), U32),
            pltpu.VMEM((Dc // 128, H * B, 128), F32),
            pltpu.VMEM((Dc // 128, B * H, 128), F32),
            pltpu.VMEM((H, B, D), F32),
            pltpu.VMEM((H * B, D), F32),
            pltpu.VMEM((B * H, D), F32),
            pltpu.VMEM((2, B, M), F32),
            pltpu.SemaphoreType.DMA((n_sems,)),
        ],
        compiler_params=pltpu.CompilerParams(vmem_limit_bytes=112 * 1024 * 1024, **params),
        name="gated_mix_decode",
    )(
        A_x.reshape(B, M),
        gate_w.reshape(M // 128, 128),
        A_c_kv.reshape(B * 4, Sk // 4, Dc),
        A_w_q.reshape(NSTR, M * H // NSTR, D),
        A_w_uk.reshape(NSTR, Dc * H // NSTR, D),
        A_w_uv.reshape(NSTR, Dc * H // NSTR, D),
        A_w_o.reshape(NSTR, HD // NSTR, M),
        B_k_cache.reshape(B * Hkv // 2, 2, SkB, D),
        B_v_cache.reshape(B * Hkv // 2, 2, SkB, D),
        B_wq.reshape(NSTR, M // NSTR, HD),
        B_wo.reshape(NSTR, HD // NSTR, M),
    )
    return out.reshape(B, 1, M)


@jax.jit
def pallas_gated_mix__compressed_kv_cla__sliding_block_cached__decode_kernel(
    A_x: jax.Array,
    A_c_kv: jax.Array,
    A_w_q: jax.Array,
    A_w_uk: jax.Array,
    A_w_uv: jax.Array,
    A_w_o: jax.Array,
    B_x: jax.Array,
    B_k_cache: jax.Array,
    B_v_cache: jax.Array,
    B_wq: jax.Array,
    B_wo: jax.Array,
    gate_w: jax.Array,
):
    return _forward(A_x, A_c_kv, A_w_q, A_w_uk, A_w_uv, A_w_o, B_k_cache, B_v_cache,
                    B_wq, B_wo, gate_w, DEFAULT_CFG, DEFAULT_PARAMS)
```

```python
import jax
import jax.numpy as jnp
import jax.experimental.pallas as pl
import jax.experimental.pallas.tpu as pltpu

F32 = jnp.float32
BF16 = jnp.bfloat16
U32 = jnp.uint32

_NT = (((1,), (1,)), ((), ()))

NSTR = 8
BURST = 8
PLANE = 264


def _divmod_pow2(u, n):
    assert n & (n - 1) == 0
    return u >> (n.bit_length() - 1), u & (n - 1)


def _mult(v, n):
    return v if isinstance(v, int) else pl.multiple_of(v, n)


def _split_heads(w_v, t_s, step, nsteps, heads):
    ns, rr, _ = w_v.shape
    per_stream = nsteps // ns
    stream, part = _divmod_pow2(step, per_stream)
    rows = rr // per_stream
    half = heads // 2
    for k in range(rows // (2 * heads)):
        r0 = pl.multiple_of(part * rows + k * 2 * heads, 2 * heads)
        w = pltpu.bitcast(w_v[stream, pl.ds(r0, 2 * heads), :], U32)
        ev, od = w[:half], w[half:]
        lo = (ev & jnp.uint32(0xFFFF)) | (od << 16)
        hi = (ev >> 16) | (od & jnp.uint32(0xFFFF0000))
        i = step * (rows // (2 * heads)) + k
        t_s[pl.ds(i, half, stride=PLANE), :] = lo
        t_s[pl.ds(half * PLANE + i, half, stride=PLANE), :] = hi


def _head(t_s, j, p, heads, rows):
    r0 = pl.multiple_of((p * (heads // 2) + j) * PLANE, 8)
    return pltpu.bitcast(t_s[pl.ds(r0, rows // 2), :], BF16)


def _make_kernel(B, M, H, D, Dc, Sk, Hkv, SkB, W, cfg):
    rep = H // Hkv
    scale = float(D) ** -0.5
    HD = H * D
    CS = 4
    CR = Sk // CS
    OR = HD // NSTR
    NBAND = OR // D
    HP = Hkv // 2
    UB = NSTR // HP
    tail_blocks = cfg["tail_blocks"]
    skews = cfg["skews"]
    assert skews[4] <= D // 4
    assert sum(tail_blocks) == NSTR and max(M, Dc) // 2 <= PLANE

    S_X, S_GW, S_WQ, S_WUK, S_BWQ, S_WUV, S_CKV = 0, 1, 2, 3, 4, 5, 6
    S_KV = S_CKV + 2
    S_W3 = S_KV + 2 * (B // UB)
    S_TAIL = S_W3 + 2 * NBAND - 1
    n_sems = S_TAIL + len(tail_blocks)

    def kernel(x_h, gw_h, ckv_h, wq_h, wuk_h, wuv_h, wo_h, kc_h, vc_h, bwq_h, bwo_h,
               o_ref,
               x_v, gw_v, ckv_v, wq_v, wuk_v, wuv_v, wo_v, kc_v, vc_v, bwq_v, bwo_v,
               t0_s, t1_s, qabs_s, lat_s, ctx_s, qb_s, ob_s, acc_s, sems):
        def start(src, dst, sem, prio):
            pltpu.make_async_copy(src, dst, sems.at[sem]).start(priority=prio)

        def wait(buf, sem):
            pltpu.make_async_copy(buf, buf, sems.at[sem]).wait()

        every = slice(None)

        def rows16(src, dst, r, sem, prio):
            sl = (every, pl.ds(_mult(r, 16), 16), every)
            start(src.at[sl], dst.at[sl], sem, prio)

        def tiles2(src, dst, lead, r, c, sem, prio):
            sl = (lead, pl.ds(_mult(r, 8), 8), pl.ds(_mult(c, 256), 256))
            start(src.at[sl], dst.at[sl], sem, prio)

        def burst(u, nblk, skew, d0, d1):
            q, r = divmod(skew, BURST)
            blk0 = [(u - q - 1) & (nblk - 1), (u - q) & (nblk - 1)]
            for i in range(BURST):
                d0(blk0[i >= r], (i - r) % BURST)
                d1(u, i)

        def d_rows(src, dst, sem, prio):
            return lambda blk, i: rows16(src, dst, blk * (16 * BURST) + 16 * i, sem, prio)

        def d_tiles(src, dst, lead, sem, prio):
            nc = src.shape[-1] // 256

            def f(blk, i):
                if nc >= BURST:
                    rb, cb = _divmod_pow2(blk, nc // BURST)
                    r, c = rb * 8, cb * (256 * BURST) + 256 * i
                else:
                    r, c = blk * (8 * BURST // nc) + 8 * (i // nc), 256 * (i % nc)
                tiles2(src, dst, lead, r, c, sem(blk) if callable(sem) else sem, prio)
            return f

        w_bursts = wq_v.shape[1] // 16 // BURST

        def burst_w1(u):
            burst(u, w_bursts, skews[0], d_rows(wq_h, wq_v, S_WQ, 0),
                  d_tiles(bwq_h, bwq_v, every, S_BWQ, 1))

        def burst_w2(u):
            burst(u, w_bursts, skews[1], d_rows(wuk_h, wuk_v, S_WUK, 0),
                  d_rows(wuv_h, wuv_v, S_WUV, 1))

        ckv_bursts = (CR // 8) * (Dc // 256) // BURST

        def burst_ckv(u):
            half, uu = _divmod_pow2(u, ckv_bursts)
            d = [d_tiles(ckv_h, ckv_v, pl.ds(half * (2 * NSTR) + t * NSTR, NSTR), S_CKV + half, t)
                 for t in range(2)]
            burst(uu, ckv_bursts, skews[2], *d)

        kv_bursts = W // 16 // BURST

        def burst_kv(u):
            q, uu = _divmod_pow2(u, kv_bursts)
            unit, which = _divmod_pow2(q, 2)
            lead = pl.ds(unit * NSTR, NSTR)

            def go(src, dst):
                def d(t):
                    def f(blk, i):
                        r = blk * (16 * BURST) + 16 * i
                        start(src.at[lead, t, pl.ds(_mult(SkB - W + r, 16), 16)],
                              dst.at[lead, t, pl.ds(_mult(r, 16), 16)], S_KV + q, t)
                    return f
                burst(uu, kv_bursts, skews[3], d(0), d(1))

            pl.when(which == 0)(lambda: go(kc_h, kc_v))
            pl.when(which == 1)(lambda: go(vc_h, vc_v))

        band_bursts = w_bursts // NBAND
        d_wo = d_tiles(wo_h, wo_v, every,
                       lambda blk: S_W3 + 2 * _divmod_pow2(blk, band_bursts)[0], 0)
        d_bwo = d_tiles(bwo_h, bwo_v, every,
                        lambda blk: S_W3 + 2 * _divmod_pow2(blk, band_bursts)[0] + 1, 1)

        def burst_w3(u):
            burst(u, w_bursts, skews[4], d_wo, d_bwo)

        plan = []
        u0 = 0
        for fn, n in ((burst_w1, w_bursts),
                      (burst_w2, w_bursts),
                      (burst_ckv, 2 * ckv_bursts),
                      (burst_kv, B * kv_bursts),
                      (burst_w3, (NBAND - 1) * band_bursts)):
            plan.append((u0, n, fn))
            u0 += n
        n_bursts = u0
        u_w2, u_ckv, u_kv, u_w3 = (p[0] for p in plan[1:])

        def issue(first, count, lo, hi):
            hits = [(u0, n, fn) for u0, n, fn in plan if u0 < hi and lo < u0 + n]

            def one(u):
                for u0, n, fn in hits:
                    if len(hits) == 1:
                        fn(u - u0)
                    else:
                        pl.when(jnp.logical_and(u >= u0, u < u0 + n))(lambda: fn(u - u0))

            if count == 1:
                one(first)
            else:
                def body(i, c):
                    one(first + i)
                    return c
                jax.lax.fori_loop(0, count, body, 0)

        class Cursor:
            pos = 0

            def to(self, hi):
                assert self.pos <= hi <= n_bursts, (self.pos, hi)
                for u0, n, _ in plan:
                    a, b = max(self.pos, u0), min(hi, u0 + n)
                    if a < b:
                        issue(a, b - a, a, b)
                self.pos = hi

            def loop(self, iters, counts):
                per = sum(counts)
                lo, hi = self.pos, self.pos + iters * per
                assert hi <= n_bursts
                self.pos = hi

                def f(i, k):
                    if counts[k]:
                        issue(lo + i * per + sum(counts[:k]), counts[k], lo, hi)
                return f

        cur = Cursor()

        def split_loop(w_v, t_s):
            n = cfg["split_steps"]
            iss = cur.loop(n, cfg["n_split"])

            def body(i, carry):
                iss(i, 0)
                _split_heads(w_v, t_s, i, n, H)
                return carry

            jax.lax.fori_loop(0, n, body, 0)

        cur.to(1)
        start(x_h, x_v, S_X, 0)
        start(gw_h, gw_v, S_GW, 1)
        cur.to(cfg["u_q"])

        assert cur.pos >= u_w2
        wait(x_v, S_X)
        wait(gw_v, S_GW)
        wait(wq_v, S_WQ)
        wait(bwq_v, S_BWQ)
        qb = jnp.dot(x_v[...], bwq_v[...].reshape(M, HD), preferred_element_type=F32)
        qb = qb.astype(BF16).astype(F32)
        for h in range(H):
            qb_s[h * B:(h + 1) * B, :] = qb[:, h * D:(h + 1) * D]

        split_loop(wq_v, t0_s)
        cur.to(cfg["u_uk"])
        assert cur.pos >= u_ckv
        wait(wuk_v, S_WUK)
        wait(wuv_v, S_WUV)
        split_loop(wuk_v, t1_s)
        iss_q = cur.loop(H // 2, cfg["n_qabs"])

        def qabs_body(j, carry):
            x = x_v[...]
            for p in range(2):
                q = jnp.dot(x, _head(t0_s, j, p, H, M),
                            preferred_element_type=F32).astype(BF16)
                qa = jax.lax.dot_general(q, _head(t1_s, j, p, H, Dc), _NT,
                                         preferred_element_type=F32) * scale
                row = pl.multiple_of((2 * j + p) * B, B)
                for t in range(Dc // 128):
                    qabs_s[t, pl.ds(row, B), :] = qa[:, t * 128:(t + 1) * 128]
            iss_q(j, 0)
            return carry

        jax.lax.fori_loop(0, H // 2, qabs_body, 0)
        split_loop(wuv_v, t0_s)

        cur.to(cfg["u_attn_a"])
        for half in range(2):
            assert cur.pos + half * (B // 2) * sum(cfg["n_attn_a"]) >= u_ckv + (half + 1) * ckv_bursts
        iss_a = cur.loop(B, cfg["n_attn_a"])

        def attn_a(b, carry):
            for half in range(2):
                pl.when(b == half * (B // 2))(
                    lambda: wait(ckv_v.at[pl.ds(half * 2 * NSTR, 2 * NSTR)], S_CKV + half))

            qa = jnp.concatenate(
                [qabs_s[t, pl.ds(b, H, stride=B), :] for t in range(Dc // 128)],
                axis=1).astype(BF16)
            def c_half(k):
                return ckv_v[pl.ds(b * CS + k * (CS // 2), CS // 2)].reshape(Sk // 2, Dc)

            s = []
            for k in range(2):
                s.append(jax.lax.dot_general(qa, c_half(k), _NT, preferred_element_type=F32))
                iss_a(b, k)
            s = jnp.concatenate(s, axis=1)
            m = jnp.max(s, axis=-1, keepdims=True)
            p = jnp.exp(s - m)
            l = jnp.sum(p, axis=-1, keepdims=True)
            p = p.astype(BF16)
            c = ckv_v[pl.ds(b * CS, CS)].reshape(Sk, Dc)
            lat = jnp.dot(p, c, preferred_element_type=F32)
            lat = lat / l
            row = pl.multiple_of(b * H, H)
            for t in range(Dc // 128):
                lat_s[t, pl.ds(row, H), :] = lat[:, t * 128:(t + 1) * 128]
            iss_a(b, 2)
            return carry

        jax.lax.fori_loop(0, B, attn_a, 0)

        iss_c = cur.loop(H // 2, cfg["n_ctx"])

        def ctx_body(j, carry):
            for p in range(2):
                lat = jnp.concatenate(
                    [lat_s[t, pl.ds(2 * j + p, B, stride=H), :] for t in range(Dc // 128)],
                    axis=1).astype(BF16)
                ctx_s[2 * j + p] = jnp.dot(lat, _head(t0_s, j, p, H, Dc),
                                           preferred_element_type=F32)
            iss_c(j, 0)
            return carry

        jax.lax.fori_loop(0, H // 2, ctx_body, 0)

        cur.to(cfg["u_attn_b"])
        for unit in range(B // UB):
            assert (cur.pos + unit * UB * sum(cfg["n_attn_b"]) + cfg["n_attn_b"][0]
                    >= u_kv + (unit + 1) * 2 * kv_bursts)
        iss_b = cur.loop(B, cfg["n_attn_b"])
        first = jax.lax.broadcasted_iota(jnp.int32, (2 * rep, 1), 0) < rep

        def attn_b(b, carry):
            iss_b(b, 0)
            unit, sub = _divmod_pow2(b, UB)

            @pl.when(sub == 0)
            def _():
                wait(kc_v.at[pl.ds(unit * NSTR, NSTR)], S_KV + 2 * unit)
                wait(vc_v.at[pl.ds(unit * NSTR, NSTR)], S_KV + 2 * unit + 1)

            for gp in range(HP):
                if gp == HP // 2:
                    iss_b(b, 1)
                a = b * HP + gp
                q = qb_s[pl.ds(gp * 2 * rep * B + b, 2 * rep, stride=B), :].astype(BF16)
                s0 = jax.lax.dot_general(q, kc_v[a, 0], _NT, preferred_element_type=F32)
                s1 = jax.lax.dot_general(q, kc_v[a, 1], _NT, preferred_element_type=F32)
                s = jnp.where(first, s0, s1) * scale
                m = jnp.max(s, axis=-1, keepdims=True)
                p = jnp.exp(s - m)
                l = jnp.sum(p, axis=-1, keepdims=True)
                p = p.astype(BF16)
                o0 = jnp.dot(p, vc_v[a, 0], preferred_element_type=F32)
                o1 = jnp.dot(p, vc_v[a, 1], preferred_element_type=F32)
                row = pl.multiple_of(a * 2 * rep, 2 * rep)
                ob_s[pl.ds(row, 2 * rep), :] = jnp.where(first, o0, o1) / l
            return carry

        jax.lax.fori_loop(0, B, attn_b, 0)

        def lhs(which, s0, ns, band):
            hs = [s * NBAND + band for s in range(s0, s0 + ns)]
            if which == 0:
                parts = [ctx_s[h] for h in hs]
            else:
                parts = [ob_s[pl.ds(h, B, stride=H), :] for h in hs]
            return jnp.concatenate(parts, axis=1).astype(BF16)

        def proj(l, which, s0, ns, band):
            w = (wo_v, bwo_v)[which][pl.ds(s0, ns), pl.ds(band * D, D), :].reshape(ns * D, M)
            return jnp.dot(l, w, preferred_element_type=F32)

        def do_band(which, band):
            wait((wo_v, bwo_v)[which].at[:, pl.ds(band * D, D)], S_W3 + 2 * band + which)
            r = proj(lhs(which, 0, NSTR, band), which, 0, NSTR, band)
            acc_s[which] = r if band == 0 else acc_s[which] + r

        last = NBAND - 1
        todo = [(which, band) for band in range(NBAND) for which in range(2)][:-1]
        for u, n in cfg["u_band"]:
            cur.to(u)
            for _ in range(n):
                which, band = todo.pop(0)
                assert band < last and (cur.pos - u_w3) * BURST >= (
                    (band + 1) * band_bursts * BURST + (skews[4] if which == 0 else 0))
                do_band(which, band)
        cur.to(n_bursts)

        starts = [sum(tail_blocks[:k]) for k in range(len(tail_blocks))]
        narrow = []
        for k, (s0, ns) in enumerate(zip(starts, tail_blocks)):
            rows = 32 // ns
            narrow += [((pl.ds(s0, ns), pl.ds(r, rows), every), S_TAIL + k)
                       for r in range(last * D, (last + 1) * D, rows)]
        assert len(narrow) == band_bursts * BURST

        def d_narrow(blk, i):
            sl, sem = narrow[(blk - last * band_bursts) * BURST + i]
            start(bwo_h.at[sl], bwo_v.at[sl], sem, 1)

        for u in range(last * band_bursts, w_bursts):
            burst(u, w_bursts, skews[4], d_wo, d_narrow)

        xf = x_v[...].astype(F32)
        gw = gw_v[...].astype(F32)
        t = xf[:, 0:128] * gw[0:1, :]
        for i in range(1, M // 128):
            t = t + xf[:, i * 128:(i + 1) * 128] * gw[i:i + 1, :]
        gate = jax.nn.sigmoid(jnp.sum(t, axis=-1, keepdims=True))

        for which, band in todo:
            do_band(which, band)
        tail_lhs = [lhs(1, s0, ns, last) for s0, ns in zip(starts, tail_blocks)]
        out = gate * acc_s[0]
        acc = acc_s[1]
        for k, (s0, ns) in enumerate(zip(starts, tail_blocks)):
            wait(bwo_v.at[pl.ds(s0, ns), pl.ds(last * D, D)], S_TAIL + k)
            acc = acc + proj(tail_lhs[k], 1, s0, ns, last)
        o_ref[...] = (out + (1.0 - gate) * acc).astype(o_ref.dtype)

    return kernel, n_sems


DEFAULT_CFG = dict(
    u_q=22, split_steps=8, n_split=(1,), u_uk=38, n_qabs=(1,),
    u_attn_a=80, n_attn_a=(2, 2, 2),
    n_ctx=(1,),
    u_attn_b=148, n_attn_b=(2, 1),
    u_band=((172, 2),),
    tail_blocks=(4, 2, 1, 1),
    skews=(124, 27, 26, 26, 0),
)
DEFAULT_PARAMS = dict(disable_bounds_checks=True, disable_semaphore_checks=True)


def _forward(A_x, A_c_kv, A_w_q, A_w_uk, A_w_uv, A_w_o, B_k_cache, B_v_cache, B_wq, B_wo,
             gate_w, cfg, params):
    B, Sq, M = A_x.shape
    assert Sq == 1
    _, Sk, Dc = A_c_kv.shape
    _, H, D = A_w_q.shape
    _, Hkv, SkB, _ = B_k_cache.shape
    W = min(4096, max(256, SkB // 4))
    HD = H * D

    kernel, n_sems = _make_kernel(B, M, H, D, Dc, Sk, Hkv, SkB, W, cfg)
    any_spec = pl.BlockSpec(memory_space=pl.ANY)
    out = pl.pallas_call(
        kernel,
        out_shape=jax.ShapeDtypeStruct((B, M), A_x.dtype),
        in_specs=[any_spec] * 11,
        out_specs=pl.BlockSpec(memory_space=pltpu.VMEM),
        scratch_shapes=[
            pltpu.VMEM((B, M), BF16),
            pltpu.VMEM((M // 128, 128), BF16),
            pltpu.VMEM((B * 4, Sk // 4, Dc), BF16),
            pltpu.VMEM((NSTR, M * H // NSTR, D), BF16),
            pltpu.VMEM((NSTR, Dc * H // NSTR, D), BF16),
            pltpu.VMEM((NSTR, Dc * H // NSTR, D), BF16),
            pltpu.VMEM((NSTR, HD // NSTR, M), BF16),
            pltpu.VMEM((B * Hkv // 2, 2, W, D), BF16),
            pltpu.VMEM((B * Hkv // 2, 2, W, D), BF16),
            pltpu.VMEM((NSTR, M // NSTR, HD), BF16),
            pltpu.VMEM((NSTR, HD // NSTR, M), BF16),
            pltpu.VMEM((H * PLANE, D), U32),
            pltpu.VMEM((H * PLANE, D), U32),
            pltpu.VMEM((Dc // 128, H * B, 128), F32),
            pltpu.VMEM((Dc // 128, B * H, 128), F32),
            pltpu.VMEM((H, B, D), F32),
            pltpu.VMEM((H * B, D), F32),
            pltpu.VMEM((B * H, D), F32),
            pltpu.VMEM((2, B, M), F32),
            pltpu.SemaphoreType.DMA((n_sems,)),
        ],
        compiler_params=pltpu.CompilerParams(vmem_limit_bytes=112 * 1024 * 1024, **params),
        name="gated_mix_decode",
    )(
        A_x.reshape(B, M),
        gate_w.reshape(M // 128, 128),
        A_c_kv.reshape(B * 4, Sk // 4, Dc),
        A_w_q.reshape(NSTR, M * H // NSTR, D),
        A_w_uk.reshape(NSTR, Dc * H // NSTR, D),
        A_w_uv.reshape(NSTR, Dc * H // NSTR, D),
        A_w_o.reshape(NSTR, HD // NSTR, M),
        B_k_cache.reshape(B * Hkv // 2, 2, SkB, D),
        B_v_cache.reshape(B * Hkv // 2, 2, SkB, D),
        B_wq.reshape(NSTR, M // NSTR, HD),
        B_wo.reshape(NSTR, HD // NSTR, M),
    )
    return out.reshape(B, 1, M)


@jax.jit
def pallas_gated_mix__compressed_kv_cla__sliding_block_cached__decode_kernel(
    A_x: jax.Array,
    A_c_kv: jax.Array,
    A_w_q: jax.Array,
    A_w_uk: jax.Array,
    A_w_uv: jax.Array,
    A_w_o: jax.Array,
    B_x: jax.Array,
    B_k_cache: jax.Array,
    B_v_cache: jax.Array,
    B_wq: jax.Array,
    B_wo: jax.Array,
    gate_w: jax.Array,
):
    return _forward(A_x, A_c_kv, A_w_q, A_w_uk, A_w_uv, A_w_o, B_k_cache, B_v_cache,
                    B_wq, B_wo, gate_w, DEFAULT_CFG, DEFAULT_PARAMS)
```

```python
import jax
import jax.numpy as jnp
import jax.experimental.pallas as pl
import jax.experimental.pallas.tpu as pltpu

F32 = jnp.float32
BF16 = jnp.bfloat16
U32 = jnp.uint32

_NT = (((1,), (1,)), ((), ()))

NSTR = 8
BURST = 8
PLANE = 264


def _divmod_pow2(u, n):
    assert n & (n - 1) == 0
    return u >> (n.bit_length() - 1), u & (n - 1)


def _mult(v, n):
    return v if isinstance(v, int) else pl.multiple_of(v, n)


def _split_heads(w_v, t_s, step, nsteps, heads):
    ns, rr, _ = w_v.shape
    per_stream = nsteps // ns
    stream, part = _divmod_pow2(step, per_stream)
    rows = rr // per_stream
    half = heads // 2
    for k in range(rows // (2 * heads)):
        r0 = pl.multiple_of(part * rows + k * 2 * heads, 2 * heads)
        w = pltpu.bitcast(w_v[stream, pl.ds(r0, 2 * heads), :], U32)
        ev, od = w[:half], w[half:]
        lo = (ev & jnp.uint32(0xFFFF)) | (od << 16)
        hi = (ev >> 16) | (od & jnp.uint32(0xFFFF0000))
        i = step * (rows // (2 * heads)) + k
        t_s[pl.ds(i, half, stride=PLANE), :] = lo
        t_s[pl.ds(half * PLANE + i, half, stride=PLANE), :] = hi


def _head(t_s, j, p, heads, rows):
    r0 = pl.multiple_of((p * (heads // 2) + j) * PLANE, 8)
    return pltpu.bitcast(t_s[pl.ds(r0, rows // 2), :], BF16)


def _make_kernel(B, M, H, D, Dc, Sk, Hkv, SkB, W, cfg):
    rep = H // Hkv
    scale = float(D) ** -0.5
    HD = H * D
    CS = 4
    CR = Sk // CS
    OR = HD // NSTR
    NBAND = OR // D
    HP = Hkv // 2
    UB = NSTR // HP
    tail_blocks = cfg["tail_blocks"]
    skews = cfg["skews"]
    assert skews[4] <= D // 4
    assert sum(tail_blocks) == NSTR and max(M, Dc) // 2 <= PLANE

    S_X, S_GW, S_WQ, S_WUK, S_BWQ, S_WUV, S_CKV = 0, 1, 2, 3, 4, 5, 6
    S_KV = S_CKV + 2
    S_W3 = S_KV + 2 * (B // UB)
    S_TAIL = S_W3 + 2 * NBAND - 1
    n_sems = S_TAIL + len(tail_blocks)

    def kernel(x_h, gw_h, ckv_h, wq_h, wuk_h, wuv_h, wo_h, kc_h, vc_h, bwq_h, bwo_h,
               o_ref,
               x_v, gw_v, ckv_v, wq_v, wuk_v, wuv_v, wo_v, kc_v, vc_v, bwq_v, bwo_v,
               t0_s, t1_s, qabs_s, lat_s, ctx_s, qb_s, ob_s, acc_s, sems):
        def start(src, dst, sem, prio):
            pltpu.make_async_copy(src, dst, sems.at[sem]).start(priority=prio)

        def wait(buf, sem):
            pltpu.make_async_copy(buf, buf, sems.at[sem]).wait()

        every = slice(None)

        def rows16(src, dst, r, sem, prio):
            sl = (every, pl.ds(_mult(r, 16), 16), every)
            start(src.at[sl], dst.at[sl], sem, prio)

        def tiles2(src, dst, lead, r, c, sem, prio):
            sl = (lead, pl.ds(_mult(r, 8), 8), pl.ds(_mult(c, 256), 256))
            start(src.at[sl], dst.at[sl], sem, prio)

        def burst(u, nblk, skew, d0, d1):
            q, r = divmod(skew, BURST)
            blk0 = [(u - q - 1) & (nblk - 1), (u - q) & (nblk - 1)]
            for i in range(BURST):
                d0(blk0[i >= r], (i - r) % BURST)
                d1(u, i)

        def d_rows(src, dst, sem, prio):
            return lambda blk, i: rows16(src, dst, blk * (16 * BURST) + 16 * i, sem, prio)

        def d_tiles(src, dst, lead, sem, prio):
            nc = src.shape[-1] // 256

            def f(blk, i):
                if nc >= BURST:
                    rb, cb = _divmod_pow2(blk, nc // BURST)
                    r, c = rb * 8, cb * (256 * BURST) + 256 * i
                else:
                    r, c = blk * (8 * BURST // nc) + 8 * (i // nc), 256 * (i % nc)
                tiles2(src, dst, lead, r, c, sem(blk) if callable(sem) else sem, prio)
            return f

        w_bursts = wq_v.shape[1] // 16 // BURST

        def burst_w1(u):
            burst(u, w_bursts, skews[0], d_rows(wq_h, wq_v, S_WQ, 0),
                  d_tiles(bwq_h, bwq_v, every, S_BWQ, 1))

        def burst_w2(u):
            burst(u, w_bursts, skews[1], d_rows(wuk_h, wuk_v, S_WUK, 0),
                  d_rows(wuv_h, wuv_v, S_WUV, 1))

        ckv_bursts = (CR // 8) * (Dc // 256) // BURST

        def burst_ckv(u):
            half, uu = _divmod_pow2(u, ckv_bursts)
            d = [d_tiles(ckv_h, ckv_v, pl.ds(half * (2 * NSTR) + t * NSTR, NSTR), S_CKV + half, t)
                 for t in range(2)]
            burst(uu, ckv_bursts, skews[2], *d)

        kv_bursts = W // 16 // BURST

        def burst_kv(u):
            q, uu = _divmod_pow2(u, kv_bursts)
            unit, which = _divmod_pow2(q, 2)
            lead = pl.ds(unit * NSTR, NSTR)

            def go(src, dst):
                def d(t):
                    def f(blk, i):
                        r = blk * (16 * BURST) + 16 * i
                        start(src.at[lead, t, pl.ds(_mult(SkB - W + r, 16), 16)],
                              dst.at[lead, t, pl.ds(_mult(r, 16), 16)], S_KV + q, t)
                    return f
                burst(uu, kv_bursts, skews[3], d(0), d(1))

            pl.when(which == 0)(lambda: go(kc_h, kc_v))
            pl.when(which == 1)(lambda: go(vc_h, vc_v))

        band_bursts = w_bursts // NBAND
        d_wo = d_tiles(wo_h, wo_v, every,
                       lambda blk: S_W3 + 2 * _divmod_pow2(blk, band_bursts)[0], 0)
        d_bwo = d_tiles(bwo_h, bwo_v, every,
                        lambda blk: S_W3 + 2 * _divmod_pow2(blk, band_bursts)[0] + 1, 1)

        def burst_w3(u):
            burst(u, w_bursts, skews[4], d_wo, d_bwo)

        plan = []
        u0 = 0
        for fn, n in ((burst_w1, w_bursts),
                      (burst_w2, w_bursts),
                      (burst_ckv, 2 * ckv_bursts),
                      (burst_kv, B * kv_bursts),
                      (burst_w3, (NBAND - 1) * band_bursts)):
            plan.append((u0, n, fn))
            u0 += n
        n_bursts = u0
        u_w2, u_ckv, u_kv, u_w3 = (p[0] for p in plan[1:])

        def issue(first, count, lo, hi):
            hits = [(u0, n, fn) for u0, n, fn in plan if u0 < hi and lo < u0 + n]

            def one(u):
                for u0, n, fn in hits:
                    if len(hits) == 1:
                        fn(u - u0)
                    else:
                        pl.when(jnp.logical_and(u >= u0, u < u0 + n))(lambda: fn(u - u0))

            if count == 1:
                one(first)
            else:
                def body(i, c):
                    one(first + i)
                    return c
                jax.lax.fori_loop(0, count, body, 0)

        class Cursor:
            pos = 0

            def to(self, hi):
                assert self.pos <= hi <= n_bursts, (self.pos, hi)
                for u0, n, _ in plan:
                    a, b = max(self.pos, u0), min(hi, u0 + n)
                    if a < b:
                        issue(a, b - a, a, b)
                self.pos = hi

            def loop(self, iters, counts):
                per = sum(counts)
                lo, hi = self.pos, self.pos + iters * per
                assert hi <= n_bursts
                self.pos = hi

                def f(i, k):
                    if counts[k]:
                        issue(lo + i * per + sum(counts[:k]), counts[k], lo, hi)
                return f

        cur = Cursor()

        def split_loop(w_v, t_s):
            n = cfg["split_steps"]
            iss = cur.loop(n, cfg["n_split"])

            def body(i, carry):
                iss(i, 0)
                _split_heads(w_v, t_s, i, n, H)
                return carry

            jax.lax.fori_loop(0, n, body, 0)

        cur.to(1)
        start(x_h, x_v, S_X, 0)
        start(gw_h, gw_v, S_GW, 1)
        cur.to(cfg["u_q"])

        assert cur.pos >= u_w2
        wait(x_v, S_X)
        wait(gw_v, S_GW)
        wait(wq_v, S_WQ)
        wait(bwq_v, S_BWQ)
        qb = jnp.dot(x_v[...], bwq_v[...].reshape(M, HD), preferred_element_type=F32)
        qb = qb.astype(BF16).astype(F32)
        for h in range(H):
            qb_s[h * B:(h + 1) * B, :] = qb[:, h * D:(h + 1) * D]

        split_loop(wq_v, t0_s)
        cur.to(cfg["u_uk"])
        assert cur.pos >= u_ckv
        wait(wuk_v, S_WUK)
        wait(wuv_v, S_WUV)
        split_loop(wuk_v, t1_s)
        iss_q = cur.loop(H // 2, cfg["n_qabs"])

        def qabs_body(j, carry):
            x = x_v[...]
            for p in range(2):
                q = jnp.dot(x, _head(t0_s, j, p, H, M),
                            preferred_element_type=F32).astype(BF16)
                qa = jax.lax.dot_general(q, _head(t1_s, j, p, H, Dc), _NT,
                                         preferred_element_type=F32) * scale
                row = pl.multiple_of((2 * j + p) * B, B)
                for t in range(Dc // 128):
                    qabs_s[t, pl.ds(row, B), :] = qa[:, t * 128:(t + 1) * 128]
            iss_q(j, 0)
            return carry

        jax.lax.fori_loop(0, H // 2, qabs_body, 0)
        split_loop(wuv_v, t0_s)

        cur.to(cfg["u_attn_a"])
        for half in range(2):
            assert cur.pos + half * (B // 2) * sum(cfg["n_attn_a"]) >= u_ckv + (half + 1) * ckv_bursts
        iss_a = cur.loop(B, cfg["n_attn_a"])

        def attn_a(b, carry):
            for half in range(2):
                pl.when(b == half * (B // 2))(
                    lambda: wait(ckv_v.at[pl.ds(half * 2 * NSTR, 2 * NSTR)], S_CKV + half))

            qa = jnp.concatenate(
                [qabs_s[t, pl.ds(b, H, stride=B), :] for t in range(Dc // 128)],
                axis=1).astype(BF16)
            def c_half(k):
                return ckv_v[pl.ds(b * CS + k * (CS // 2), CS // 2)].reshape(Sk // 2, Dc)

            s = []
            for k in range(2):
                s.append(jax.lax.dot_general(qa, c_half(k), _NT, preferred_element_type=F32))
                iss_a(b, k)
            s = jnp.concatenate(s, axis=1)
            m = jnp.max(s, axis=-1, keepdims=True)
            p = jnp.exp(s - m)
            l = jnp.sum(p, axis=-1, keepdims=True)
            p = p.astype(BF16)
            c = ckv_v[pl.ds(b * CS, CS)].reshape(Sk, Dc)
            lat = jnp.dot(p, c, preferred_element_type=F32)
            lat = lat / l
            row = pl.multiple_of(b * H, H)
            for t in range(Dc // 128):
                lat_s[t, pl.ds(row, H), :] = lat[:, t * 128:(t + 1) * 128]
            iss_a(b, 2)
            return carry

        jax.lax.fori_loop(0, B, attn_a, 0)

        iss_c = cur.loop(H // 2, cfg["n_ctx"])

        def ctx_body(j, carry):
            for p in range(2):
                lat = jnp.concatenate(
                    [lat_s[t, pl.ds(2 * j + p, B, stride=H), :] for t in range(Dc // 128)],
                    axis=1).astype(BF16)
                ctx_s[2 * j + p] = jnp.dot(lat, _head(t0_s, j, p, H, Dc),
                                           preferred_element_type=F32)
            iss_c(j, 0)
            return carry

        jax.lax.fori_loop(0, H // 2, ctx_body, 0)

        cur.to(cfg["u_attn_b"])
        for unit in range(B // UB):
            assert (cur.pos + unit * UB * sum(cfg["n_attn_b"]) + cfg["n_attn_b"][0]
                    >= u_kv + (unit + 1) * 2 * kv_bursts)
        iss_b = cur.loop(B, cfg["n_attn_b"])
        first = jax.lax.broadcasted_iota(jnp.int32, (2 * rep, 1), 0) < rep

        def attn_b(b, carry):
            iss_b(b, 0)
            unit, sub = _divmod_pow2(b, UB)

            @pl.when(sub == 0)
            def _():
                wait(kc_v.at[pl.ds(unit * NSTR, NSTR)], S_KV + 2 * unit)
                wait(vc_v.at[pl.ds(unit * NSTR, NSTR)], S_KV + 2 * unit + 1)

            for gp in range(HP):
                if gp == HP // 2:
                    iss_b(b, 1)
                a = b * HP + gp
                q = qb_s[pl.ds(gp * 2 * rep * B + b, 2 * rep, stride=B), :].astype(BF16)
                s0 = jax.lax.dot_general(q, kc_v[a, 0], _NT, preferred_element_type=F32)
                s1 = jax.lax.dot_general(q, kc_v[a, 1], _NT, preferred_element_type=F32)
                s = jnp.where(first, s0, s1) * scale
                m = jnp.max(s, axis=-1, keepdims=True)
                p = jnp.exp(s - m)
                l = jnp.sum(p, axis=-1, keepdims=True)
                p = p.astype(BF16)
                o0 = jnp.dot(p, vc_v[a, 0], preferred_element_type=F32)
                o1 = jnp.dot(p, vc_v[a, 1], preferred_element_type=F32)
                row = pl.multiple_of(a * 2 * rep, 2 * rep)
                ob_s[pl.ds(row, 2 * rep), :] = jnp.where(first, o0, o1) / l
            return carry

        jax.lax.fori_loop(0, B, attn_b, 0)

        def lhs(which, s0, ns, band):
            hs = [s * NBAND + band for s in range(s0, s0 + ns)]
            if which == 0:
                parts = [ctx_s[h] for h in hs]
            else:
                parts = [ob_s[pl.ds(h, B, stride=H), :] for h in hs]
            return jnp.concatenate(parts, axis=1).astype(BF16)

        def proj(l, which, s0, ns, band):
            w = (wo_v, bwo_v)[which][pl.ds(s0, ns), pl.ds(band * D, D), :].reshape(ns * D, M)
            return jnp.dot(l, w, preferred_element_type=F32)

        def do_band(which, band):
            wait((wo_v, bwo_v)[which].at[:, pl.ds(band * D, D)], S_W3 + 2 * band + which)
            r = proj(lhs(which, 0, NSTR, band), which, 0, NSTR, band)
            acc_s[which] = r if band == 0 else acc_s[which] + r

        last = NBAND - 1
        todo = [(which, band) for band in range(NBAND) for which in range(2)][:-1]
        for u, n in cfg["u_band"]:
            cur.to(u)
            for _ in range(n):
                which, band = todo.pop(0)
                assert band < last and (cur.pos - u_w3) * BURST >= (
                    (band + 1) * band_bursts * BURST + (skews[4] if which == 0 else 0))
                do_band(which, band)
        cur.to(n_bursts)

        starts = [sum(tail_blocks[:k]) for k in range(len(tail_blocks))]
        narrow = []
        for k, (s0, ns) in enumerate(zip(starts, tail_blocks)):
            rows = 32 // ns
            narrow += [((pl.ds(s0, ns), pl.ds(r, rows), every), S_TAIL + k)
                       for r in range(last * D, (last + 1) * D, rows)]
        assert len(narrow) == band_bursts * BURST

        def d_narrow(blk, i):
            sl, sem = narrow[(blk - last * band_bursts) * BURST + i]
            start(bwo_h.at[sl], bwo_v.at[sl], sem, 1)

        for u in range(last * band_bursts, w_bursts):
            burst(u, w_bursts, skews[4], d_wo, d_narrow)

        xf = x_v[...].astype(F32)
        gw = gw_v[...].astype(F32)
        t = xf[:, 0:128] * gw[0:1, :]
        for i in range(1, M // 128):
            t = t + xf[:, i * 128:(i + 1) * 128] * gw[i:i + 1, :]
        gate = jax.nn.sigmoid(jnp.sum(t, axis=-1, keepdims=True))

        for which, band in todo:
            do_band(which, band)
        tail_lhs = [lhs(1, s0, ns, last) for s0, ns in zip(starts, tail_blocks)]
        out = gate * acc_s[0]
        acc = acc_s[1]
        for k, (s0, ns) in enumerate(zip(starts, tail_blocks)):
            wait(bwo_v.at[pl.ds(s0, ns), pl.ds(last * D, D)], S_TAIL + k)
            acc = acc + proj(tail_lhs[k], 1, s0, ns, last)
        o_ref[...] = (out + (1.0 - gate) * acc).astype(o_ref.dtype)

    return kernel, n_sems


DEFAULT_CFG = dict(
    u_q=22, split_steps=8, n_split=(1,), u_uk=38, n_qabs=(1,),
    u_attn_a=80, n_attn_a=(2, 2, 2),
    n_ctx=(1,),
    u_attn_b=148, n_attn_b=(2, 1),
    u_band=((172, 2),),
    tail_blocks=(4, 2, 1, 1),
    skews=(124, 27, 26, 26, 0),
)
DEFAULT_PARAMS = dict(disable_bounds_checks=True, disable_semaphore_checks=True)


def _compiler_params(params):
    vmem = 112 * 1024 * 1024
    try:
        return pltpu.CompilerParams(vmem_limit_bytes=vmem, **params)
    except TypeError:
        params = {k: v for k, v in params.items() if k != "disable_semaphore_checks"}
        return pltpu.CompilerParams(vmem_limit_bytes=vmem, **params)


def _forward(A_x, A_c_kv, A_w_q, A_w_uk, A_w_uv, A_w_o, B_k_cache, B_v_cache, B_wq, B_wo,
             gate_w, cfg, params):
    B, Sq, M = A_x.shape
    assert Sq == 1
    _, Sk, Dc = A_c_kv.shape
    _, H, D = A_w_q.shape
    _, Hkv, SkB, _ = B_k_cache.shape
    W = min(4096, max(256, SkB // 4))
    HD = H * D

    kernel, n_sems = _make_kernel(B, M, H, D, Dc, Sk, Hkv, SkB, W, cfg)
    any_spec = pl.BlockSpec(memory_space=pl.ANY)
    out = pl.pallas_call(
        kernel,
        out_shape=jax.ShapeDtypeStruct((B, M), A_x.dtype),
        in_specs=[any_spec] * 11,
        out_specs=pl.BlockSpec(memory_space=pltpu.VMEM),
        scratch_shapes=[
            pltpu.VMEM((B, M), BF16),
            pltpu.VMEM((M // 128, 128), BF16),
            pltpu.VMEM((B * 4, Sk // 4, Dc), BF16),
            pltpu.VMEM((NSTR, M * H // NSTR, D), BF16),
            pltpu.VMEM((NSTR, Dc * H // NSTR, D), BF16),
            pltpu.VMEM((NSTR, Dc * H // NSTR, D), BF16),
            pltpu.VMEM((NSTR, HD // NSTR, M), BF16),
            pltpu.VMEM((B * Hkv // 2, 2, W, D), BF16),
            pltpu.VMEM((B * Hkv // 2, 2, W, D), BF16),
            pltpu.VMEM((NSTR, M // NSTR, HD), BF16),
            pltpu.VMEM((NSTR, HD // NSTR, M), BF16),
            pltpu.VMEM(((H + 1) * PLANE, D), U32),
            pltpu.VMEM(((H + 1) * PLANE, D), U32),
            pltpu.VMEM((Dc // 128, (H + 1) * B, 128), F32),
            pltpu.VMEM((Dc // 128, (B + 1) * H, 128), F32),
            pltpu.VMEM((H, B, D), F32),
            pltpu.VMEM(((H + 1) * B, D), F32),
            pltpu.VMEM(((B + 1) * H, D), F32),
            pltpu.VMEM((2, B, M), F32),
            pltpu.SemaphoreType.DMA((n_sems,)),
        ],
        compiler_params=_compiler_params(params),
        name="gated_mix_decode",
    )(
        A_x.reshape(B, M),
        gate_w.reshape(M // 128, 128),
        A_c_kv.reshape(B * 4, Sk // 4, Dc),
        A_w_q.reshape(NSTR, M * H // NSTR, D),
        A_w_uk.reshape(NSTR, Dc * H // NSTR, D),
        A_w_uv.reshape(NSTR, Dc * H // NSTR, D),
        A_w_o.reshape(NSTR, HD // NSTR, M),
        B_k_cache.reshape(B * Hkv // 2, 2, SkB, D),
        B_v_cache.reshape(B * Hkv // 2, 2, SkB, D),
        B_wq.reshape(NSTR, M // NSTR, HD),
        B_wo.reshape(NSTR, HD // NSTR, M),
    )
    return out.reshape(B, 1, M)


@jax.jit
def pallas_gated_mix__compressed_kv_cla__sliding_block_cached__decode_kernel(
    A_x: jax.Array,
    A_c_kv: jax.Array,
    A_w_q: jax.Array,
    A_w_uk: jax.Array,
    A_w_uv: jax.Array,
    A_w_o: jax.Array,
    B_x: jax.Array,
    B_k_cache: jax.Array,
    B_v_cache: jax.Array,
    B_wq: jax.Array,
    B_wo: jax.Array,
    gate_w: jax.Array,
):
    return _forward(A_x, A_c_kv, A_w_q, A_w_uk, A_w_uv, A_w_o, B_k_cache, B_v_cache,
                    B_wq, B_wo, gate_w, DEFAULT_CFG, DEFAULT_PARAMS)
```

```python
import jax
import jax.numpy as jnp
import jax.experimental.pallas as pl
import jax.experimental.pallas.tpu as pltpu

F32 = jnp.float32
BF16 = jnp.bfloat16
U32 = jnp.uint32

_NT = (((1,), (1,)), ((), ()))

NSTR = 8
BURST = 8
PLANE = 264


def _divmod_pow2(u, n):
    assert n & (n - 1) == 0
    return u >> (n.bit_length() - 1), u & (n - 1)


def _mult(v, n):
    return v if isinstance(v, int) else pl.multiple_of(v, n)


def _split_heads(w_v, t_s, step, nsteps, heads):
    ns, rr, _ = w_v.shape
    per_stream = nsteps // ns
    stream, part = _divmod_pow2(step, per_stream)
    rows = rr // per_stream
    half = heads // 2
    for k in range(rows // (2 * heads)):
        r0 = pl.multiple_of(part * rows + k * 2 * heads, 2 * heads)
        w = pltpu.bitcast(w_v[stream, pl.ds(r0, 2 * heads), :], U32)
        ev, od = w[:half], w[half:]
        lo = (ev & jnp.uint32(0xFFFF)) | (od << 16)
        hi = (ev >> 16) | (od & jnp.uint32(0xFFFF0000))
        i = step * (rows // (2 * heads)) + k
        t_s[pl.ds(i, half, stride=PLANE), :] = lo
        t_s[pl.ds(half * PLANE + i, half, stride=PLANE), :] = hi


def _head(t_s, j, p, heads, rows):
    r0 = pl.multiple_of((p * (heads // 2) + j) * PLANE, 8)
    return pltpu.bitcast(t_s[pl.ds(r0, rows // 2), :], BF16)


def _make_kernel(B, M, H, D, Dc, Sk, Hkv, SkB, W, cfg):
    rep = H // Hkv
    scale = float(D) ** -0.5
    HD = H * D
    CS = 4
    CR = Sk // CS
    OR = HD // NSTR
    NBAND = OR // D
    HP = Hkv // 2
    UB = NSTR // HP
    tail_blocks = cfg["tail_blocks"]
    skews = cfg["skews"]
    assert skews[4] <= D // 4
    assert sum(tail_blocks) == NSTR and max(M, Dc) // 2 <= PLANE

    S_X, S_GW, S_WQ, S_WUK, S_BWQ, S_WUV, S_CKV = 0, 1, 2, 3, 4, 5, 6
    S_KV = S_CKV + 2
    S_W3 = S_KV + 2 * (B // UB)
    S_TAIL = S_W3 + 2 * NBAND - 1
    n_sems = S_TAIL + len(tail_blocks)

    def kernel(x_h, gw_h, ckv_h, wq_h, wuk_h, wuv_h, wo_h, kc_h, vc_h, bwq_h, bwo_h,
               o_ref,
               x_v, gw_v, ckv_v, wq_v, wuk_v, wuv_v, wo_v, kc_v, vc_v, bwq_v, bwo_v,
               t0_s, t1_s, qabs_s, lat_s, ctx_s, qb_s, ob_s, acc_s, sems):
        def start(src, dst, sem, prio):
            pltpu.make_async_copy(src, dst, sems.at[sem]).start(priority=prio)

        def wait(buf, sem):
            pltpu.make_async_copy(buf, buf, sems.at[sem]).wait()

        every = slice(None)

        def rows16(src, dst, r, sem, prio):
            sl = (every, pl.ds(_mult(r, 16), 16), every)
            start(src.at[sl], dst.at[sl], sem, prio)

        def tiles2(src, dst, lead, r, c, sem, prio):
            sl = (lead, pl.ds(_mult(r, 8), 8), pl.ds(_mult(c, 256), 256))
            start(src.at[sl], dst.at[sl], sem, prio)

        def burst(u, nblk, skew, d0, d1):
            q, r = divmod(skew, BURST)
            blk0 = [(u - q - 1) & (nblk - 1), (u - q) & (nblk - 1)]
            for i in range(BURST):
                d0(blk0[i >= r], (i - r) % BURST)
                d1(u, i)

        def d_rows(src, dst, sem, prio):
            return lambda blk, i: rows16(src, dst, blk * (16 * BURST) + 16 * i, sem, prio)

        def d_tiles(src, dst, lead, sem, prio):
            nc = src.shape[-1] // 256

            def f(blk, i):
                if nc >= BURST:
                    rb, cb = _divmod_pow2(blk, nc // BURST)
                    r, c = rb * 8, cb * (256 * BURST) + 256 * i
                else:
                    r, c = blk * (8 * BURST // nc) + 8 * (i // nc), 256 * (i % nc)
                tiles2(src, dst, lead, r, c, sem(blk) if callable(sem) else sem, prio)
            return f

        w_bursts = wq_v.shape[1] // 16 // BURST

        def burst_w1(u):
            burst(u, w_bursts, skews[0], d_rows(wq_h, wq_v, S_WQ, 0),
                  d_tiles(bwq_h, bwq_v, every, S_BWQ, 1))

        def burst_w2(u):
            burst(u, w_bursts, skews[1], d_rows(wuk_h, wuk_v, S_WUK, 0),
                  d_rows(wuv_h, wuv_v, S_WUV, 1))

        ckv_bursts = (CR // 8) * (Dc // 256) // BURST

        def burst_ckv(u):
            half, uu = _divmod_pow2(u, ckv_bursts)
            d = [d_tiles(ckv_h, ckv_v, pl.ds(half * (2 * NSTR) + t * NSTR, NSTR), S_CKV + half, t)
                 for t in range(2)]
            burst(uu, ckv_bursts, skews[2], *d)

        kv_bursts = W // 16 // BURST

        def burst_kv(u):
            q, uu = _divmod_pow2(u, kv_bursts)
            unit, which = _divmod_pow2(q, 2)
            lead = pl.ds(unit * NSTR, NSTR)

            def go(src, dst):
                def d(t):
                    def f(blk, i):
                        r = blk * (16 * BURST) + 16 * i
                        start(src.at[lead, t, pl.ds(_mult(SkB - W + r, 16), 16)],
                              dst.at[lead, t, pl.ds(_mult(r, 16), 16)], S_KV + q, t)
                    return f
                burst(uu, kv_bursts, skews[3], d(0), d(1))

            pl.when(which == 0)(lambda: go(kc_h, kc_v))
            pl.when(which == 1)(lambda: go(vc_h, vc_v))

        band_bursts = w_bursts // NBAND
        d_wo = d_tiles(wo_h, wo_v, every,
                       lambda blk: S_W3 + 2 * _divmod_pow2(blk, band_bursts)[0], 0)
        d_bwo = d_tiles(bwo_h, bwo_v, every,
                        lambda blk: S_W3 + 2 * _divmod_pow2(blk, band_bursts)[0] + 1, 1)

        def burst_w3(u):
            burst(u, w_bursts, skews[4], d_wo, d_bwo)

        plan = []
        u0 = 0
        for fn, n in ((burst_w1, w_bursts),
                      (burst_w2, w_bursts),
                      (burst_ckv, 2 * ckv_bursts),
                      (burst_kv, B * kv_bursts),
                      (burst_w3, (NBAND - 1) * band_bursts)):
            plan.append((u0, n, fn))
            u0 += n
        n_bursts = u0
        u_w2, u_ckv, u_kv, u_w3 = (p[0] for p in plan[1:])

        def issue(first, count, lo, hi):
            hits = [(u0, n, fn) for u0, n, fn in plan if u0 < hi and lo < u0 + n]

            def one(u):
                for u0, n, fn in hits:
                    if len(hits) == 1:
                        fn(u - u0)
                    else:
                        pl.when(jnp.logical_and(u >= u0, u < u0 + n))(lambda: fn(u - u0))

            if count == 1:
                one(first)
            else:
                def body(i, c):
                    one(first + i)
                    return c
                jax.lax.fori_loop(0, count, body, 0)

        class Cursor:
            pos = 0

            def to(self, hi):
                assert self.pos <= hi <= n_bursts, (self.pos, hi)
                for u0, n, _ in plan:
                    a, b = max(self.pos, u0), min(hi, u0 + n)
                    if a < b:
                        issue(a, b - a, a, b)
                self.pos = hi

            def loop(self, iters, counts):
                per = sum(counts)
                lo, hi = self.pos, self.pos + iters * per
                assert hi <= n_bursts
                self.pos = hi

                def f(i, k):
                    if counts[k]:
                        issue(lo + i * per + sum(counts[:k]), counts[k], lo, hi)
                return f

        cur = Cursor()

        def split_loop(w_v, t_s):
            n = cfg["split_steps"]
            iss = cur.loop(n, cfg["n_split"])

            def body(i, carry):
                iss(i, 0)
                _split_heads(w_v, t_s, i, n, H)
                return carry

            jax.lax.fori_loop(0, n, body, 0)

        if cfg["head"]:
            head, rot = cfg["head"]
            n = w_bursts * BURST

            def wq_piece(j, prio):
                rows16(wq_h, wq_v, ((j + rot) & (n - 1)) * 16, S_WQ, prio)

            def bwq_piece(j):
                rb, cb = _divmod_pow2(j, HD // 256)
                tiles2(bwq_h, bwq_v, every, rb * 8, cb * 256, S_BWQ, 1)

            def sloop(cnt, f):
                def body(j, c):
                    f(j)
                    return c
                jax.lax.fori_loop(0, cnt, body, 0)

            for j in range(head):
                bwq_piece(j)
            sloop(n - head, lambda j: (wq_piece(j, 0), bwq_piece(j + head)))
            sloop(head // 2, lambda j: (wq_piece(n - head + j, 0), wq_piece(n - head // 2 + j, 1)))
            cur.pos = w_bursts
        else:
            cur.to(1)
        start(x_h, x_v, S_X, 0)
        start(gw_h, gw_v, S_GW, 1)
        cur.to(cfg["u_q"])

        assert cur.pos >= u_w2
        wait(x_v, S_X)
        wait(gw_v, S_GW)
        wait(wq_v, S_WQ)
        wait(bwq_v, S_BWQ)
        qb = jnp.dot(x_v[...], bwq_v[...].reshape(M, HD), preferred_element_type=F32)
        qb = qb.astype(BF16).astype(F32)
        for h in range(H):
            qb_s[h * B:(h + 1) * B, :] = qb[:, h * D:(h + 1) * D]

        split_loop(wq_v, t0_s)
        cur.to(cfg["u_uk"])
        assert cur.pos >= u_ckv
        wait(wuk_v, S_WUK)
        wait(wuv_v, S_WUV)
        split_loop(wuk_v, t1_s)
        iss_q = cur.loop(H // 2, cfg["n_qabs"])

        def qabs_body(j, carry):
            x = x_v[...]
            for p in range(2):
                q = jnp.dot(x, _head(t0_s, j, p, H, M),
                            preferred_element_type=F32).astype(BF16)
                qa = jax.lax.dot_general(q, _head(t1_s, j, p, H, Dc), _NT,
                                         preferred_element_type=F32) * scale
                row = pl.multiple_of((2 * j + p) * B, B)
                for t in range(Dc // 128):
                    qabs_s[t, pl.ds(row, B), :] = qa[:, t * 128:(t + 1) * 128]
            iss_q(j, 0)
            return carry

        jax.lax.fori_loop(0, H // 2, qabs_body, 0)
        split_loop(wuv_v, t0_s)

        cur.to(cfg["u_attn_a"])
        for half in range(2):
            assert cur.pos + half * (B // 2) * sum(cfg["n_attn_a"]) >= u_ckv + (half + 1) * ckv_bursts
        iss_a = cur.loop(B, cfg["n_attn_a"])

        def attn_a(b, carry):
            for half in range(2):
                pl.when(b == half * (B // 2))(
                    lambda: wait(ckv_v.at[pl.ds(half * 2 * NSTR, 2 * NSTR)], S_CKV + half))

            qa = jnp.concatenate(
                [qabs_s[t, pl.ds(b, H, stride=B), :] for t in range(Dc // 128)],
                axis=1).astype(BF16)
            def c_half(k):
                return ckv_v[pl.ds(b * CS + k * (CS // 2), CS // 2)].reshape(Sk // 2, Dc)

            s = []
            for k in range(2):
                s.append(jax.lax.dot_general(qa, c_half(k), _NT, preferred_element_type=F32))
                iss_a(b, k)
            s = jnp.concatenate(s, axis=1)
            m = jnp.max(s, axis=-1, keepdims=True)
            p = jnp.exp(s - m)
            l = jnp.sum(p, axis=-1, keepdims=True)
            p = p.astype(BF16)
            c = ckv_v[pl.ds(b * CS, CS)].reshape(Sk, Dc)
            lat = jnp.dot(p, c, preferred_element_type=F32)
            lat = lat / l
            row = pl.multiple_of(b * H, H)
            for t in range(Dc // 128):
                lat_s[t, pl.ds(row, H), :] = lat[:, t * 128:(t + 1) * 128]
            iss_a(b, 2)
            return carry

        jax.lax.fori_loop(0, B, attn_a, 0)

        iss_c = cur.loop(H // 2, cfg["n_ctx"])

        def ctx_body(j, carry):
            for p in range(2):
                lat = jnp.concatenate(
                    [lat_s[t, pl.ds(2 * j + p, B, stride=H), :] for t in range(Dc // 128)],
                    axis=1).astype(BF16)
                ctx_s[2 * j + p] = jnp.dot(lat, _head(t0_s, j, p, H, Dc),
                                           preferred_element_type=F32)
            iss_c(j, 0)
            return carry

        jax.lax.fori_loop(0, H // 2, ctx_body, 0)

        cur.to(cfg["u_attn_b"])
        for unit in range(B // UB):
            assert (cur.pos + unit * UB * sum(cfg["n_attn_b"]) + cfg["n_attn_b"][0]
                    >= u_kv + (unit + 1) * 2 * kv_bursts)
        iss_b = cur.loop(B, cfg["n_attn_b"])
        first = jax.lax.broadcasted_iota(jnp.int32, (2 * rep, 1), 0) < rep

        def attn_b(b, carry):
            iss_b(b, 0)
            unit, sub = _divmod_pow2(b, UB)

            @pl.when(sub == 0)
            def _():
                wait(kc_v.at[pl.ds(unit * NSTR, NSTR)], S_KV + 2 * unit)
                wait(vc_v.at[pl.ds(unit * NSTR, NSTR)], S_KV + 2 * unit + 1)

            for gp in range(HP):
                if gp == HP // 2:
                    iss_b(b, 1)
                a = b * HP + gp
                q = qb_s[pl.ds(gp * 2 * rep * B + b, 2 * rep, stride=B), :].astype(BF16)
                s0 = jax.lax.dot_general(q, kc_v[a, 0], _NT, preferred_element_type=F32)
                s1 = jax.lax.dot_general(q, kc_v[a, 1], _NT, preferred_element_type=F32)
                s = jnp.where(first, s0, s1) * scale
                m = jnp.max(s, axis=-1, keepdims=True)
                p = jnp.exp(s - m)
                l = jnp.sum(p, axis=-1, keepdims=True)
                p = p.astype(BF16)
                o0 = jnp.dot(p, vc_v[a, 0], preferred_element_type=F32)
                o1 = jnp.dot(p, vc_v[a, 1], preferred_element_type=F32)
                row = pl.multiple_of(a * 2 * rep, 2 * rep)
                ob_s[pl.ds(row, 2 * rep), :] = jnp.where(first, o0, o1) / l
            return carry

        jax.lax.fori_loop(0, B, attn_b, 0)

        def lhs(which, s0, ns, band):
            hs = [s * NBAND + band for s in range(s0, s0 + ns)]
            if which == 0:
                parts = [ctx_s[h] for h in hs]
            else:
                parts = [ob_s[pl.ds(h, B, stride=H), :] for h in hs]
            return jnp.concatenate(parts, axis=1).astype(BF16)

        def proj(l, which, s0, ns, band):
            w = (wo_v, bwo_v)[which][pl.ds(s0, ns), pl.ds(band * D, D), :].reshape(ns * D, M)
            return jnp.dot(l, w, preferred_element_type=F32)

        def do_band(which, band):
            wait((wo_v, bwo_v)[which].at[:, pl.ds(band * D, D)], S_W3 + 2 * band + which)
            r = proj(lhs(which, 0, NSTR, band), which, 0, NSTR, band)
            acc_s[which] = r if band == 0 else acc_s[which] + r

        last = NBAND - 1
        todo = [(which, band) for band in range(NBAND) for which in range(2)][:-1]
        for u, n in cfg["u_band"]:
            cur.to(u)
            for _ in range(n):
                which, band = todo.pop(0)
                assert band < last and (cur.pos - u_w3) * BURST >= (
                    (band + 1) * band_bursts * BURST + (skews[4] if which == 0 else 0))
                do_band(which, band)
        cur.to(n_bursts)

        starts = [sum(tail_blocks[:k]) for k in range(len(tail_blocks))]
        narrow = []
        for k, (s0, ns) in enumerate(zip(starts, tail_blocks)):
            rows = 32 // ns
            narrow += [((pl.ds(s0, ns), pl.ds(r, rows), every), S_TAIL + k)
                       for r in range(last * D, (last + 1) * D, rows)]
        assert len(narrow) == band_bursts * BURST

        def d_narrow(blk, i):
            sl, sem = narrow[(blk - last * band_bursts) * BURST + i]
            start(bwo_h.at[sl], bwo_v.at[sl], sem, 1)

        for u in range(last * band_bursts, w_bursts):
            burst(u, w_bursts, skews[4], d_wo, d_narrow)

        xf = x_v[...].astype(F32)
        gw = gw_v[...].astype(F32)
        t = xf[:, 0:128] * gw[0:1, :]
        for i in range(1, M // 128):
            t = t + xf[:, i * 128:(i + 1) * 128] * gw[i:i + 1, :]
        gate = jax.nn.sigmoid(jnp.sum(t, axis=-1, keepdims=True))

        for which, band in todo:
            do_band(which, band)
        tail_lhs = [lhs(1, s0, ns, last) for s0, ns in zip(starts, tail_blocks)]
        out = gate * acc_s[0]
        acc = acc_s[1]
        for k, (s0, ns) in enumerate(zip(starts, tail_blocks)):
            wait(bwo_v.at[pl.ds(s0, ns), pl.ds(last * D, D)], S_TAIL + k)
            acc = acc + proj(tail_lhs[k], 1, s0, ns, last)
        o_ref[...] = (out + (1.0 - gate) * acc).astype(o_ref.dtype)

    return kernel, n_sems


DEFAULT_CFG = dict(
    u_q=22, split_steps=8, n_split=(1,), u_uk=38, n_qabs=(1,),
    u_attn_a=80, n_attn_a=(2, 2, 2),
    n_ctx=(1,),
    u_attn_b=148, n_attn_b=(2, 1),
    u_band=((172, 2),),
    tail_blocks=(4, 2, 1, 1),
    skews=(124, 27, 26, 26, 0),
    head=(26, 30),
)
DEFAULT_PARAMS = dict(disable_bounds_checks=True, disable_semaphore_checks=True)


def _compiler_params(params):
    vmem = 112 * 1024 * 1024
    try:
        return pltpu.CompilerParams(vmem_limit_bytes=vmem, **params)
    except TypeError:
        params = {k: v for k, v in params.items() if k != "disable_semaphore_checks"}
        return pltpu.CompilerParams(vmem_limit_bytes=vmem, **params)


def _forward(A_x, A_c_kv, A_w_q, A_w_uk, A_w_uv, A_w_o, B_k_cache, B_v_cache, B_wq, B_wo,
             gate_w, cfg, params):
    B, Sq, M = A_x.shape
    assert Sq == 1
    _, Sk, Dc = A_c_kv.shape
    _, H, D = A_w_q.shape
    _, Hkv, SkB, _ = B_k_cache.shape
    W = min(4096, max(256, SkB // 4))
    HD = H * D

    kernel, n_sems = _make_kernel(B, M, H, D, Dc, Sk, Hkv, SkB, W, cfg)
    any_spec = pl.BlockSpec(memory_space=pl.ANY)
    out = pl.pallas_call(
        kernel,
        out_shape=jax.ShapeDtypeStruct((B, M), A_x.dtype),
        in_specs=[any_spec] * 11,
        out_specs=pl.BlockSpec(memory_space=pltpu.VMEM),
        scratch_shapes=[
            pltpu.VMEM((B, M), BF16),
            pltpu.VMEM((M // 128, 128), BF16),
            pltpu.VMEM((B * 4, Sk // 4, Dc), BF16),
            pltpu.VMEM((NSTR, M * H // NSTR, D), BF16),
            pltpu.VMEM((NSTR, Dc * H // NSTR, D), BF16),
            pltpu.VMEM((NSTR, Dc * H // NSTR, D), BF16),
            pltpu.VMEM((NSTR, HD // NSTR, M), BF16),
            pltpu.VMEM((B * Hkv // 2, 2, W, D), BF16),
            pltpu.VMEM((B * Hkv // 2, 2, W, D), BF16),
            pltpu.VMEM((NSTR, M // NSTR, HD), BF16),
            pltpu.VMEM((NSTR, HD // NSTR, M), BF16),
            pltpu.VMEM(((H + 1) * PLANE, D), U32),
            pltpu.VMEM(((H + 1) * PLANE, D), U32),
            pltpu.VMEM((Dc // 128, (H + 1) * B, 128), F32),
            pltpu.VMEM((Dc // 128, (B + 1) * H, 128), F32),
            pltpu.VMEM((H, B, D), F32),
            pltpu.VMEM(((H + 1) * B, D), F32),
            pltpu.VMEM(((B + 1) * H, D), F32),
            pltpu.VMEM((2, B, M), F32),
            pltpu.SemaphoreType.DMA((n_sems,)),
        ],
        compiler_params=_compiler_params(params),
        name="gated_mix_decode",
    )(
        A_x.reshape(B, M),
        gate_w.reshape(M // 128, 128),
        A_c_kv.reshape(B * 4, Sk // 4, Dc),
        A_w_q.reshape(NSTR, M * H // NSTR, D),
        A_w_uk.reshape(NSTR, Dc * H // NSTR, D),
        A_w_uv.reshape(NSTR, Dc * H // NSTR, D),
        A_w_o.reshape(NSTR, HD // NSTR, M),
        B_k_cache.reshape(B * Hkv // 2, 2, SkB, D),
        B_v_cache.reshape(B * Hkv // 2, 2, SkB, D),
        B_wq.reshape(NSTR, M // NSTR, HD),
        B_wo.reshape(NSTR, HD // NSTR, M),
    )
    return out.reshape(B, 1, M)


@jax.jit
def pallas_gated_mix__compressed_kv_cla__sliding_block_cached__decode_kernel(
    A_x: jax.Array,
    A_c_kv: jax.Array,
    A_w_q: jax.Array,
    A_w_uk: jax.Array,
    A_w_uv: jax.Array,
    A_w_o: jax.Array,
    B_x: jax.Array,
    B_k_cache: jax.Array,
    B_v_cache: jax.Array,
    B_wq: jax.Array,
    B_wo: jax.Array,
    gate_w: jax.Array,
):
    return _forward(A_x, A_c_kv, A_w_q, A_w_uk, A_w_uv, A_w_o, B_k_cache, B_v_cache,
                    B_wq, B_wo, gate_w, DEFAULT_CFG, DEFAULT_PARAMS)
```

```python
import jax
import jax.numpy as jnp
import jax.experimental.pallas as pl
import jax.experimental.pallas.tpu as pltpu

F32 = jnp.float32
BF16 = jnp.bfloat16
U32 = jnp.uint32

_NT = (((1,), (1,)), ((), ()))

NSTR = 8
BURST = 8
PLANE = 264


def _divmod_pow2(u, n):
    assert n & (n - 1) == 0
    return u >> (n.bit_length() - 1), u & (n - 1)


def _mult(v, n):
    return v if isinstance(v, int) else pl.multiple_of(v, n)


def _split_heads(w_v, t_s, step, nsteps, heads):
    ns, rr, _ = w_v.shape
    per_stream = nsteps // ns
    stream, part = _divmod_pow2(step, per_stream)
    rows = rr // per_stream
    half = heads // 2
    for k in range(rows // (2 * heads)):
        r0 = pl.multiple_of(part * rows + k * 2 * heads, 2 * heads)
        w = pltpu.bitcast(w_v[stream, pl.ds(r0, 2 * heads), :], U32)
        ev, od = w[:half], w[half:]
        lo = (ev & jnp.uint32(0xFFFF)) | (od << 16)
        hi = (ev >> 16) | (od & jnp.uint32(0xFFFF0000))
        i = step * (rows // (2 * heads)) + k
        t_s[pl.ds(i, half, stride=PLANE), :] = lo
        t_s[pl.ds(half * PLANE + i, half, stride=PLANE), :] = hi


def _head(t_s, j, p, heads, rows):
    r0 = pl.multiple_of((p * (heads // 2) + j) * PLANE, 8)
    return pltpu.bitcast(t_s[pl.ds(r0, rows // 2), :], BF16)


def _make_kernel(B, M, H, D, Dc, Sk, Hkv, SkB, W, cfg):
    rep = H // Hkv
    scale = float(D) ** -0.5
    HD = H * D
    CS = 4
    CR = Sk // CS
    OR = HD // NSTR
    NBAND = OR // D
    HP = Hkv // 2
    UB = NSTR // HP
    tail_blocks = cfg["tail_blocks"]
    skews = cfg["skews"]
    assert sum(tail_blocks) == NSTR and max(M, Dc) // 2 <= PLANE

    S_X, S_GW, S_WQ, S_WUK, S_BWQ, S_WUV, S_CKV = 0, 1, 2, 3, 4, 5, 6
    S_KV = S_CKV + 2
    S_W3 = S_KV + 2 * (B // UB)
    S_TAIL = S_W3 + 2 * NBAND - 1
    n_sems = S_TAIL + len(tail_blocks)

    def kernel(x_h, gw_h, ckv_h, wq_h, wuk_h, wuv_h, wo_h, kc_h, vc_h, bwq_h, bwo_h,
               o_ref,
               x_v, gw_v, ckv_v, wq_v, wuk_v, wuv_v, wo_v, kc_v, vc_v, bwq_v, bwo_v,
               t0_s, t1_s, qabs_s, lat_s, ctx_s, qb_s, ob_s, acc_s, sems):
        def start(src, dst, sem, prio):
            pltpu.make_async_copy(src, dst, sems.at[sem]).start(priority=prio)

        def wait(buf, sem):
            pltpu.make_async_copy(buf, buf, sems.at[sem]).wait()

        every = slice(None)

        def rows16(src, dst, r, sem, prio):
            sl = (every, pl.ds(_mult(r, 16), 16), every)
            start(src.at[sl], dst.at[sl], sem, prio)

        def tiles2(src, dst, lead, r, c, sem, prio):
            sl = (lead, pl.ds(_mult(r, 8), 8), pl.ds(_mult(c, 256), 256))
            start(src.at[sl], dst.at[sl], sem, prio)

        def burst(u, nblk, skew, d0, d1):
            q, r = divmod(skew, BURST)
            blk0 = [(u - q - 1) & (nblk - 1), (u - q) & (nblk - 1)]
            for i in range(BURST):
                d0(blk0[i >= r], (i - r) % BURST)
                d1(u, i)

        def d_rows(src, dst, sem, prio):
            return lambda blk, i: rows16(src, dst, blk * (16 * BURST) + 16 * i, sem, prio)

        def d_tiles(src, dst, lead, sem, prio):
            nc = src.shape[-1] // 256

            def f(blk, i):
                if nc >= BURST:
                    rb, cb = _divmod_pow2(blk, nc // BURST)
                    r, c = rb * 8, cb * (256 * BURST) + 256 * i
                else:
                    r, c = blk * (8 * BURST // nc) + 8 * (i // nc), 256 * (i % nc)
                tiles2(src, dst, lead, r, c, sem(blk) if callable(sem) else sem, prio)
            return f

        w_bursts = wq_v.shape[1] // 16 // BURST

        def burst_w1(u):
            burst(u, w_bursts, skews[0], d_rows(wq_h, wq_v, S_WQ, 0),
                  d_tiles(bwq_h, bwq_v, every, S_BWQ, 1))

        def burst_w2(u):
            burst(u, w_bursts, skews[1], d_rows(wuk_h, wuk_v, S_WUK, 0),
                  d_rows(wuv_h, wuv_v, S_WUV, 1))

        ckv_bursts = (CR // 8) * (Dc // 256) // BURST

        def burst_ckv(u):
            half, uu = _divmod_pow2(u, ckv_bursts)
            d = [d_tiles(ckv_h, ckv_v, pl.ds(half * (2 * NSTR) + t * NSTR, NSTR), S_CKV + half, t)
                 for t in range(2)]
            burst(uu, ckv_bursts, skews[2], *d)

        kv_bursts = W // 16 // BURST

        def burst_kv(u):
            q, uu = _divmod_pow2(u, kv_bursts)
            unit, which = _divmod_pow2(q, 2)
            lead = pl.ds(unit * NSTR, NSTR)

            def go(src, dst):
                def d(t):
                    def f(blk, i):
                        r = blk * (16 * BURST) + 16 * i
                        start(src.at[lead, t, pl.ds(_mult(SkB - W + r, 16), 16)],
                              dst.at[lead, t, pl.ds(_mult(r, 16), 16)], S_KV + q, t)
                    return f
                burst(uu, kv_bursts, skews[3], d(0), d(1))

            pl.when(which == 0)(lambda: go(kc_h, kc_v))
            pl.when(which == 1)(lambda: go(vc_h, vc_v))

        band_bursts = w_bursts // NBAND
        d_wo = d_tiles(wo_h, wo_v, every,
                       lambda blk: S_W3 + 2 * _divmod_pow2(blk, band_bursts)[0], 0)
        d_bwo = d_tiles(bwo_h, bwo_v, every,
                        lambda blk: S_W3 + 2 * _divmod_pow2(blk, band_bursts)[0] + 1, 1)

        def burst_w3(u):
            burst(u, w_bursts, skews[4], d_wo, d_bwo)

        plan = []
        u0 = 0
        for fn, n in ((burst_w1, w_bursts),
                      (burst_w2, w_bursts),
                      (burst_ckv, 2 * ckv_bursts),
                      (burst_kv, B * kv_bursts),
                      (burst_w3, (NBAND - 1) * band_bursts)):
            plan.append((u0, n, fn))
            u0 += n
        n_bursts = u0
        u_w2, u_ckv, u_kv, u_w3 = (p[0] for p in plan[1:])

        def issue(first, count, lo, hi):
            hits = [(u0, n, fn) for u0, n, fn in plan if u0 < hi and lo < u0 + n]

            def one(u):
                for u0, n, fn in hits:
                    if len(hits) == 1:
                        fn(u - u0)
                    else:
                        pl.when(jnp.logical_and(u >= u0, u < u0 + n))(lambda: fn(u - u0))

            if count == 1:
                one(first)
            else:
                def body(i, c):
                    one(first + i)
                    return c
                jax.lax.fori_loop(0, count, body, 0)

        class Cursor:
            pos = 0

            def to(self, hi):
                assert self.pos <= hi <= n_bursts, (self.pos, hi)
                for u0, n, _ in plan:
                    a, b = max(self.pos, u0), min(hi, u0 + n)
                    if a < b:
                        issue(a, b - a, a, b)
                self.pos = hi

            def loop(self, iters, counts):
                per = sum(counts)
                lo, hi = self.pos, self.pos + iters * per
                assert hi <= n_bursts
                self.pos = hi

                def f(i, k):
                    if counts[k]:
                        issue(lo + i * per + sum(counts[:k]), counts[k], lo, hi)
                return f

        cur = Cursor()

        def split_loop(w_v, t_s):
            n = cfg["split_steps"]
            iss = cur.loop(n, cfg["n_split"])

            def body(i, carry):
                iss(i, 0)
                _split_heads(w_v, t_s, i, n, H)
                return carry

            jax.lax.fori_loop(0, n, body, 0)

        if cfg["head"]:
            head, rot = cfg["head"]
            n = w_bursts * BURST

            def wq_piece(j, prio):
                rows16(wq_h, wq_v, ((j + rot) & (n - 1)) * 16, S_WQ, prio)

            def bwq_piece(j):
                rb, cb = _divmod_pow2(j, HD // 256)
                tiles2(bwq_h, bwq_v, every, rb * 8, cb * 256, S_BWQ, 1)

            def sloop(cnt, f):
                def body(j, c):
                    f(j)
                    return c
                jax.lax.fori_loop(0, cnt, body, 0)

            for j in range(head):
                bwq_piece(j)
            sloop(n - head, lambda j: (wq_piece(j, 0), bwq_piece(j + head)))
            sloop(head // 2, lambda j: (wq_piece(n - head + j, 0), wq_piece(n - head // 2 + j, 1)))
            cur.pos = w_bursts
        else:
            cur.to(1)
        start(x_h, x_v, S_X, 0)
        start(gw_h, gw_v, S_GW, 1)
        cur.to(cfg["u_q"])

        assert cur.pos >= u_w2
        wait(x_v, S_X)
        wait(gw_v, S_GW)
        wait(wq_v, S_WQ)
        wait(bwq_v, S_BWQ)
        qb = jnp.dot(x_v[...], bwq_v[...].reshape(M, HD), preferred_element_type=F32)
        qb = qb.astype(BF16).astype(F32)
        for h in range(H):
            qb_s[h * B:(h + 1) * B, :] = qb[:, h * D:(h + 1) * D]

        split_loop(wq_v, t0_s)
        cur.to(cfg["u_uk"])
        assert cur.pos >= u_ckv
        wait(wuk_v, S_WUK)
        wait(wuv_v, S_WUV)
        split_loop(wuk_v, t1_s)
        iss_q = cur.loop(H // 2, cfg["n_qabs"])

        def qabs_body(j, carry):
            x = x_v[...]
            for p in range(2):
                q = jnp.dot(x, _head(t0_s, j, p, H, M),
                            preferred_element_type=F32).astype(BF16)
                qa = jax.lax.dot_general(q, _head(t1_s, j, p, H, Dc), _NT,
                                         preferred_element_type=F32) * scale
                row = pl.multiple_of((2 * j + p) * B, B)
                for t in range(Dc // 128):
                    qabs_s[t, pl.ds(row, B), :] = qa[:, t * 128:(t + 1) * 128]
            iss_q(j, 0)
            return carry

        jax.lax.fori_loop(0, H // 2, qabs_body, 0)
        split_loop(wuv_v, t0_s)

        cur.to(cfg["u_attn_a"])
        for half in range(2):
            assert cur.pos + half * (B // 2) * sum(cfg["n_attn_a"]) >= u_ckv + (half + 1) * ckv_bursts
        iss_a = cur.loop(B, cfg["n_attn_a"])

        def attn_a(b, carry):
            for half in range(2):
                pl.when(b == half * (B // 2))(
                    lambda: wait(ckv_v.at[pl.ds(half * 2 * NSTR, 2 * NSTR)], S_CKV + half))

            qa = jnp.concatenate(
                [qabs_s[t, pl.ds(b, H, stride=B), :] for t in range(Dc // 128)],
                axis=1).astype(BF16)
            def c_half(k):
                return ckv_v[pl.ds(b * CS + k * (CS // 2), CS // 2)].reshape(Sk // 2, Dc)

            s = []
            for k in range(2):
                s.append(jax.lax.dot_general(qa, c_half(k), _NT, preferred_element_type=F32))
                iss_a(b, k)
            s = jnp.concatenate(s, axis=1)
            m = jnp.max(s, axis=-1, keepdims=True)
            p = jnp.exp(s - m)
            l = jnp.sum(p, axis=-1, keepdims=True)
            p = p.astype(BF16)
            c = ckv_v[pl.ds(b * CS, CS)].reshape(Sk, Dc)
            lat = jnp.dot(p, c, preferred_element_type=F32)
            lat = lat / l
            row = pl.multiple_of(b * H, H)
            for t in range(Dc // 128):
                lat_s[t, pl.ds(row, H), :] = lat[:, t * 128:(t + 1) * 128]
            iss_a(b, 2)
            return carry

        jax.lax.fori_loop(0, B, attn_a, 0)

        iss_c = cur.loop(H // 2, cfg["n_ctx"])

        def ctx_body(j, carry):
            for p in range(2):
                lat = jnp.concatenate(
                    [lat_s[t, pl.ds(2 * j + p, B, stride=H), :] for t in range(Dc // 128)],
                    axis=1).astype(BF16)
                ctx_s[2 * j + p] = jnp.dot(lat, _head(t0_s, j, p, H, Dc),
                                           preferred_element_type=F32)
            iss_c(j, 0)
            return carry

        jax.lax.fori_loop(0, H // 2, ctx_body, 0)

        cur.to(cfg["u_attn_b"])
        for unit in range(B // UB):
            assert (cur.pos + unit * UB * sum(cfg["n_attn_b"]) + cfg["n_attn_b"][0]
                    >= u_kv + (unit + 1) * 2 * kv_bursts)
        iss_b = cur.loop(B, cfg["n_attn_b"])
        first = jax.lax.broadcasted_iota(jnp.int32, (2 * rep, 1), 0) < rep

        def attn_b(b, carry):
            iss_b(b, 0)
            unit, sub = _divmod_pow2(b, UB)

            @pl.when(sub == 0)
            def _():
                wait(kc_v.at[pl.ds(unit * NSTR, NSTR)], S_KV + 2 * unit)
                wait(vc_v.at[pl.ds(unit * NSTR, NSTR)], S_KV + 2 * unit + 1)

            for gp in range(HP):
                if gp == HP // 2:
                    iss_b(b, 1)
                a = b * HP + gp
                q = qb_s[pl.ds(gp * 2 * rep * B + b, 2 * rep, stride=B), :].astype(BF16)
                s0 = jax.lax.dot_general(q, kc_v[a, 0], _NT, preferred_element_type=F32)
                s1 = jax.lax.dot_general(q, kc_v[a, 1], _NT, preferred_element_type=F32)
                s = jnp.where(first, s0, s1) * scale
                m = jnp.max(s, axis=-1, keepdims=True)
                p = jnp.exp(s - m)
                l = jnp.sum(p, axis=-1, keepdims=True)
                p = p.astype(BF16)
                o0 = jnp.dot(p, vc_v[a, 0], preferred_element_type=F32)
                o1 = jnp.dot(p, vc_v[a, 1], preferred_element_type=F32)
                row = pl.multiple_of(a * 2 * rep, 2 * rep)
                ob_s[pl.ds(row, 2 * rep), :] = jnp.where(first, o0, o1) / l
            return carry

        jax.lax.fori_loop(0, B, attn_b, 0)

        def lhs(which, s0, ns, band):
            hs = [s * NBAND + band for s in range(s0, s0 + ns)]
            if which == 0:
                parts = [ctx_s[h] for h in hs]
            else:
                parts = [ob_s[pl.ds(h, B, stride=H), :] for h in hs]
            return jnp.concatenate(parts, axis=1).astype(BF16)

        def proj(l, which, s0, ns, band):
            w = (wo_v, bwo_v)[which][pl.ds(s0, ns), pl.ds(band * D, D), :].reshape(ns * D, M)
            return jnp.dot(l, w, preferred_element_type=F32)

        band_skew, rem = divmod(skews[4], band_bursts * BURST)
        assert rem == 0

        def do_band(which, k):
            band = k if which else (k - band_skew) % NBAND
            wait((wo_v, bwo_v)[which].at[:, pl.ds(band * D, D)], S_W3 + 2 * band + which)
            r = proj(lhs(which, 0, NSTR, band), which, 0, NSTR, band)
            acc_s[which] = r if k == 0 else acc_s[which] + r

        last = NBAND - 1
        todo = [(which, k) for k in range(NBAND) for which in range(2)][:-1]
        for u, n in cfg["u_band"]:
            cur.to(u)
            for _ in range(n):
                which, k = todo.pop(0)
                assert k < last and cur.pos >= u_w3 + (k + 1) * band_bursts
                do_band(which, k)
        cur.to(n_bursts)

        starts = [sum(tail_blocks[:k]) for k in range(len(tail_blocks))]
        narrow = []
        for k, (s0, ns) in enumerate(zip(starts, tail_blocks)):
            rows = 32 // ns
            narrow += [((pl.ds(s0, ns), pl.ds(r, rows), every), S_TAIL + k)
                       for r in range(last * D, (last + 1) * D, rows)]
        assert len(narrow) == band_bursts * BURST

        def d_narrow(blk, i):
            sl, sem = narrow[(blk - last * band_bursts) * BURST + i]
            start(bwo_h.at[sl], bwo_v.at[sl], sem, 1)

        for u in range(last * band_bursts, w_bursts):
            burst(u, w_bursts, skews[4], d_wo, d_narrow)

        xf = x_v[...].astype(F32)
        gw = gw_v[...].astype(F32)
        t = xf[:, 0:128] * gw[0:1, :]
        for i in range(1, M // 128):
            t = t + xf[:, i * 128:(i + 1) * 128] * gw[i:i + 1, :]
        gate = jax.nn.sigmoid(jnp.sum(t, axis=-1, keepdims=True))

        for which, k in todo:
            do_band(which, k)
        tail_lhs = [lhs(1, s0, ns, last) for s0, ns in zip(starts, tail_blocks)]
        out = gate * acc_s[0]
        acc = acc_s[1]
        for k, (s0, ns) in enumerate(zip(starts, tail_blocks)):
            wait(bwo_v.at[pl.ds(s0, ns), pl.ds(last * D, D)], S_TAIL + k)
            acc = acc + proj(tail_lhs[k], 1, s0, ns, last)
        o_ref[...] = (out + (1.0 - gate) * acc).astype(o_ref.dtype)

    return kernel, n_sems


DEFAULT_CFG = dict(
    u_q=22, split_steps=8, n_split=(1,), u_uk=38, n_qabs=(1,),
    u_attn_a=80, n_attn_a=(2, 2, 2),
    n_ctx=(1,),
    u_attn_b=148, n_attn_b=(2, 1),
    u_band=((172, 2),),
    tail_blocks=(4, 2, 1, 1),
    skews=(124, 28, 27, 26, 32),
    head=(26, 30),
)
DEFAULT_PARAMS = dict(disable_bounds_checks=True, disable_semaphore_checks=True)


def _compiler_params(params):
    vmem = 112 * 1024 * 1024
    try:
        return pltpu.CompilerParams(vmem_limit_bytes=vmem, **params)
    except TypeError:
        params = {k: v for k, v in params.items() if k != "disable_semaphore_checks"}
        return pltpu.CompilerParams(vmem_limit_bytes=vmem, **params)


def _forward(A_x, A_c_kv, A_w_q, A_w_uk, A_w_uv, A_w_o, B_k_cache, B_v_cache, B_wq, B_wo,
             gate_w, cfg, params):
    B, Sq, M = A_x.shape
    assert Sq == 1
    _, Sk, Dc = A_c_kv.shape
    _, H, D = A_w_q.shape
    _, Hkv, SkB, _ = B_k_cache.shape
    W = min(4096, max(256, SkB // 4))
    HD = H * D

    kernel, n_sems = _make_kernel(B, M, H, D, Dc, Sk, Hkv, SkB, W, cfg)
    any_spec = pl.BlockSpec(memory_space=pl.ANY)
    out = pl.pallas_call(
        kernel,
        out_shape=jax.ShapeDtypeStruct((B, M), A_x.dtype),
        in_specs=[any_spec] * 11,
        out_specs=pl.BlockSpec(memory_space=pltpu.VMEM),
        scratch_shapes=[
            pltpu.VMEM((B, M), BF16),
            pltpu.VMEM((M // 128, 128), BF16),
            pltpu.VMEM((B * 4, Sk // 4, Dc), BF16),
            pltpu.VMEM((NSTR, M * H // NSTR, D), BF16),
            pltpu.VMEM((NSTR, Dc * H // NSTR, D), BF16),
            pltpu.VMEM((NSTR, Dc * H // NSTR, D), BF16),
            pltpu.VMEM((NSTR, HD // NSTR, M), BF16),
            pltpu.VMEM((B * Hkv // 2, 2, W, D), BF16),
            pltpu.VMEM((B * Hkv // 2, 2, W, D), BF16),
            pltpu.VMEM((NSTR, M // NSTR, HD), BF16),
            pltpu.VMEM((NSTR, HD // NSTR, M), BF16),
            pltpu.VMEM(((H + 1) * PLANE, D), U32),
            pltpu.VMEM(((H + 1) * PLANE, D), U32),
            pltpu.VMEM((Dc // 128, (H + 1) * B, 128), F32),
            pltpu.VMEM((Dc // 128, (B + 1) * H, 128), F32),
            pltpu.VMEM((H, B, D), F32),
            pltpu.VMEM(((H + 1) * B, D), F32),
            pltpu.VMEM(((B + 1) * H, D), F32),
            pltpu.VMEM((2, B, M), F32),
            pltpu.SemaphoreType.DMA((n_sems,)),
        ],
        compiler_params=_compiler_params(params),
        name="gated_mix_decode",
    )(
        A_x.reshape(B, M),
        gate_w.reshape(M // 128, 128),
        A_c_kv.reshape(B * 4, Sk // 4, Dc),
        A_w_q.reshape(NSTR, M * H // NSTR, D),
        A_w_uk.reshape(NSTR, Dc * H // NSTR, D),
        A_w_uv.reshape(NSTR, Dc * H // NSTR, D),
        A_w_o.reshape(NSTR, HD // NSTR, M),
        B_k_cache.reshape(B * Hkv // 2, 2, SkB, D),
        B_v_cache.reshape(B * Hkv // 2, 2, SkB, D),
        B_wq.reshape(NSTR, M // NSTR, HD),
        B_wo.reshape(NSTR, HD // NSTR, M),
    )
    return out.reshape(B, 1, M)


@jax.jit
def pallas_gated_mix__compressed_kv_cla__sliding_block_cached__decode_kernel(
    A_x: jax.Array,
    A_c_kv: jax.Array,
    A_w_q: jax.Array,
    A_w_uk: jax.Array,
    A_w_uv: jax.Array,
    A_w_o: jax.Array,
    B_x: jax.Array,
    B_k_cache: jax.Array,
    B_v_cache: jax.Array,
    B_wq: jax.Array,
    B_wo: jax.Array,
    gate_w: jax.Array,
):
    return _forward(A_x, A_c_kv, A_w_q, A_w_uk, A_w_uv, A_w_o, B_k_cache, B_v_cache,
                    B_wq, B_wo, gate_w, DEFAULT_CFG, DEFAULT_PARAMS)
```

```python
import jax
import jax.numpy as jnp
import jax.experimental.pallas as pl
import jax.experimental.pallas.tpu as pltpu

F32 = jnp.float32
BF16 = jnp.bfloat16
U32 = jnp.uint32

_NT = (((1,), (1,)), ((), ()))

NSTR = 8
BURST = 8
PLANE = 264


def _divmod_pow2(u, n):
    assert n & (n - 1) == 0
    return u >> (n.bit_length() - 1), u & (n - 1)


def _mult(v, n):
    return v if isinstance(v, int) else pl.multiple_of(v, n)


def _split_heads(w_v, t_s, step, nsteps, heads):
    ns, rr, _ = w_v.shape
    per_stream = nsteps // ns
    stream, part = _divmod_pow2(step, per_stream)
    rows = rr // per_stream
    half = heads // 2
    for k in range(rows // (2 * heads)):
        r0 = pl.multiple_of(part * rows + k * 2 * heads, 2 * heads)
        w = pltpu.bitcast(w_v[stream, pl.ds(r0, 2 * heads), :], U32)
        ev, od = w[:half], w[half:]
        lo = (ev & jnp.uint32(0xFFFF)) | (od << 16)
        hi = (ev >> 16) | (od & jnp.uint32(0xFFFF0000))
        i = step * (rows // (2 * heads)) + k
        t_s[pl.ds(i, half, stride=PLANE), :] = lo
        t_s[pl.ds(half * PLANE + i, half, stride=PLANE), :] = hi


def _head(t_s, j, p, heads, rows):
    r0 = pl.multiple_of((p * (heads // 2) + j) * PLANE, 8)
    return pltpu.bitcast(t_s[pl.ds(r0, rows // 2), :], BF16)


def _make_kernel(B, M, H, D, Dc, Sk, Hkv, SkB, W, cfg):
    rep = H // Hkv
    scale = float(D) ** -0.5
    HD = H * D
    CS = 4
    CR = Sk // CS
    OR = HD // NSTR
    NBAND = OR // D
    HP = Hkv // 2
    UB = NSTR // HP
    tail_blocks = cfg["tail_blocks"]
    skew_w2, skew_ckv, skew_kv, skew_w3 = cfg["skews"]
    assert sum(tail_blocks) == NSTR and max(M, Dc) // 2 <= PLANE

    S_X, S_GW, S_WQ, S_WUK, S_BWQ, S_WUV, S_CKV = 0, 1, 2, 3, 4, 5, 6
    S_KV = S_CKV + 2
    S_W3 = S_KV + 2 * (B // UB)
    S_TAIL = S_W3 + 2 * NBAND - 1
    n_sems = S_TAIL + len(tail_blocks)

    def kernel(x_h, gw_h, ckv_h, wq_h, wuk_h, wuv_h, wo_h, kc_h, vc_h, bwq_h, bwo_h,
               o_ref,
               x_v, gw_v, ckv_v, wq_v, wuk_v, wuv_v, wo_v, kc_v, vc_v, bwq_v, bwo_v,
               t0_s, t1_s, qabs_s, lat_s, ctx_s, qb_s, ob_s, acc_s, sems):
        def start(src, dst, sem, prio):
            pltpu.make_async_copy(src, dst, sems.at[sem]).start(priority=prio)

        def wait(buf, sem):
            pltpu.make_async_copy(buf, buf, sems.at[sem]).wait()

        every = slice(None)

        def rows16(src, dst, r, sem, prio):
            sl = (every, pl.ds(_mult(r, 16), 16), every)
            start(src.at[sl], dst.at[sl], sem, prio)

        def tiles2(src, dst, lead, r, c, sem, prio):
            sl = (lead, pl.ds(_mult(r, 8), 8), pl.ds(_mult(c, 256), 256))
            start(src.at[sl], dst.at[sl], sem, prio)

        def burst(u, nblk, skew, d0, d1):
            q, r = divmod(skew, BURST)
            blk0 = [(u - q - 1) & (nblk - 1), (u - q) & (nblk - 1)]
            for i in range(BURST):
                d0(blk0[i >= r], (i - r) % BURST)
                d1(u, i)

        def d_rows(src, dst, sem, prio):
            return lambda blk, i: rows16(src, dst, blk * (16 * BURST) + 16 * i, sem, prio)

        def d_tiles(src, dst, lead, sem, prio):
            nc = src.shape[-1] // 256

            def f(blk, i):
                r, c = blk * (8 * BURST // nc) + 8 * (i // nc), 256 * (i % nc)
                tiles2(src, dst, lead, r, c, sem(blk) if callable(sem) else sem, prio)
            return f

        w_bursts = wq_v.shape[1] // 16 // BURST

        def burst_w2(u):
            burst(u, w_bursts, skew_w2, d_rows(wuk_h, wuk_v, S_WUK, 0),
                  d_rows(wuv_h, wuv_v, S_WUV, 1))

        ckv_bursts = (CR // 8) * (Dc // 256) // BURST

        def burst_ckv(u):
            half, uu = _divmod_pow2(u, ckv_bursts)
            d = [d_tiles(ckv_h, ckv_v, pl.ds(half * (2 * NSTR) + t * NSTR, NSTR), S_CKV + half, t)
                 for t in range(2)]
            burst(uu, ckv_bursts, skew_ckv, *d)

        kv_bursts = W // 16 // BURST

        def burst_kv(u):
            q, uu = _divmod_pow2(u, kv_bursts)
            unit, which = _divmod_pow2(q, 2)
            lead = pl.ds(unit * NSTR, NSTR)

            def go(src, dst):
                def d(t):
                    def f(blk, i):
                        r = blk * (16 * BURST) + 16 * i
                        start(src.at[lead, t, pl.ds(_mult(SkB - W + r, 16), 16)],
                              dst.at[lead, t, pl.ds(_mult(r, 16), 16)], S_KV + q, t)
                    return f
                burst(uu, kv_bursts, skew_kv, d(0), d(1))

            pl.when(which == 0)(lambda: go(kc_h, kc_v))
            pl.when(which == 1)(lambda: go(vc_h, vc_v))

        band_bursts = w_bursts // NBAND
        d_wo = d_tiles(wo_h, wo_v, every,
                       lambda blk: S_W3 + 2 * _divmod_pow2(blk, band_bursts)[0], 0)
        d_bwo = d_tiles(bwo_h, bwo_v, every,
                        lambda blk: S_W3 + 2 * _divmod_pow2(blk, band_bursts)[0] + 1, 1)

        def burst_w3(u):
            burst(u, w_bursts, skew_w3, d_wo, d_bwo)

        plan = []
        u0 = w_bursts
        for fn, n in ((burst_w2, w_bursts),
                      (burst_ckv, 2 * ckv_bursts),
                      (burst_kv, B * kv_bursts),
                      (burst_w3, (NBAND - 1) * band_bursts)):
            plan.append((u0, n, fn))
            u0 += n
        n_bursts = u0
        u_w2, u_ckv, u_kv, u_w3 = (p[0] for p in plan)

        def issue(first, count, lo, hi):
            hits = [(u0, n, fn) for u0, n, fn in plan if u0 < hi and lo < u0 + n]

            def one(u):
                for u0, n, fn in hits:
                    if len(hits) == 1:
                        fn(u - u0)
                    else:
                        pl.when(jnp.logical_and(u >= u0, u < u0 + n))(lambda: fn(u - u0))

            if count == 1:
                one(first)
            else:
                def body(i, c):
                    one(first + i)
                    return c
                jax.lax.fori_loop(0, count, body, 0)

        class Cursor:
            pos = u_w2

            def to(self, hi):
                assert self.pos <= hi <= n_bursts, (self.pos, hi)
                for u0, n, _ in plan:
                    a, b = max(self.pos, u0), min(hi, u0 + n)
                    if a < b:
                        issue(a, b - a, a, b)
                self.pos = hi

            def loop(self, iters, counts):
                per = sum(counts)
                lo, hi = self.pos, self.pos + iters * per
                assert hi <= n_bursts
                self.pos = hi

                def f(i, k):
                    if counts[k]:
                        issue(lo + i * per + sum(counts[:k]), counts[k], lo, hi)
                return f

        cur = Cursor()

        def split_loop(w_v, t_s):
            n = cfg["split_steps"]
            iss = cur.loop(n, cfg["n_split"])

            def body(i, carry):
                iss(i, 0)
                _split_heads(w_v, t_s, i, n, H)
                return carry

            jax.lax.fori_loop(0, n, body, 0)

        head, rot = cfg["head"]
        n = w_bursts * BURST

        def wq_piece(j, prio):
            rows16(wq_h, wq_v, ((j + rot) & (n - 1)) * 16, S_WQ, prio)

        def bwq_piece(j):
            rb, cb = _divmod_pow2(j, HD // 256)
            tiles2(bwq_h, bwq_v, every, rb * 8, cb * 256, S_BWQ, 1)

        def repeat(count, f):
            def body(j, carry):
                f(j)
                return carry
            jax.lax.fori_loop(0, count, body, 0)

        assert head % 2 == 0
        for j in range(head):
            bwq_piece(j)
        repeat(n - head, lambda j: (wq_piece(j, 0), bwq_piece(j + head)))
        repeat(head // 2, lambda j: (wq_piece(n - head + j, 0), wq_piece(n - head // 2 + j, 1)))
        start(x_h, x_v, S_X, 0)
        start(gw_h, gw_v, S_GW, 1)
        cur.to(cfg["u_q"])

        wait(x_v, S_X)
        wait(gw_v, S_GW)
        wait(wq_v, S_WQ)
        wait(bwq_v, S_BWQ)
        qb = jnp.dot(x_v[...], bwq_v[...].reshape(M, HD), preferred_element_type=F32)
        qb = qb.astype(BF16).astype(F32)
        for h in range(H):
            qb_s[h * B:(h + 1) * B, :] = qb[:, h * D:(h + 1) * D]

        split_loop(wq_v, t0_s)
        cur.to(cfg["u_uk"])
        assert cur.pos >= u_ckv
        wait(wuk_v, S_WUK)
        wait(wuv_v, S_WUV)
        split_loop(wuk_v, t1_s)
        iss_q = cur.loop(H // 2, cfg["n_qabs"])

        def qabs_body(j, carry):
            x = x_v[...]
            for p in range(2):
                q = jnp.dot(x, _head(t0_s, j, p, H, M),
                            preferred_element_type=F32).astype(BF16)
                qa = jax.lax.dot_general(q, _head(t1_s, j, p, H, Dc), _NT,
                                         preferred_element_type=F32) * scale
                row = pl.multiple_of((2 * j + p) * B, B)
                for t in range(Dc // 128):
                    qabs_s[t, pl.ds(row, B), :] = qa[:, t * 128:(t + 1) * 128]
            iss_q(j, 0)
            return carry

        jax.lax.fori_loop(0, H // 2, qabs_body, 0)
        split_loop(wuv_v, t0_s)

        cur.to(cfg["u_attn_a"])
        for half in range(2):
            assert cur.pos + half * (B // 2) * sum(cfg["n_attn_a"]) >= u_ckv + (half + 1) * ckv_bursts
        iss_a = cur.loop(B, cfg["n_attn_a"])

        def attn_a(b, carry):
            for half in range(2):
                pl.when(b == half * (B // 2))(
                    lambda: wait(ckv_v.at[pl.ds(half * 2 * NSTR, 2 * NSTR)], S_CKV + half))

            qa = jnp.concatenate(
                [qabs_s[t, pl.ds(b, H, stride=B), :] for t in range(Dc // 128)],
                axis=1).astype(BF16)
            def c_half(k):
                return ckv_v[pl.ds(b * CS + k * (CS // 2), CS // 2)].reshape(Sk // 2, Dc)

            s = []
            for k in range(2):
                s.append(jax.lax.dot_general(qa, c_half(k), _NT, preferred_element_type=F32))
                iss_a(b, k)
            s = jnp.concatenate(s, axis=1)
            m = jnp.max(s, axis=-1, keepdims=True)
            p = jnp.exp(s - m)
            l = jnp.sum(p, axis=-1, keepdims=True)
            p = p.astype(BF16)
            c = ckv_v[pl.ds(b * CS, CS)].reshape(Sk, Dc)
            lat = jnp.dot(p, c, preferred_element_type=F32)
            lat = lat / l
            row = pl.multiple_of(b * H, H)
            for t in range(Dc // 128):
                lat_s[t, pl.ds(row, H), :] = lat[:, t * 128:(t + 1) * 128]
            iss_a(b, 2)
            return carry

        jax.lax.fori_loop(0, B, attn_a, 0)

        iss_c = cur.loop(H // 2, cfg["n_ctx"])

        def ctx_body(j, carry):
            for p in range(2):
                lat = jnp.concatenate(
                    [lat_s[t, pl.ds(2 * j + p, B, stride=H), :] for t in range(Dc // 128)],
                    axis=1).astype(BF16)
                ctx_s[2 * j + p] = jnp.dot(lat, _head(t0_s, j, p, H, Dc),
                                           preferred_element_type=F32)
            iss_c(j, 0)
            return carry

        jax.lax.fori_loop(0, H // 2, ctx_body, 0)

        cur.to(cfg["u_attn_b"])
        for unit in range(B // UB):
            assert (cur.pos + unit * UB * sum(cfg["n_attn_b"]) + cfg["n_attn_b"][0]
                    >= u_kv + (unit + 1) * 2 * kv_bursts)
        iss_b = cur.loop(B, cfg["n_attn_b"])
        first = jax.lax.broadcasted_iota(jnp.int32, (2 * rep, 1), 0) < rep

        def attn_b(b, carry):
            iss_b(b, 0)
            unit, sub = _divmod_pow2(b, UB)

            @pl.when(sub == 0)
            def _():
                wait(kc_v.at[pl.ds(unit * NSTR, NSTR)], S_KV + 2 * unit)
                wait(vc_v.at[pl.ds(unit * NSTR, NSTR)], S_KV + 2 * unit + 1)

            for gp in range(HP):
                if gp == HP // 2:
                    iss_b(b, 1)
                a = b * HP + gp
                q = qb_s[pl.ds(gp * 2 * rep * B + b, 2 * rep, stride=B), :].astype(BF16)
                s0 = jax.lax.dot_general(q, kc_v[a, 0], _NT, preferred_element_type=F32)
                s1 = jax.lax.dot_general(q, kc_v[a, 1], _NT, preferred_element_type=F32)
                s = jnp.where(first, s0, s1) * scale
                m = jnp.max(s, axis=-1, keepdims=True)
                p = jnp.exp(s - m)
                l = jnp.sum(p, axis=-1, keepdims=True)
                p = p.astype(BF16)
                o0 = jnp.dot(p, vc_v[a, 0], preferred_element_type=F32)
                o1 = jnp.dot(p, vc_v[a, 1], preferred_element_type=F32)
                row = pl.multiple_of(a * 2 * rep, 2 * rep)
                ob_s[pl.ds(row, 2 * rep), :] = jnp.where(first, o0, o1) / l
            return carry

        jax.lax.fori_loop(0, B, attn_b, 0)

        def lhs(which, s0, ns, band):
            hs = [s * NBAND + band for s in range(s0, s0 + ns)]
            if which == 0:
                parts = [ctx_s[h] for h in hs]
            else:
                parts = [ob_s[pl.ds(h, B, stride=H), :] for h in hs]
            return jnp.concatenate(parts, axis=1).astype(BF16)

        def proj(l, which, s0, ns, band):
            w = (wo_v, bwo_v)[which][pl.ds(s0, ns), pl.ds(band * D, D), :].reshape(ns * D, M)
            return jnp.dot(l, w, preferred_element_type=F32)

        band_skew, rem = divmod(skew_w3, band_bursts * BURST)
        assert rem == 0

        def do_band(which, k):
            band = k if which else (k - band_skew) % NBAND
            wait((wo_v, bwo_v)[which].at[:, pl.ds(band * D, D)], S_W3 + 2 * band + which)
            r = proj(lhs(which, 0, NSTR, band), which, 0, NSTR, band)
            acc_s[which] = r if k == 0 else acc_s[which] + r

        last = NBAND - 1
        todo = [(which, k) for k in range(NBAND) for which in range(2)][:-1]
        for u, n in cfg["u_band"]:
            cur.to(u)
            for _ in range(n):
                which, k = todo.pop(0)
                assert k < last and cur.pos >= u_w3 + (k + 1) * band_bursts
                do_band(which, k)
        cur.to(n_bursts)

        starts = [sum(tail_blocks[:k]) for k in range(len(tail_blocks))]
        narrow = []
        for k, (s0, ns) in enumerate(zip(starts, tail_blocks)):
            rows = 32 // ns
            narrow += [((pl.ds(s0, ns), pl.ds(r, rows), every), S_TAIL + k)
                       for r in range(last * D, (last + 1) * D, rows)]
        assert len(narrow) == band_bursts * BURST

        def d_narrow(blk, i):
            sl, sem = narrow[(blk - last * band_bursts) * BURST + i]
            start(bwo_h.at[sl], bwo_v.at[sl], sem, 1)

        for u in range(last * band_bursts, w_bursts):
            burst(u, w_bursts, skew_w3, d_wo, d_narrow)

        xf = x_v[...].astype(F32)
        gw = gw_v[...].astype(F32)
        t = xf[:, 0:128] * gw[0:1, :]
        for i in range(1, M // 128):
            t = t + xf[:, i * 128:(i + 1) * 128] * gw[i:i + 1, :]
        gate = jax.nn.sigmoid(jnp.sum(t, axis=-1, keepdims=True))

        for which, k in todo:
            do_band(which, k)
        tail_lhs = [lhs(1, s0, ns, last) for s0, ns in zip(starts, tail_blocks)]
        out = gate * acc_s[0]
        acc = acc_s[1]
        for k, (s0, ns) in enumerate(zip(starts, tail_blocks)):
            wait(bwo_v.at[pl.ds(s0, ns), pl.ds(last * D, D)], S_TAIL + k)
            acc = acc + proj(tail_lhs[k], 1, s0, ns, last)
        o_ref[...] = (out + (1.0 - gate) * acc).astype(o_ref.dtype)

    return kernel, n_sems


DEFAULT_CFG = dict(
    head=(26, 30), skews=(28, 27, 26, 32),
    u_q=22, split_steps=8, n_split=(1,), u_uk=38, n_qabs=(1,),
    u_attn_a=80, n_attn_a=(2, 2, 2),
    n_ctx=(1,),
    u_attn_b=148, n_attn_b=(2, 1),
    u_band=((172, 2),),
    tail_blocks=(4, 2, 1, 1),
)
DEFAULT_PARAMS = dict(disable_bounds_checks=True, disable_semaphore_checks=True)


def _compiler_params(params):
    vmem = 112 * 1024 * 1024
    try:
        return pltpu.CompilerParams(vmem_limit_bytes=vmem, **params)
    except TypeError:
        params = {k: v for k, v in params.items() if k != "disable_semaphore_checks"}
        return pltpu.CompilerParams(vmem_limit_bytes=vmem, **params)


def _forward(A_x, A_c_kv, A_w_q, A_w_uk, A_w_uv, A_w_o, B_k_cache, B_v_cache, B_wq, B_wo,
             gate_w, cfg, params):
    B, Sq, M = A_x.shape
    assert Sq == 1
    _, Sk, Dc = A_c_kv.shape
    _, H, D = A_w_q.shape
    _, Hkv, SkB, _ = B_k_cache.shape
    W = min(4096, max(256, SkB // 4))
    HD = H * D

    kernel, n_sems = _make_kernel(B, M, H, D, Dc, Sk, Hkv, SkB, W, cfg)
    any_spec = pl.BlockSpec(memory_space=pl.ANY)
    out = pl.pallas_call(
        kernel,
        out_shape=jax.ShapeDtypeStruct((B, M), A_x.dtype),
        in_specs=[any_spec] * 11,
        out_specs=pl.BlockSpec(memory_space=pltpu.VMEM),
        scratch_shapes=[
            pltpu.VMEM((B, M), BF16),
            pltpu.VMEM((M // 128, 128), BF16),
            pltpu.VMEM((B * 4, Sk // 4, Dc), BF16),
            pltpu.VMEM((NSTR, M * H // NSTR, D), BF16),
            pltpu.VMEM((NSTR, Dc * H // NSTR, D), BF16),
            pltpu.VMEM((NSTR, Dc * H // NSTR, D), BF16),
            pltpu.VMEM((NSTR, HD // NSTR, M), BF16),
            pltpu.VMEM((B * Hkv // 2, 2, W, D), BF16),
            pltpu.VMEM((B * Hkv // 2, 2, W, D), BF16),
            pltpu.VMEM((NSTR, M // NSTR, HD), BF16),
            pltpu.VMEM((NSTR, HD // NSTR, M), BF16),
            pltpu.VMEM(((H + 1) * PLANE, D), U32),
            pltpu.VMEM(((H + 1) * PLANE, D), U32),
            pltpu.VMEM((Dc // 128, (H + 1) * B, 128), F32),
            pltpu.VMEM((Dc // 128, (B + 1) * H, 128), F32),
            pltpu.VMEM((H, B, D), F32),
            pltpu.VMEM(((H + 1) * B, D), F32),
            pltpu.VMEM(((B + 1) * H, D), F32),
            pltpu.VMEM((2, B, M), F32),
            pltpu.SemaphoreType.DMA((n_sems,)),
        ],
        compiler_params=_compiler_params(params),
        name="gated_mix_decode",
    )(
        A_x.reshape(B, M),
        gate_w.reshape(M // 128, 128),
        A_c_kv.reshape(B * 4, Sk // 4, Dc),
        A_w_q.reshape(NSTR, M * H // NSTR, D),
        A_w_uk.reshape(NSTR, Dc * H // NSTR, D),
        A_w_uv.reshape(NSTR, Dc * H // NSTR, D),
        A_w_o.reshape(NSTR, HD // NSTR, M),
        B_k_cache.reshape(B * Hkv // 2, 2, SkB, D),
        B_v_cache.reshape(B * Hkv // 2, 2, SkB, D),
        B_wq.reshape(NSTR, M // NSTR, HD),
        B_wo.reshape(NSTR, HD // NSTR, M),
    )
    return out.reshape(B, 1, M)


@jax.jit
def pallas_gated_mix__compressed_kv_cla__sliding_block_cached__decode_kernel(
    A_x: jax.Array,
    A_c_kv: jax.Array,
    A_w_q: jax.Array,
    A_w_uk: jax.Array,
    A_w_uv: jax.Array,
    A_w_o: jax.Array,
    B_x: jax.Array,
    B_k_cache: jax.Array,
    B_v_cache: jax.Array,
    B_wq: jax.Array,
    B_wo: jax.Array,
    gate_w: jax.Array,
):
    return _forward(A_x, A_c_kv, A_w_q, A_w_uk, A_w_uv, A_w_o, B_k_cache, B_v_cache,
                    B_wq, B_wo, gate_w, DEFAULT_CFG, DEFAULT_PARAMS)
```

```python
import jax
import jax.numpy as jnp
import jax.experimental.pallas as pl
import jax.experimental.pallas.tpu as pltpu

F32 = jnp.float32
BF16 = jnp.bfloat16
U32 = jnp.uint32

_NT = (((1,), (1,)), ((), ()))

NSTR = 8
BURST = 8
PLANE = 264


def _divmod_pow2(u, n, nq=None):
    assert n & (n - 1) == 0
    q = u >> (n.bit_length() - 1)
    if nq is not None:
        assert nq & (nq - 1) == 0
        q = q & (nq - 1)
    return q, u & (n - 1)


def _mult(v, n):
    return v if isinstance(v, int) else pl.multiple_of(v, n)


def _split_heads(w_v, t_s, step, nsteps, heads):
    ns, rr, _ = w_v.shape
    per_stream = nsteps // ns
    stream, part = _divmod_pow2(step, per_stream)
    rows = rr // per_stream
    half = heads // 2
    for k in range(rows // (2 * heads)):
        r0 = pl.multiple_of(part * rows + k * 2 * heads, 2 * heads)
        w = pltpu.bitcast(w_v[stream, pl.ds(r0, 2 * heads), :], U32)
        ev, od = w[:half], w[half:]
        lo = (ev & jnp.uint32(0xFFFF)) | (od << 16)
        hi = (ev >> 16) | (od & jnp.uint32(0xFFFF0000))
        i = step * (rows // (2 * heads)) + k
        t_s[pl.ds(i, half, stride=PLANE), :] = lo
        t_s[pl.ds(half * PLANE + i, half, stride=PLANE), :] = hi


def _head(t_s, j, p, heads, rows):
    r0 = pl.multiple_of((p * (heads // 2) + j) * PLANE, 8)
    return pltpu.bitcast(t_s[pl.ds(r0, rows // 2), :], BF16)


def _make_kernel(B, M, H, D, Dc, Sk, Hkv, SkB, W, cfg):
    rep = H // Hkv
    scale = float(D) ** -0.5
    HD = H * D
    CS = 4
    CR = Sk // CS
    OR = HD // NSTR
    NBAND = OR // D
    HP = Hkv // 2
    UB = NSTR // HP
    tail_blocks = cfg["tail_blocks"]
    skew_w2, skew_ckv, skew_kv, skew_w3 = cfg["skews"]
    assert sum(tail_blocks) == NSTR and max(M, Dc) // 2 <= PLANE

    S_X, S_GW, S_WQ, S_WUK, S_BWQ, S_WUV, S_CKV = 0, 1, 2, 3, 4, 5, 6
    S_KV = S_CKV + 2
    S_W3 = S_KV + 2 * (B // UB)
    S_TAIL = S_W3 + 2 * NBAND - 1
    n_sems = S_TAIL + len(tail_blocks)

    def kernel(x_h, gw_h, ckv_h, wq_h, wuk_h, wuv_h, wo_h, kc_h, vc_h, bwq_h, bwo_h,
               o_ref,
               x_v, gw_v, ckv_v, wq_v, wuk_v, wuv_v, wo_v, kc_v, vc_v, bwq_v, bwo_v,
               t0_s, t1_s, qabs_s, lat_s, ctx_s, qb_s, ob_s, acc_s, sems):
        def start(src, dst, sem, prio):
            pltpu.make_async_copy(src, dst, sems.at[sem]).start(priority=prio)

        def wait(buf, sem):
            pltpu.make_async_copy(buf, buf, sems.at[sem]).wait()

        every = slice(None)

        def rows16(src, dst, r, sem, prio):
            sl = (every, pl.ds(_mult(r, 16), 16), every)
            start(src.at[sl], dst.at[sl], sem, prio)

        def tiles2(src, dst, lead, r, c, sem, prio):
            sl = (lead, pl.ds(_mult(r, 8), 8), pl.ds(_mult(c, 256), 256))
            start(src.at[sl], dst.at[sl], sem, prio)

        def burst(u, nblk, skew, d0, d1):
            q, r = divmod(skew, BURST)
            blk0 = [(u - q - 1) & (nblk - 1), (u - q) & (nblk - 1)]
            for i in range(BURST):
                d0(blk0[i >= r], (i - r) % BURST)
                d1(u & (nblk - 1), i)

        def d_rows(src, dst, sem, prio):
            return lambda blk, i: rows16(src, dst, blk * (16 * BURST) + 16 * i, sem, prio)

        def d_tiles(src, dst, lead, sem, prio):
            nc = src.shape[-1] // 256

            def f(blk, i):
                r, c = blk * (8 * BURST // nc) + 8 * (i // nc), 256 * (i % nc)
                tiles2(src, dst, lead, r, c, sem(blk) if callable(sem) else sem, prio)
            return f

        w_bursts = wq_v.shape[1] // 16 // BURST

        def burst_w2(u):
            burst(u, w_bursts, skew_w2, d_rows(wuk_h, wuk_v, S_WUK, 0),
                  d_rows(wuv_h, wuv_v, S_WUV, 1))

        ckv_bursts = (CR // 8) * (Dc // 256) // BURST

        def burst_ckv(u):
            half, uu = _divmod_pow2(u, ckv_bursts, 2)
            d = [d_tiles(ckv_h, ckv_v, pl.ds(half * (2 * NSTR) + t * NSTR, NSTR), S_CKV + half, t)
                 for t in range(2)]
            burst(uu, ckv_bursts, skew_ckv, *d)

        kv_bursts = W // 16 // BURST

        def burst_kv(u):
            q, uu = _divmod_pow2(u, kv_bursts, 2 * (B // UB))
            unit, which = _divmod_pow2(q, 2)
            lead = pl.ds(unit * NSTR, NSTR)

            def go(src, dst):
                def d(t):
                    def f(blk, i):
                        r = blk * (16 * BURST) + 16 * i
                        start(src.at[lead, t, pl.ds(_mult(SkB - W + r, 16), 16)],
                              dst.at[lead, t, pl.ds(_mult(r, 16), 16)], S_KV + q, t)
                    return f
                burst(uu, kv_bursts, skew_kv, d(0), d(1))

            pl.when(which == 0)(lambda: go(kc_h, kc_v))
            pl.when(which == 1)(lambda: go(vc_h, vc_v))

        band_bursts = w_bursts // NBAND
        d_wo = d_tiles(wo_h, wo_v, every,
                       lambda blk: S_W3 + 2 * _divmod_pow2(blk, band_bursts)[0], 0)
        d_bwo = d_tiles(bwo_h, bwo_v, every,
                        lambda blk: S_W3 + 2 * _divmod_pow2(blk, band_bursts)[0] + 1, 1)

        def burst_w3(u):
            burst(u, w_bursts, skew_w3, d_wo, d_bwo)

        plan = []
        u0 = w_bursts
        for fn, n in ((burst_w2, w_bursts),
                      (burst_ckv, 2 * ckv_bursts),
                      (burst_kv, B * kv_bursts),
                      (burst_w3, (NBAND - 1) * band_bursts)):
            plan.append((u0, n, fn))
            u0 += n
        n_bursts = u0
        u_w2, u_ckv, u_kv, u_w3 = (p[0] for p in plan)

        def issue(first, count, lo, hi):
            hits = [(u0, n, fn) for u0, n, fn in plan if u0 < hi and lo < u0 + n]

            def one(u):
                for u0, n, fn in hits:
                    if len(hits) == 1:
                        fn(u - u0)
                    else:
                        pl.when(jnp.logical_and(u >= u0, u < u0 + n))(lambda: fn(u - u0))

            if count == 1:
                one(first)
            else:
                def body(i, c):
                    one(first + i)
                    return c
                jax.lax.fori_loop(0, count, body, 0)

        class Cursor:
            pos = u_w2

            def to(self, hi):
                assert self.pos <= hi <= n_bursts, (self.pos, hi)
                for u0, n, _ in plan:
                    a, b = max(self.pos, u0), min(hi, u0 + n)
                    if a < b:
                        issue(a, b - a, a, b)
                self.pos = hi

            def loop(self, iters, counts):
                per = sum(counts)
                lo, hi = self.pos, self.pos + iters * per
                assert hi <= n_bursts
                self.pos = hi

                def f(i, k):
                    if counts[k]:
                        issue(lo + i * per + sum(counts[:k]), counts[k], lo, hi)
                return f

        cur = Cursor()

        def split_loop(w_v, t_s):
            n = cfg["split_steps"]
            iss = cur.loop(n, cfg["n_split"])

            def body(i, carry):
                iss(i, 0)
                _split_heads(w_v, t_s, i, n, H)
                return carry

            jax.lax.fori_loop(0, n, body, 0)

        head, rot = cfg["head"]
        n = w_bursts * BURST

        def wq_piece(j, prio):
            rows16(wq_h, wq_v, ((j + rot) & (n - 1)) * 16, S_WQ, prio)

        def bwq_piece(j):
            rb, cb = _divmod_pow2(j, HD // 256, M // NSTR // 8)
            tiles2(bwq_h, bwq_v, every, rb * 8, cb * 256, S_BWQ, 1)

        def repeat(count, f):
            def body(j, carry):
                f(j)
                return carry
            jax.lax.fori_loop(0, count, body, 0)

        assert head % 2 == 0
        for j in range(head):
            bwq_piece(j)
        repeat(n - head, lambda j: (wq_piece(j, 0), bwq_piece(j + head)))
        repeat(head // 2, lambda j: (wq_piece(n - head + j, 0), wq_piece(n - head // 2 + j, 1)))
        start(x_h, x_v, S_X, 0)
        start(gw_h, gw_v, S_GW, 1)
        cur.to(cfg["u_q"])

        wait(x_v, S_X)
        wait(gw_v, S_GW)
        wait(wq_v, S_WQ)
        wait(bwq_v, S_BWQ)
        qb = jnp.dot(x_v[...], bwq_v[...].reshape(M, HD), preferred_element_type=F32)
        qb = qb.astype(BF16).astype(F32)
        for h in range(H):
            qb_s[h * B:(h + 1) * B, :] = qb[:, h * D:(h + 1) * D]

        split_loop(wq_v, t0_s)
        cur.to(cfg["u_uk"])
        assert cur.pos >= u_ckv
        wait(wuk_v, S_WUK)
        wait(wuv_v, S_WUV)
        split_loop(wuk_v, t1_s)
        iss_q = cur.loop(H // 2, cfg["n_qabs"])

        def qabs_body(j, carry):
            x = x_v[...]
            for p in range(2):
                q = jnp.dot(x, _head(t0_s, j, p, H, M),
                            preferred_element_type=F32).astype(BF16)
                qa = jax.lax.dot_general(q, _head(t1_s, j, p, H, Dc), _NT,
                                         preferred_element_type=F32) * scale
                row = pl.multiple_of((2 * j + p) * B, B)
                for t in range(Dc // 128):
                    qabs_s[t, pl.ds(row, B), :] = qa[:, t * 128:(t + 1) * 128]
            iss_q(j, 0)
            return carry

        jax.lax.fori_loop(0, H // 2, qabs_body, 0)
        split_loop(wuv_v, t0_s)

        cur.to(cfg["u_attn_a"])
        for half in range(2):
            assert cur.pos + half * (B // 2) * sum(cfg["n_attn_a"]) >= u_ckv + (half + 1) * ckv_bursts
        iss_a = cur.loop(B, cfg["n_attn_a"])

        def attn_a(b, carry):
            for half in range(2):
                pl.when(b == half * (B // 2))(
                    lambda: wait(ckv_v.at[pl.ds(half * 2 * NSTR, 2 * NSTR)], S_CKV + half))

            qa = jnp.concatenate(
                [qabs_s[t, pl.ds(b, H, stride=B), :] for t in range(Dc // 128)],
                axis=1).astype(BF16)
            def c_half(k):
                return ckv_v[pl.ds(b * CS + k * (CS // 2), CS // 2)].reshape(Sk // 2, Dc)

            s = []
            for k in range(2):
                s.append(jax.lax.dot_general(qa, c_half(k), _NT, preferred_element_type=F32))
                iss_a(b, k)
            s = jnp.concatenate(s, axis=1)
            m = jnp.max(s, axis=-1, keepdims=True)
            p = jnp.exp(s - m)
            l = jnp.sum(p, axis=-1, keepdims=True)
            p = p.astype(BF16)
            c = ckv_v[pl.ds(b * CS, CS)].reshape(Sk, Dc)
            lat = jnp.dot(p, c, preferred_element_type=F32)
            lat = lat / l
            row = pl.multiple_of(b * H, H)
            for t in range(Dc // 128):
                lat_s[t, pl.ds(row, H), :] = lat[:, t * 128:(t + 1) * 128]
            iss_a(b, 2)
            return carry

        jax.lax.fori_loop(0, B, attn_a, 0)

        iss_c = cur.loop(H // 2, cfg["n_ctx"])

        def ctx_body(j, carry):
            for p in range(2):
                lat = jnp.concatenate(
                    [lat_s[t, pl.ds(2 * j + p, B, stride=H), :] for t in range(Dc // 128)],
                    axis=1).astype(BF16)
                ctx_s[2 * j + p] = jnp.dot(lat, _head(t0_s, j, p, H, Dc),
                                           preferred_element_type=F32)
            iss_c(j, 0)
            return carry

        jax.lax.fori_loop(0, H // 2, ctx_body, 0)

        cur.to(cfg["u_attn_b"])
        for unit in range(B // UB):
            assert (cur.pos + unit * UB * sum(cfg["n_attn_b"]) + cfg["n_attn_b"][0]
                    >= u_kv + (unit + 1) * 2 * kv_bursts)
        iss_b = cur.loop(B, cfg["n_attn_b"])
        first = jax.lax.broadcasted_iota(jnp.int32, (2 * rep, 1), 0) < rep

        def attn_b(b, carry):
            iss_b(b, 0)
            unit, sub = _divmod_pow2(b, UB)

            @pl.when(sub == 0)
            def _():
                wait(kc_v.at[pl.ds(unit * NSTR, NSTR)], S_KV + 2 * unit)
                wait(vc_v.at[pl.ds(unit * NSTR, NSTR)], S_KV + 2 * unit + 1)

            for gp in range(HP):
                if gp == HP // 2:
                    iss_b(b, 1)
                a = b * HP + gp
                q = qb_s[pl.ds(gp * 2 * rep * B + b, 2 * rep, stride=B), :].astype(BF16)
                s0 = jax.lax.dot_general(q, kc_v[a, 0], _NT, preferred_element_type=F32)
                s1 = jax.lax.dot_general(q, kc_v[a, 1], _NT, preferred_element_type=F32)
                s = jnp.where(first, s0, s1) * scale
                m = jnp.max(s, axis=-1, keepdims=True)
                p = jnp.exp(s - m)
                l = jnp.sum(p, axis=-1, keepdims=True)
                p = p.astype(BF16)
                o0 = jnp.dot(p, vc_v[a, 0], preferred_element_type=F32)
                o1 = jnp.dot(p, vc_v[a, 1], preferred_element_type=F32)
                row = pl.multiple_of(a * 2 * rep, 2 * rep)
                ob_s[pl.ds(row, 2 * rep), :] = jnp.where(first, o0, o1) / l
            return carry

        jax.lax.fori_loop(0, B, attn_b, 0)

        def lhs(which, s0, ns, band):
            hs = [s * NBAND + band for s in range(s0, s0 + ns)]
            if which == 0:
                parts = [ctx_s[h] for h in hs]
            else:
                parts = [ob_s[pl.ds(h, B, stride=H), :] for h in hs]
            return jnp.concatenate(parts, axis=1).astype(BF16)

        def proj(l, which, s0, ns, band):
            w = (wo_v, bwo_v)[which][pl.ds(s0, ns), pl.ds(band * D, D), :].reshape(ns * D, M)
            return jnp.dot(l, w, preferred_element_type=F32)

        band_skew, rem = divmod(skew_w3, band_bursts * BURST)
        assert rem == 0

        def do_band(which, k):
            band = k if which else (k - band_skew) % NBAND
            wait((wo_v, bwo_v)[which].at[:, pl.ds(band * D, D)], S_W3 + 2 * band + which)
            r = proj(lhs(which, 0, NSTR, band), which, 0, NSTR, band)
            acc_s[which] = r if k == 0 else acc_s[which] + r

        last = NBAND - 1
        todo = [(which, k) for k in range(NBAND) for which in range(2)][:-1]
        for u, n in cfg["u_band"]:
            cur.to(u)
            for _ in range(n):
                which, k = todo.pop(0)
                assert k < last and cur.pos >= u_w3 + (k + 1) * band_bursts
                do_band(which, k)
        cur.to(n_bursts)

        starts = [sum(tail_blocks[:k]) for k in range(len(tail_blocks))]
        narrow = []
        for k, (s0, ns) in enumerate(zip(starts, tail_blocks)):
            rows = 32 // ns
            narrow += [((pl.ds(s0, ns), pl.ds(r, rows), every), S_TAIL + k)
                       for r in range(last * D, (last + 1) * D, rows)]
        assert len(narrow) == band_bursts * BURST

        def d_narrow(blk, i):
            sl, sem = narrow[(blk - last * band_bursts) * BURST + i]
            start(bwo_h.at[sl], bwo_v.at[sl], sem, 1)

        for u in range(last * band_bursts, w_bursts):
            burst(u, w_bursts, skew_w3, d_wo, d_narrow)

        xf = x_v[...].astype(F32)
        gw = gw_v[...].astype(F32)
        t = xf[:, 0:128] * gw[0:1, :]
        for i in range(1, M // 128):
            t = t + xf[:, i * 128:(i + 1) * 128] * gw[i:i + 1, :]
        gate = jax.nn.sigmoid(jnp.sum(t, axis=-1, keepdims=True))

        for which, k in todo:
            do_band(which, k)
        tail_lhs = [lhs(1, s0, ns, last) for s0, ns in zip(starts, tail_blocks)]
        out = gate * acc_s[0]
        acc = acc_s[1]
        for k, (s0, ns) in enumerate(zip(starts, tail_blocks)):
            wait(bwo_v.at[pl.ds(s0, ns), pl.ds(last * D, D)], S_TAIL + k)
            acc = acc + proj(tail_lhs[k], 1, s0, ns, last)
        o_ref[...] = (out + (1.0 - gate) * acc).astype(o_ref.dtype)

    return kernel, n_sems


DEFAULT_CFG = dict(
    head=(26, 30), skews=(28, 27, 26, 32),
    u_q=22, split_steps=8, n_split=(1,), u_uk=38, n_qabs=(1,),
    u_attn_a=80, n_attn_a=(2, 2, 2),
    n_ctx=(1,),
    u_attn_b=148, n_attn_b=(2, 1),
    u_band=((172, 2),),
    tail_blocks=(4, 2, 1, 1),
)
DEFAULT_PARAMS = dict(disable_bounds_checks=True, disable_semaphore_checks=True)


def _compiler_params(params):
    vmem = 112 * 1024 * 1024
    try:
        return pltpu.CompilerParams(vmem_limit_bytes=vmem, **params)
    except TypeError:
        params = {k: v for k, v in params.items() if k != "disable_semaphore_checks"}
        return pltpu.CompilerParams(vmem_limit_bytes=vmem, **params)


def _forward(A_x, A_c_kv, A_w_q, A_w_uk, A_w_uv, A_w_o, B_k_cache, B_v_cache, B_wq, B_wo,
             gate_w, cfg, params):
    B, Sq, M = A_x.shape
    assert Sq == 1
    _, Sk, Dc = A_c_kv.shape
    _, H, D = A_w_q.shape
    _, Hkv, SkB, _ = B_k_cache.shape
    W = min(4096, max(256, SkB // 4))
    HD = H * D

    kernel, n_sems = _make_kernel(B, M, H, D, Dc, Sk, Hkv, SkB, W, cfg)
    any_spec = pl.BlockSpec(memory_space=pl.ANY)
    out = pl.pallas_call(
        kernel,
        out_shape=jax.ShapeDtypeStruct((B, M), A_x.dtype),
        in_specs=[any_spec] * 11,
        out_specs=pl.BlockSpec(memory_space=pltpu.VMEM),
        scratch_shapes=[
            pltpu.VMEM((B, M), BF16),
            pltpu.VMEM((M // 128, 128), BF16),
            pltpu.VMEM((B * 4, Sk // 4, Dc), BF16),
            pltpu.VMEM((NSTR, M * H // NSTR, D), BF16),
            pltpu.VMEM((NSTR, Dc * H // NSTR, D), BF16),
            pltpu.VMEM((NSTR, Dc * H // NSTR, D), BF16),
            pltpu.VMEM((NSTR, HD // NSTR, M), BF16),
            pltpu.VMEM((B * Hkv // 2, 2, W, D), BF16),
            pltpu.VMEM((B * Hkv // 2, 2, W, D), BF16),
            pltpu.VMEM((NSTR, M // NSTR, HD), BF16),
            pltpu.VMEM((NSTR, HD // NSTR, M), BF16),
            pltpu.VMEM(((H + 1) * PLANE, D), U32),
            pltpu.VMEM(((H + 1) * PLANE, D), U32),
            pltpu.VMEM((Dc // 128, (H + 1) * B, 128), F32),
            pltpu.VMEM((Dc // 128, (B + 1) * H, 128), F32),
            pltpu.VMEM((H, B, D), F32),
            pltpu.VMEM(((H + 1) * B, D), F32),
            pltpu.VMEM(((B + 1) * H, D), F32),
            pltpu.VMEM((2, B, M), F32),
            pltpu.SemaphoreType.DMA((n_sems,)),
        ],
        compiler_params=_compiler_params(params),
        name="gated_mix_decode",
    )(
        A_x.reshape(B, M),
        gate_w.reshape(M // 128, 128),
        A_c_kv.reshape(B * 4, Sk // 4, Dc),
        A_w_q.reshape(NSTR, M * H // NSTR, D),
        A_w_uk.reshape(NSTR, Dc * H // NSTR, D),
        A_w_uv.reshape(NSTR, Dc * H // NSTR, D),
        A_w_o.reshape(NSTR, HD // NSTR, M),
        B_k_cache.reshape(B * Hkv // 2, 2, SkB, D),
        B_v_cache.reshape(B * Hkv // 2, 2, SkB, D),
        B_wq.reshape(NSTR, M // NSTR, HD),
        B_wo.reshape(NSTR, HD // NSTR, M),
    )
    return out.reshape(B, 1, M)


@jax.jit
def pallas_gated_mix__compressed_kv_cla__sliding_block_cached__decode_kernel(
    A_x: jax.Array,
    A_c_kv: jax.Array,
    A_w_q: jax.Array,
    A_w_uk: jax.Array,
    A_w_uv: jax.Array,
    A_w_o: jax.Array,
    B_x: jax.Array,
    B_k_cache: jax.Array,
    B_v_cache: jax.Array,
    B_wq: jax.Array,
    B_wo: jax.Array,
    gate_w: jax.Array,
):
    return _forward(A_x, A_c_kv, A_w_q, A_w_uk, A_w_uv, A_w_o, B_k_cache, B_v_cache,
                    B_wq, B_wo, gate_w, DEFAULT_CFG, DEFAULT_PARAMS)
```

```python
import jax
import jax.numpy as jnp
import jax.experimental.pallas as pl
import jax.experimental.pallas.tpu as pltpu

F32 = jnp.float32
BF16 = jnp.bfloat16
U32 = jnp.uint32

_NT = (((1,), (1,)), ((), ()))

NSTR = 8
BURST = 8
PLANE = 264


def _divmod_pow2(u, n, nq=None):
    assert n & (n - 1) == 0
    q = u >> (n.bit_length() - 1)
    if nq is not None:
        assert nq & (nq - 1) == 0
        q = q & (nq - 1)
    return q, u & (n - 1)


def _mult(v, n):
    return v if isinstance(v, int) else pl.multiple_of(v, n)


def _split_heads(w_v, t_s, step, nsteps, heads):
    ns, rr, _ = w_v.shape
    per_stream = nsteps // ns
    stream, part = _divmod_pow2(step, per_stream)
    rows = rr // per_stream
    half = heads // 2
    for k in range(rows // (2 * heads)):
        r0 = pl.multiple_of(part * rows + k * 2 * heads, 2 * heads)
        w = pltpu.bitcast(w_v[stream, pl.ds(r0, 2 * heads), :], U32)
        ev, od = w[:half], w[half:]
        lo = (ev & jnp.uint32(0xFFFF)) | (od << 16)
        hi = (ev >> 16) | (od & jnp.uint32(0xFFFF0000))
        i = step * (rows // (2 * heads)) + k
        t_s[pl.ds(i, half, stride=PLANE), :] = lo
        t_s[pl.ds(half * PLANE + i, half, stride=PLANE), :] = hi


def _head(t_s, j, p, heads, rows):
    r0 = pl.multiple_of((p * (heads // 2) + j) * PLANE, 8)
    return pltpu.bitcast(t_s[pl.ds(r0, rows // 2), :], BF16)


def _make_kernel(B, M, H, D, Dc, Sk, Hkv, SkB, W, cfg):
    rep = H // Hkv
    scale = float(D) ** -0.5
    HD = H * D
    CS = 4
    CR = Sk // CS
    OR = HD // NSTR
    NBAND = OR // D
    HP = Hkv // 2
    UB = NSTR // HP
    tail_blocks = cfg["tail_blocks"]
    skew_w2, skew_ckv, skew_kv, skew_w3 = cfg["skews"]
    assert sum(tail_blocks) == NSTR and max(M, Dc) // 2 <= PLANE

    S_X, S_GW, S_WQ, S_WUK, S_BWQ, S_WUV, S_CKV = 0, 1, 2, 3, 4, 5, 6
    S_KV = S_CKV + 2
    S_W3 = S_KV + 2 * (B // UB)
    S_TAIL = S_W3 + 2 * NBAND - 1
    n_sems = S_TAIL + len(tail_blocks)

    def body(x_h, gw_h, ckv_h, wq_h, wuk_h, wuv_h, wo_h, kc_h, vc_h, bwq_h, bwo_h,
             o_ref,
             x_v, gw_v, ckv_v, wq_v, wuk_v, wuv_v, wo_v, kc_v, vc_v, bwq_v, bwo_v,
             t0_s, t1_s, qabs_s, lat_s, ctx_s, qb_s, ob_s, acc_s, sems):
        def start(src, dst, sem, prio):
            pltpu.make_async_copy(src, dst, sems.at[sem]).start(priority=prio)

        def wait(buf, sem):
            pltpu.make_async_copy(buf, buf, sems.at[sem]).wait()

        every = slice(None)

        def rows16(src, dst, r, sem, prio):
            sl = (every, pl.ds(_mult(r, 16), 16), every)
            start(src.at[sl], dst.at[sl], sem, prio)

        def tiles2(src, dst, lead, r, c, sem, prio):
            sl = (lead, pl.ds(_mult(r, 8), 8), pl.ds(_mult(c, 256), 256))
            start(src.at[sl], dst.at[sl], sem, prio)

        def burst(u, nblk, skew, d0, d1):
            q, r = divmod(skew, BURST)
            blk0 = [(u - q - 1) & (nblk - 1), (u - q) & (nblk - 1)]
            for i in range(BURST):
                d0(blk0[i >= r], (i - r) % BURST)
                d1(u & (nblk - 1), i)

        def d_rows(src, dst, sem, prio):
            return lambda blk, i: rows16(src, dst, blk * (16 * BURST) + 16 * i, sem, prio)

        def d_tiles(src, dst, lead, sem, prio):
            nc = src.shape[-1] // 256

            def f(blk, i):
                r, c = blk * (8 * BURST // nc) + 8 * (i // nc), 256 * (i % nc)
                tiles2(src, dst, lead, r, c, sem(blk) if callable(sem) else sem, prio)
            return f

        w_bursts = wq_v.shape[1] // 16 // BURST

        def burst_w2(u):
            burst(u, w_bursts, skew_w2, d_rows(wuk_h, wuk_v, S_WUK, 0),
                  d_rows(wuv_h, wuv_v, S_WUV, 1))

        ckv_bursts = (CR // 8) * (Dc // 256) // BURST

        def burst_ckv(u):
            half, uu = _divmod_pow2(u, ckv_bursts, 2)
            d = [d_tiles(ckv_h, ckv_v, pl.ds(half * (2 * NSTR) + t * NSTR, NSTR), S_CKV + half, t)
                 for t in range(2)]
            burst(uu, ckv_bursts, skew_ckv, *d)

        kv_bursts = W // 16 // BURST

        def burst_kv(u):
            q, uu = _divmod_pow2(u, kv_bursts, 2 * (B // UB))
            unit, which = _divmod_pow2(q, 2)
            lead = pl.ds(unit * NSTR, NSTR)

            def go(src, dst):
                def d(t):
                    def f(blk, i):
                        r = blk * (16 * BURST) + 16 * i
                        start(src.at[lead, t, pl.ds(_mult(SkB - W + r, 16), 16)],
                              dst.at[lead, t, pl.ds(_mult(r, 16), 16)], S_KV + q, t)
                    return f
                burst(uu, kv_bursts, skew_kv, d(0), d(1))

            pl.when(which == 0)(lambda: go(kc_h, kc_v))
            pl.when(which == 1)(lambda: go(vc_h, vc_v))

        band_bursts = w_bursts // NBAND
        d_wo = d_tiles(wo_h, wo_v, every,
                       lambda blk: S_W3 + 2 * _divmod_pow2(blk, band_bursts)[0], 0)
        d_bwo = d_tiles(bwo_h, bwo_v, every,
                        lambda blk: S_W3 + 2 * _divmod_pow2(blk, band_bursts)[0] + 1, 1)

        def burst_w3(u):
            burst(u, w_bursts, skew_w3, d_wo, d_bwo)

        plan = []
        u0 = w_bursts
        for fn, n in ((burst_w2, w_bursts),
                      (burst_ckv, 2 * ckv_bursts),
                      (burst_kv, B * kv_bursts),
                      (burst_w3, (NBAND - 1) * band_bursts)):
            plan.append((u0, n, fn))
            u0 += n
        n_bursts = u0
        u_w2, u_ckv, u_kv, u_w3 = (p[0] for p in plan)

        def issue(first, count, lo, hi):
            hits = [(u0, n, fn) for u0, n, fn in plan if u0 < hi and lo < u0 + n]

            def one(u):
                for u0, n, fn in hits:
                    if len(hits) == 1:
                        fn(u - u0)
                    else:
                        pl.when(jnp.logical_and(u >= u0, u < u0 + n))(lambda: fn(u - u0))

            if count == 1:
                one(first)
            else:
                def body(i, c):
                    one(first + i)
                    return c
                jax.lax.fori_loop(0, count, body, 0)

        class Cursor:
            pos = u_w2

            def to(self, hi):
                assert self.pos <= hi <= n_bursts, (self.pos, hi)
                for u0, n, _ in plan:
                    a, b = max(self.pos, u0), min(hi, u0 + n)
                    if a < b:
                        issue(a, b - a, a, b)
                self.pos = hi

            def loop(self, iters, counts):
                per = sum(counts)
                lo, hi = self.pos, self.pos + iters * per
                assert hi <= n_bursts
                self.pos = hi

                def f(i, k):
                    if counts[k]:
                        issue(lo + i * per + sum(counts[:k]), counts[k], lo, hi)
                return f

        cur = Cursor()

        def split_loop(w_v, t_s):
            n = cfg["split_steps"]
            iss = cur.loop(n, cfg["n_split"])

            def body(i, carry):
                iss(i, 0)
                _split_heads(w_v, t_s, i, n, H)
                return carry

            jax.lax.fori_loop(0, n, body, 0)

        head, rot = cfg["head"]
        n = w_bursts * BURST

        def wq_piece(j, prio):
            rows16(wq_h, wq_v, ((j + rot) & (n - 1)) * 16, S_WQ, prio)

        def bwq_piece(j):
            rb, cb = _divmod_pow2(j, HD // 256, M // NSTR // 8)
            tiles2(bwq_h, bwq_v, every, rb * 8, cb * 256, S_BWQ, 1)

        def repeat(count, f):
            def body(j, carry):
                f(j)
                return carry
            jax.lax.fori_loop(0, count, body, 0)

        assert head % 2 == 0
        for j in range(head):
            bwq_piece(j)
        repeat(n - head, lambda j: (wq_piece(j, 0), bwq_piece(j + head)))
        repeat(head // 2, lambda j: (wq_piece(n - head + j, 0), wq_piece(n - head // 2 + j, 1)))
        start(x_h, x_v, S_X, 0)
        start(gw_h, gw_v, S_GW, 1)
        cur.to(cfg["u_q"])

        wait(x_v, S_X)
        wait(gw_v, S_GW)
        wait(wq_v, S_WQ)
        wait(bwq_v, S_BWQ)
        qb = jnp.dot(x_v[...], bwq_v[...].reshape(M, HD), preferred_element_type=F32)
        qb = qb.astype(BF16).astype(F32)
        for h in range(H):
            qb_s[h * B:(h + 1) * B, :] = qb[:, h * D:(h + 1) * D]

        split_loop(wq_v, t0_s)
        cur.to(cfg["u_uk"])
        assert cur.pos >= u_ckv
        wait(wuk_v, S_WUK)
        wait(wuv_v, S_WUV)
        split_loop(wuk_v, t1_s)
        iss_q = cur.loop(H // 2, cfg["n_qabs"])

        def qabs_body(j, carry):
            x = x_v[...]
            for p in range(2):
                q = jnp.dot(x, _head(t0_s, j, p, H, M),
                            preferred_element_type=F32).astype(BF16)
                qa = jax.lax.dot_general(q, _head(t1_s, j, p, H, Dc), _NT,
                                         preferred_element_type=F32) * scale
                row = pl.multiple_of((2 * j + p) * B, B)
                for t in range(Dc // 128):
                    qabs_s[t, pl.ds(row, B), :] = qa[:, t * 128:(t + 1) * 128]
            iss_q(j, 0)
            return carry

        jax.lax.fori_loop(0, H // 2, qabs_body, 0)
        split_loop(wuv_v, t0_s)

        cur.to(cfg["u_attn_a"])
        for half in range(2):
            assert cur.pos + half * (B // 2) * sum(cfg["n_attn_a"]) >= u_ckv + (half + 1) * ckv_bursts
        iss_a = cur.loop(B, cfg["n_attn_a"])

        def attn_a(b, carry):
            for half in range(2):
                pl.when(b == half * (B // 2))(
                    lambda: wait(ckv_v.at[pl.ds(half * 2 * NSTR, 2 * NSTR)], S_CKV + half))

            qa = jnp.concatenate(
                [qabs_s[t, pl.ds(b, H, stride=B), :] for t in range(Dc // 128)],
                axis=1).astype(BF16)
            def c_half(k):
                return ckv_v[pl.ds(b * CS + k * (CS // 2), CS // 2)].reshape(Sk // 2, Dc)

            s = []
            for k in range(2):
                s.append(jax.lax.dot_general(qa, c_half(k), _NT, preferred_element_type=F32))
                iss_a(b, k)
            s = jnp.concatenate(s, axis=1)
            m = jnp.max(s, axis=-1, keepdims=True)
            p = jnp.exp(s - m)
            l = jnp.sum(p, axis=-1, keepdims=True)
            p = p.astype(BF16)
            c = ckv_v[pl.ds(b * CS, CS)].reshape(Sk, Dc)
            lat = jnp.dot(p, c, preferred_element_type=F32)
            lat = lat / l
            row = pl.multiple_of(b * H, H)
            for t in range(Dc // 128):
                lat_s[t, pl.ds(row, H), :] = lat[:, t * 128:(t + 1) * 128]
            iss_a(b, 2)
            return carry

        jax.lax.fori_loop(0, B, attn_a, 0)

        iss_c = cur.loop(H // 2, cfg["n_ctx"])

        def ctx_body(j, carry):
            for p in range(2):
                lat = jnp.concatenate(
                    [lat_s[t, pl.ds(2 * j + p, B, stride=H), :] for t in range(Dc // 128)],
                    axis=1).astype(BF16)
                ctx_s[2 * j + p] = jnp.dot(lat, _head(t0_s, j, p, H, Dc),
                                           preferred_element_type=F32)
            iss_c(j, 0)
            return carry

        jax.lax.fori_loop(0, H // 2, ctx_body, 0)

        cur.to(cfg["u_attn_b"])
        for unit in range(B // UB):
            assert (cur.pos + unit * UB * sum(cfg["n_attn_b"]) + cfg["n_attn_b"][0]
                    >= u_kv + (unit + 1) * 2 * kv_bursts)
        iss_b = cur.loop(B, cfg["n_attn_b"])
        first = jax.lax.broadcasted_iota(jnp.int32, (2 * rep, 1), 0) < rep

        def attn_b(b, carry):
            iss_b(b, 0)
            unit, sub = _divmod_pow2(b, UB)

            @pl.when(sub == 0)
            def _():
                wait(kc_v.at[pl.ds(unit * NSTR, NSTR)], S_KV + 2 * unit)
                wait(vc_v.at[pl.ds(unit * NSTR, NSTR)], S_KV + 2 * unit + 1)

            for gp in range(HP):
                if gp == HP // 2:
                    iss_b(b, 1)
                a = b * HP + gp
                q = qb_s[pl.ds(gp * 2 * rep * B + b, 2 * rep, stride=B), :].astype(BF16)
                s0 = jax.lax.dot_general(q, kc_v[a, 0], _NT, preferred_element_type=F32)
                s1 = jax.lax.dot_general(q, kc_v[a, 1], _NT, preferred_element_type=F32)
                s = jnp.where(first, s0, s1) * scale
                m = jnp.max(s, axis=-1, keepdims=True)
                p = jnp.exp(s - m)
                l = jnp.sum(p, axis=-1, keepdims=True)
                p = p.astype(BF16)
                o0 = jnp.dot(p, vc_v[a, 0], preferred_element_type=F32)
                o1 = jnp.dot(p, vc_v[a, 1], preferred_element_type=F32)
                row = pl.multiple_of(a * 2 * rep, 2 * rep)
                ob_s[pl.ds(row, 2 * rep), :] = jnp.where(first, o0, o1) / l
            return carry

        jax.lax.fori_loop(0, B, attn_b, 0)

        def lhs(which, s0, ns, band):
            hs = [s * NBAND + band for s in range(s0, s0 + ns)]
            if which == 0:
                parts = [ctx_s[h] for h in hs]
            else:
                parts = [ob_s[pl.ds(h, B, stride=H), :] for h in hs]
            return jnp.concatenate(parts, axis=1).astype(BF16)

        def proj(l, which, s0, ns, band):
            w = (wo_v, bwo_v)[which][pl.ds(s0, ns), pl.ds(band * D, D), :].reshape(ns * D, M)
            return jnp.dot(l, w, preferred_element_type=F32)

        band_skew, rem = divmod(skew_w3, band_bursts * BURST)
        assert rem == 0

        def do_band(which, k):
            band = k if which else (k - band_skew) % NBAND
            wait((wo_v, bwo_v)[which].at[:, pl.ds(band * D, D)], S_W3 + 2 * band + which)
            r = proj(lhs(which, 0, NSTR, band), which, 0, NSTR, band)
            acc_s[which] = r if k == 0 else acc_s[which] + r

        last = NBAND - 1
        todo = [(which, k) for k in range(NBAND) for which in range(2)][:-1]
        for u, n in cfg["u_band"]:
            cur.to(u)
            for _ in range(n):
                which, k = todo.pop(0)
                assert k < last and cur.pos >= u_w3 + (k + 1) * band_bursts
                do_band(which, k)
        cur.to(n_bursts)

        starts = [sum(tail_blocks[:k]) for k in range(len(tail_blocks))]
        narrow = []
        for k, (s0, ns) in enumerate(zip(starts, tail_blocks)):
            rows = 32 // ns
            narrow += [((pl.ds(s0, ns), pl.ds(r, rows), every), S_TAIL + k)
                       for r in range(last * D, (last + 1) * D, rows)]
        assert len(narrow) == band_bursts * BURST

        def d_narrow(blk, i):
            sl, sem = narrow[(blk - last * band_bursts) * BURST + i]
            start(bwo_h.at[sl], bwo_v.at[sl], sem, 1)

        for u in range(last * band_bursts, w_bursts):
            burst(u, w_bursts, skew_w3, d_wo, d_narrow)

        xf = x_v[...].astype(F32)
        gw = gw_v[...].astype(F32)
        t = xf[:, 0:128] * gw[0:1, :]
        for i in range(1, M // 128):
            t = t + xf[:, i * 128:(i + 1) * 128] * gw[i:i + 1, :]
        gate = jax.nn.sigmoid(jnp.sum(t, axis=-1, keepdims=True))

        for which, k in todo:
            do_band(which, k)
        tail_lhs = [lhs(1, s0, ns, last) for s0, ns in zip(starts, tail_blocks)]
        out = gate * acc_s[0]
        acc = acc_s[1]
        for k, (s0, ns) in enumerate(zip(starts, tail_blocks)):
            wait(bwo_v.at[pl.ds(s0, ns), pl.ds(last * D, D)], S_TAIL + k)
            acc = acc + proj(tail_lhs[k], 1, s0, ns, last)
        o_ref[...] = (out + (1.0 - gate) * acc).astype(o_ref.dtype)

    def kernel(*refs):
        pl.run_scoped(lambda sems: body(*refs, sems), pltpu.SemaphoreType.DMA((n_sems,)))

    return kernel


DEFAULT_CFG = dict(
    head=(26, 30), skews=(28, 27, 26, 32),
    u_q=22, split_steps=8, n_split=(1,), u_uk=38, n_qabs=(1,),
    u_attn_a=80, n_attn_a=(2, 2, 2),
    n_ctx=(1,),
    u_attn_b=148, n_attn_b=(2, 1),
    u_band=((172, 2),),
    tail_blocks=(4, 2, 1, 1),
)


def _forward(A_x, A_c_kv, A_w_q, A_w_uk, A_w_uv, A_w_o, B_k_cache, B_v_cache, B_wq, B_wo,
             gate_w, cfg):
    B, Sq, M = A_x.shape
    assert Sq == 1
    _, Sk, Dc = A_c_kv.shape
    _, H, D = A_w_q.shape
    _, Hkv, SkB, _ = B_k_cache.shape
    W = min(4096, max(256, SkB // 4))
    HD = H * D

    kernel = _make_kernel(B, M, H, D, Dc, Sk, Hkv, SkB, W, cfg)
    any_spec = pl.BlockSpec(memory_space=pl.ANY)
    out = pl.pallas_call(
        kernel,
        out_shape=jax.ShapeDtypeStruct((B, M), A_x.dtype),
        in_specs=[any_spec] * 11,
        out_specs=pl.BlockSpec(memory_space=pltpu.VMEM),
        scratch_shapes=[
            pltpu.VMEM((B, M), BF16),
            pltpu.VMEM((M // 128, 128), BF16),
            pltpu.VMEM((B * 4, Sk // 4, Dc), BF16),
            pltpu.VMEM((NSTR, M * H // NSTR, D), BF16),
            pltpu.VMEM((NSTR, Dc * H // NSTR, D), BF16),
            pltpu.VMEM((NSTR, Dc * H // NSTR, D), BF16),
            pltpu.VMEM((NSTR, HD // NSTR, M), BF16),
            pltpu.VMEM((B * Hkv // 2, 2, W, D), BF16),
            pltpu.VMEM((B * Hkv // 2, 2, W, D), BF16),
            pltpu.VMEM((NSTR, M // NSTR, HD), BF16),
            pltpu.VMEM((NSTR, HD // NSTR, M), BF16),
            pltpu.VMEM(((H + 1) * PLANE, D), U32),
            pltpu.VMEM(((H + 1) * PLANE, D), U32),
            pltpu.VMEM((Dc // 128, (H + 1) * B, 128), F32),
            pltpu.VMEM((Dc // 128, (B + 1) * H, 128), F32),
            pltpu.VMEM((H, B, D), F32),
            pltpu.VMEM(((H + 1) * B, D), F32),
            pltpu.VMEM(((B + 1) * H, D), F32),
            pltpu.VMEM((2, B, M), F32),
        ],
        compiler_params=pltpu.CompilerParams(vmem_limit_bytes=112 * 1024 * 1024),
        name="gated_mix_decode",
    )(
        A_x.reshape(B, M),
        gate_w.reshape(M // 128, 128),
        A_c_kv.reshape(B * 4, Sk // 4, Dc),
        A_w_q.reshape(NSTR, M * H // NSTR, D),
        A_w_uk.reshape(NSTR, Dc * H // NSTR, D),
        A_w_uv.reshape(NSTR, Dc * H // NSTR, D),
        A_w_o.reshape(NSTR, HD // NSTR, M),
        B_k_cache.reshape(B * Hkv // 2, 2, SkB, D),
        B_v_cache.reshape(B * Hkv // 2, 2, SkB, D),
        B_wq.reshape(NSTR, M // NSTR, HD),
        B_wo.reshape(NSTR, HD // NSTR, M),
    )
    return out.reshape(B, 1, M)


@jax.jit
def pallas_gated_mix__compressed_kv_cla__sliding_block_cached__decode_kernel(
    A_x: jax.Array,
    A_c_kv: jax.Array,
    A_w_q: jax.Array,
    A_w_uk: jax.Array,
    A_w_uv: jax.Array,
    A_w_o: jax.Array,
    B_x: jax.Array,
    B_k_cache: jax.Array,
    B_v_cache: jax.Array,
    B_wq: jax.Array,
    B_wo: jax.Array,
    gate_w: jax.Array,
):
    return _forward(A_x, A_c_kv, A_w_q, A_w_uk, A_w_uv, A_w_o, B_k_cache, B_v_cache,
                    B_wq, B_wo, gate_w, DEFAULT_CFG)
```
